```python
import jax
import jax.numpy as jnp

def _softmax(x, axis=-1):
    return jax.nn.softmax(x, axis=axis)

def _gelu(x):
    return jax.nn.gelu(x, approximate=True)

def _silu(x):
    return jax.nn.silu(x)

def _sigmoid(x):
    return jax.nn.sigmoid(x)

def _layernorm(x, axis=-1, eps=1e-05):
    m = jnp.mean(x, axis=axis, keepdims=True)
    v = jnp.var(x, axis=axis, keepdims=True)
    return (x - m) / jnp.sqrt(v + eps)

def _scatter_add(tgt, idx, src, axis=0):
    return tgt.at[idx].add(src)

def _segment_sum(src, seg, n):
    return jax.ops.segment_sum(src, seg, n)

class _Rng:

    def __init__(self, key):
        self._k = key

    def _next(self):
        self._k, sub = jax.random.split(self._k)
        return sub

    def normal(self, shape):
        return jax.random.normal(self._next(), shape, dtype=jnp.bfloat16)

    def randint(self, lo, hi, shape):
        return jax.random.randint(self._next(), shape, lo, hi, dtype=jnp.int32)

    def uniform(self, shape, lo=0.0, hi=1.0):
        return jax.random.uniform(self._next(), shape, jnp.bfloat16, lo, hi)

    def permutation(self, n):
        return jax.random.permutation(self._next(), n)
kernel_name = 'adaLN_cond__sliding_local_dilated__glu_gated_bilinear__prompt'

def setup_inputs():
    _rng = _Rng(jax.random.key(int.from_bytes(__import__("os").urandom(4), "little")))
    _w = lambda a: (lambda t: t.astype(jnp.bfloat16) if jnp.issubdtype(t.dtype, jnp.floating) else t)(jnp.asarray(a))

    def _A_setup():
        B, S, D = (1, 2048, 576)
        return {'x': _w((lambda *s: _rng.normal(s) * 0.05)(B, S, D)), 'wqkv': _w((lambda *s: _rng.normal(s) * 0.05)(D, 3 * D)), 'wo': _w((lambda *s: _rng.normal(s) * 0.05)(D, D))}
    _A_in = _A_setup()

    def _B_setup():
        B, S, D, F = (1, 2048, 576, 4608)
        return {'x': _w((lambda *s: _rng.normal(s) * 0.05)(B, S, D)), 'w_gate': _w((lambda *s: _rng.normal(s) * 0.05)(D, F) * D ** (-0.5)), 'w_up': _w((lambda *s: _rng.normal(s) * 0.05)(D, F) * D ** (-0.5)), 'w_down': _w((lambda *s: _rng.normal(s) * 0.05)(F, D) * F ** (-0.5))}
    _B_in = _B_setup()
    return {'A_x': _A_in['x'], 'A_wqkv': _A_in['wqkv'], 'A_wo': _A_in['wo'], 'B_x': _B_in['x'], 'B_w_gate': _B_in['w_gate'], 'B_w_up': _B_in['w_up'], 'B_w_down': _B_in['w_down'], 'c': _w((lambda *s: _rng.normal(s) * 0.05)(1, 576)), 'w_mod': _w((lambda *s: _rng.normal(s) * 0.05)(576, 6 * 576) * 576 ** (-0.5))}

def reference(A_x, A_wqkv, A_wo, B_x, B_w_gate, B_w_up, B_w_down, c, w_mod):

    def _A_ref(x, wqkv, wo):
        B, S, D = x.shape
        H = 32
        Dh = D // H
        W, dil = (8, 2)
        qkv = (lambda x, *d: x.transpose(*d))((x @ wqkv).reshape(B, S, 3, H, Dh), 2, 0, 3, 1, 4)
        q, k, v = (qkv[0], qkv[1], qkv[2])
        scale = Dh ** (-0.5)
        pos = jnp.arange(S)
        off = jnp.arange(W) * dil
        idx = pos[:, None] - off[None, :]
        mask = idx >= 0
        idx_c = jnp.where(mask, idx, 0).reshape(-1)
        kg = k[:, :, idx_c, :].reshape(B, H, S, W, Dh)
        vg = v[:, :, idx_c, :].reshape(B, H, S, W, Dh)
        logits = jnp.einsum('bhsd,bhswd->bhsw', q, kg) * scale
        logits = jnp.where(mask[None, None, :, :], logits, -1000000000.0)
        attn = _softmax(logits, axis=-1)
        o = jnp.einsum('bhsw,bhswd->bhsd', attn, vg)
        return (lambda x, *d: x.transpose(*d))(o, 0, 2, 1, 3).reshape(B, S, D) @ wo

    def _B_ref(x, w_gate, w_up, w_down):
        g = jnp.einsum('bsd,df->bsf', x, w_gate)
        u = jnp.einsum('bsd,df->bsf', x, w_up)
        h = g * u
        return jnp.einsum('bsf,fd->bsd', h, w_down)
    x = A_x
    mod = (_silu(c) @ w_mod).reshape(c.shape[0], 6, 1, -1)
    sa, ca, ga, sb, cb, gb = (mod[:, 0].copy(), mod[:, 1].copy(), mod[:, 2].copy(), mod[:, 3].copy(), mod[:, 4].copy(), mod[:, 5].copy())
    h = _layernorm(x, axis=-1) * (1 + ca) + sa
    x = x + ga * _A_ref(h, A_wqkv, A_wo)
    h = _layernorm(x, axis=-1) * (1 + cb) + sb
    x = x + gb * _B_ref(h, B_w_gate, B_w_up, B_w_down)
    return x
```

```python
import functools
import jax
import jax.numpy as jnp
from jax import lax
from jax.experimental import pallas as pl
from jax.experimental.pallas import tpu as pltpu

S, D, F = 2048, 576, 4608
H, DH, W, DIL = 32, 18, 8, 2
EPS = 1e-5
NT_DIMS = (((1,), (1,)), ((), ()))
LANES = 128
NTILE = S // LANES
f32, bf16, u32 = jnp.float32, jnp.bfloat16, jnp.uint32


def _unpack(w):
    lo = pltpu.unpack_elementwise(w, index=0, packed_dtype=bf16, unpacked_dtype=f32)
    hi = pltpu.unpack_elementwise(w, index=1, packed_dtype=bf16, unpacked_dtype=f32)
    return lo, hi


def _ln_mod(x, scale1, shift):
    m = jnp.sum(x, axis=0, keepdims=True) * (1.0 / D)
    xc = x - m
    v = jnp.sum(xc * xc, axis=0, keepdims=True) * (1.0 / D)
    return xc * lax.rsqrt(v + EPS) * scale1 + shift


def make_kernel(TA=512, TF=512, order="pipe"):
    na = S // TA
    tpa = TA // LANES
    nf = S // TF

    def kern(xT_hbm, wqkv_hbm, wo_hbm, wg_hbm, wu_hbm, wdT_hbm, c_hbm, wmod_hbm, out_hbm,
             x_s, wqkv_s, wo_s, wg_s, wu_s, wdT_s, c_s, wmod_s,
             wqkvT_s, woT_s, mod_s, qkv_s, o_s, x1_s, h2_s, out_s, sems, osems):
        cp_c = pltpu.make_async_copy(c_hbm, c_s, sems.at[0])
        cp_m0 = pltpu.make_async_copy(wmod_hbm.at[:, pl.ds(0, 2 * D)], wmod_s.at[:, pl.ds(0, 2 * D)], sems.at[1])
        cp_m1 = pltpu.make_async_copy(wmod_hbm.at[:, pl.ds(2 * D, 4 * D)], wmod_s.at[:, pl.ds(2 * D, 4 * D)], sems.at[2])
        cp_wqkv = pltpu.make_async_copy(wqkv_hbm, wqkv_s, sems.at[3])
        cp_wo = pltpu.make_async_copy(wo_hbm, wo_s, sems.at[4])
        cp_wg = pltpu.make_async_copy(wg_hbm, wg_s, sems.at[5])
        cp_wu = pltpu.make_async_copy(wu_hbm, wu_s, sems.at[6])
        cp_wd = pltpu.make_async_copy(wdT_hbm, wdT_s, sems.at[7])
        cp_x = [pltpu.make_async_copy(xT_hbm.at[:, pl.ds(i * TA, TA)], x_s.at[:, pl.ds(i * TA, TA)], sems.at[8 + i])
                for i in range(na)]
        cp_c.start(); cp_m0.start(); cp_wqkv.start(); cp_x[0].start()
        cp_m1.start(); cp_wo.start()
        for i in range(1, na):
            cp_x[i].start()
        cp_wg.start(); cp_wu.start(); cp_wd.start()

        cp_c.wait()
        cv = c_s[...].astype(f32)
        sc = (cv * jax.nn.sigmoid(cv)).astype(bf16)
        sc = jnp.broadcast_to(sc, (16, D))

        def mod_part(c0, n):
            r = jnp.dot(sc, wmod_s[:, c0:c0 + n], preferred_element_type=f32)
            for j in range(n // LANES):
                t = jnp.broadcast_to(r[0:1, j * LANES:(j + 1) * LANES], (LANES, LANES))
                mod_s[c0 + j * LANES:c0 + (j + 1) * LANES, :] = t.T

        def mod(i):
            return mod_s[i * D:(i + 1) * D, :]

        cp_m0.wait()
        mod_part(0, 2 * D)
        cp_wqkv.wait()
        wqkvT_s[...] = wqkv_s[...].T

        def stage_qkv(i):
            cp_x[i].wait()
            hs = []
            for t in range(tpa):
                n = i * tpa + t
                x = x_s[:, n * LANES:(n + 1) * LANES].astype(f32)
                hs.append(_ln_mod(x, 1.0 + mod(1), mod(0)).astype(bf16))
            h = jnp.concatenate(hs, axis=1)
            qkv = jnp.dot(wqkvT_s[...], h, preferred_element_type=f32).astype(bf16)
            for t in range(tpa):
                qkv_s[1 + i * tpa + t] = pltpu.bitcast(qkv[:, t * LANES:(t + 1) * LANES], u32)
            if i == 0:
                qkv_s[0, pl.ds(D // 2, D), :] = jnp.broadcast_to(qkv_s[1, pl.ds(D // 2, D), 0:1], (D, LANES))

        lane = lax.broadcasted_iota(jnp.int32, (8, LANES), 1)

        def shifted(cur, prev):
            out = [cur]
            for w in range(1, W):
                s = DIL * w
                out.append(pltpu.roll(jnp.where(lane >= LANES - s, prev, cur), s, 1))
            return out

        def attn_unit(n, hg):
            acc = [None] * W
            for p in range(DH // 2):
                rows = lambda part: pl.ds(part * (D // 2) + hg * 8 * (DH // 2) + p, 8, stride=DH // 2)
                qlo, qhi = _unpack(qkv_s[n + 1, rows(0), :])
                ks = shifted(qkv_s[n + 1, rows(1), :], qkv_s[n, rows(1), :])
                for w in range(W):
                    klo, khi = _unpack(ks[w])
                    t = qlo * klo + qhi * khi
                    acc[w] = t if acc[w] is None else acc[w] + t
            lg = [a * (DH ** -0.5) for a in acc]
            if n == 0:
                lg = [lg[0]] + [jnp.where(lane >= DIL * w, lg[w], -1e9) for w in range(1, W)]
            m = functools.reduce(jnp.maximum, lg)
            e = [jnp.exp(l - m) for l in lg]
            inv = 1.0 / functools.reduce(lambda a, b: a + b, e)
            a = [x * inv for x in e]
            for p in range(DH // 2):
                rows = lambda part: pl.ds(part * (D // 2) + hg * 8 * (DH // 2) + p, 8, stride=DH // 2)
                vs = shifted(qkv_s[n + 1, rows(2), :], qkv_s[n, rows(2), :])
                olo = ohi = None
                for w in range(W):
                    vlo, vhi = _unpack(vs[w])
                    olo = a[w] * vlo if olo is None else olo + a[w] * vlo
                    ohi = a[w] * vhi if ohi is None else ohi + a[w] * vhi
                o_s[n, rows(0), :] = pltpu.pack_elementwise([olo, ohi], packed_dtype=bf16).astype(u32)

        def stage_attn(i):
            for t in range(tpa):
                for hg in range(H // 8):
                    attn_unit(i * tpa + t, hg)

        def stage_proj(i):
            o = jnp.concatenate([pltpu.bitcast(o_s[i * tpa + t], bf16) for t in range(tpa)], axis=1)
            a = jnp.dot(woT_s[...], o, preferred_element_type=f32)
            for t in range(tpa):
                n = i * tpa + t
                x = x_s[:, n * LANES:(n + 1) * LANES].astype(f32)
                x1 = x + mod(2) * a[:, t * LANES:(t + 1) * LANES]
                x1_s[n] = x1
                h2 = _ln_mod(x1, 1.0 + mod(4), mod(3)).astype(bf16)
                h2_s[n * LANES:(n + 1) * LANES, :] = h2.T

        stage_qkv(0)
        cp_m1.wait()
        mod_part(2 * D, 4 * D)
        cp_wo.wait()
        woT_s[...] = wo_s[...].T
        for i in range(na):
            if i + 1 < na:
                stage_qkv(i + 1)
            stage_attn(i)
            if order == "pipe":
                if i >= 1:
                    stage_proj(i - 1)
            else:
                stage_proj(i)
        if order == "pipe":
            stage_proj(na - 1)

        cp_wg.wait(); cp_wu.wait(); cp_wd.wait()
        tpf = TF // LANES

        def out_copy(i, slot):
            return pltpu.make_async_copy(out_s.at[slot], out_hbm.at[:, pl.ds(pl.multiple_of(i * TF, TF), TF)], osems.at[slot])

        def ffn(i, carry):
            slot = i % 2
            h = h2_s[pl.ds(pl.multiple_of(i * TF, TF), TF), :]
            g = jnp.dot(h, wg_s[...], preferred_element_type=f32)
            u = jnp.dot(h, wu_s[...], preferred_element_type=f32)
            hh = (g * u).astype(bf16)
            y = lax.dot_general(wdT_s[...], hh, NT_DIMS, preferred_element_type=f32)

            @pl.when(i >= 2)
            def _():
                out_copy(i - 2, slot).wait()

            for t in range(tpf):
                res = x1_s[i * tpf + t] + mod(5) * y[:, t * LANES:(t + 1) * LANES]
                out_s[slot, :, t * LANES:(t + 1) * LANES] = res.astype(bf16)
            out_copy(i, slot).start()
            return carry

        lax.fori_loop(0, nf, ffn, 0)
        for i in range(max(nf - 2, 0), nf):
            out_copy(i, i % 2).wait()

    def fn(A_x, A_wqkv, A_wo, B_x, B_w_gate, B_w_up, B_w_down, c, w_mod):
        del B_x
        xT = jnp.swapaxes(A_x[0], 0, 1)
        wdT = jnp.swapaxes(B_w_down, 0, 1)
        any_spec = pl.BlockSpec(memory_space=pl.ANY)
        outT = pl.pallas_call(
            kern,
            out_shape=jax.ShapeDtypeStruct((D, S), bf16),
            in_specs=[any_spec] * 8,
            out_specs=any_spec,
            scratch_shapes=[
                pltpu.VMEM((D, S), bf16), pltpu.VMEM((D, 3 * D), bf16), pltpu.VMEM((D, D), bf16),
                pltpu.VMEM((D, F), bf16), pltpu.VMEM((D, F), bf16), pltpu.VMEM((D, F), bf16),
                pltpu.VMEM((1, D), bf16), pltpu.VMEM((D, 6 * D), bf16),
                pltpu.VMEM((3 * D, D), bf16), pltpu.VMEM((D, D), bf16), pltpu.VMEM((6 * D, LANES), f32),
                pltpu.VMEM((NTILE + 1, 3 * D // 2, LANES), u32), pltpu.VMEM((NTILE, D // 2, LANES), u32),
                pltpu.VMEM((NTILE, D, LANES), f32), pltpu.VMEM((S, D), bf16), pltpu.VMEM((2, D, TF), bf16),
                pltpu.SemaphoreType.DMA((8 + na,)), pltpu.SemaphoreType.DMA((2,)),
            ],
            compiler_params=pltpu.CompilerParams(vmem_limit_bytes=120 * 2**20),
        )(xT, A_wqkv, A_wo, B_w_gate, B_w_up, wdT, c, w_mod)
        return jnp.swapaxes(outT, 0, 1)[None]

    return fn


@jax.jit
def pallas_adaLN_cond__sliding_local_dilated__glu_gated_bilinear__prompt_kernel(
    A_x: jax.Array,
    A_wqkv: jax.Array,
    A_wo: jax.Array,
    B_x: jax.Array,
    B_w_gate: jax.Array,
    B_w_up: jax.Array,
    B_w_down: jax.Array,
    c: jax.Array,
    w_mod: jax.Array,
):
    return make_kernel()(A_x, A_wqkv, A_wo, B_x, B_w_gate, B_w_up, B_w_down, c, w_mod)
```

```python
import functools
import jax
import jax.numpy as jnp
from jax import lax
from jax.experimental import pallas as pl
from jax.experimental.pallas import tpu as pltpu

S, D, F = 2048, 576, 4608
H, DH, W, DIL = 32, 18, 8, 2
EPS = 1e-5
NT_DIMS = (((1,), (1,)), ((), ()))
LANES = 128
NTILE = S // LANES
f32, bf16, u32 = jnp.float32, jnp.bfloat16, jnp.uint32

T = 512
TH = T // 2
TPB = T // LANES
NB = S // T
KH = 256
NC = 256
NCH = F // (2 * NC)
FT = F // 2 // LANES
RH = D // 2
KT = pl.cdiv(D, LANES)
ST = 16
QP = 192
NQP = 3 * D // QP
M1 = 23 * LANES


def _unpack(w):
    lo = pltpu.unpack_elementwise(w, index=0, packed_dtype=bf16, unpacked_dtype=f32)
    hi = pltpu.unpack_elementwise(w, index=1, packed_dtype=bf16, unpacked_dtype=f32)
    return lo, hi


def _dot(a, b):
    return jnp.dot(a, b, preferred_element_type=f32)


def _dot_nt(a, b):
    return lax.dot_general(a, b, NT_DIMS, preferred_element_type=f32)


def _add(a, b):
    return b if a is None else a + b


def _rows(r, n=ST):
    return slice(r * n, (r + 1) * n)


def _tile(n):
    return slice(n * LANES, (n + 1) * LANES)


def _operand(tiles):
    return jnp.concatenate([pltpu.bitcast(w, bf16) for w in tiles], axis=1)


def make_kernel(GA=3, wd_wait_chunk=3, mode=None, nside=6, B0=4, B2=7, P0=5, proj0=3, qbud=400, fbud=450, dbud=450,
                slots=(2, 3, 5, 6, 10, 11, 13, 14), slots0=(2, 3, 4, 5, 6, 7, 10, 11, 12, 13, 14, 15), dskip=2, stop=None):
    def kern(xT_hbm, wqkv_hbm, wo_hbm, wg_hbm, wu_hbm, wdT_hbm, c_hbm, wmod_hbm, out_hbm,
             x_s, wqkv_s, wo_s, wg_s, wu_s, wdT_s, c_s, wmod_s,
             wqkvT_s, woT_s, mod_s, sc_s, h_s, qkv_s, o_s, x1_s, ha_s, hl_s, tg_s, tu_s, sd_s, hb_s, out_s,
             z_s, sems):
        sem_id = iter(range(64))

        def copy(src, dst):
            return pltpu.make_async_copy(src, dst, sems.at[next(sem_id)])

        def cols(src, dst, c0, n):
            return copy(src.at[:, pl.ds(c0, n)], dst.at[:, pl.ds(c0, n)])

        cp_c = copy(c_hbm, c_s)
        cp_m0 = cols(wmod_hbm, wmod_s, 0, 2 * D)
        cp_m1 = cols(wmod_hbm, wmod_s, 2 * D, M1 - 2 * D)
        cp_m2 = cols(wmod_hbm, wmod_s, M1, 6 * D - M1)
        cp_wqkv = copy(wqkv_hbm, wqkv_s)
        cp_wo = copy(wo_hbm, wo_s)
        cp_x0 = cols(xT_hbm, x_s, 0, T)
        cp_x1 = cols(xT_hbm, x_s, T, S - T)
        cp_wg = copy(wg_hbm, wg_s)
        cp_wu = copy(wu_hbm, wu_s)
        cp_wd = copy(wdT_hbm, wdT_s)

        queue = []
        pending = []

        def mark(v):
            if v.dtype != u32:
                v = pltpu.bitcast(v, u32)
            for r in range(v.shape[0] // 8):
                for t in range(v.shape[1] // LANES):
                    q = v[_rows(r, 8), _tile(t)]
                    pending[:] = [q | pending[0]] if pending else [q]

        def run(budget):
            spent = 0
            while queue and spent + queue[0][0] // 2 <= budget:
                cost, step = queue.pop(0)
                step()
                spent += cost

        def zero_after(v):
            return z_s[pl.ds(1, 8), :] & v

        def anchor(tiles, r0=0):
            if not pending:
                return tiles
            z = zero_after(pending.pop())
            return [jnp.concatenate([p for p in (w[:r0], w[r0:r0 + 8] | z[:, :w.shape[1]], w[r0 + 8:]) if p.shape[0]], axis=0)
                    for w in tiles]

        def after(x, v):
            return pltpu.bitcast(pltpu.bitcast(x, u32) | zero_after(pltpu.bitcast(v[0:8, 0:LANES], u32)), f32)

        def words(ref, *idx, rows=slice(None), lanes=slice(None)):
            if rows.start is not None:
                rows = slice(rows.start // 2, rows.stop // 2)
            return ref.bitcast(u32)[(*idx, rows, lanes)]

        def k_tiles(ref, rows=slice(None)):
            return [words(ref, k, rows=rows, lanes=slice(0, min(LANES, D - k * LANES))) for k in range(KT)]

        def transpose_into(dst, src, k):
            n = min(LANES, D - k * LANES)
            t = src[k * LANES:k * LANES + n, :].T
            dst[k, :, 0:n] = t
            return t

        def mod_tiles(js, marked=True):
            acc = [None] * len(js)
            for r in range(D // ST):
                sc = sc_s[_rows(r), :]
                for k, j in enumerate(js):
                    acc[k] = _add(acc[k], sc * wmod_s[_rows(r), _tile(j)].astype(f32))
            for k, j in enumerate(js):
                col = j * LANES + lax.broadcasted_iota(jnp.int32, (1, LANES), 1)
                is_scale = ((col >= D) & (col < 2 * D)) | ((col >= 4 * D) & (col < 5 * D))
                r = jnp.sum(acc[k], axis=0, keepdims=True) + jnp.where(is_scale, 1.0, 0.0)
                t = jnp.broadcast_to(r, (LANES, LANES)).T
                mod_s[_tile(j), :] = t
                if marked:
                    mark(t[LANES - 8:])

        def mod(i, rs):
            return mod_s[i * D + rs.start:i * D + rs.stop, :]

        def col_mean(strips):
            total = jnp.sum(functools.reduce(_add, strips), axis=0, keepdims=True) * (1.0 / D)
            return jnp.broadcast_to(total, (8, LANES))

        def twice(v):
            return jnp.concatenate([v, v], axis=0)

        def inv_std(get, m):
            return lax.rsqrt(col_mean(jnp.square(get(r) - twice(m)) for r in range(D // ST)) + EPS)

        def ln1_steps(n):
            st = {}

            def get(r):
                return x_s[_rows(r), _tile(n)].astype(f32)

            def mean():
                st["m"] = col_mean(get(r) for r in range(D // ST))
                mark(st["m"])

            def scale():
                st["rstd"] = inv_std(get, st["m"])
                mark(st["rstd"])

            def apply(rs):
                for r in rs:
                    hh = (get(r) - twice(st["m"])) * twice(st["rstd"]) * mod(1, _rows(r)) + mod(0, _rows(r))
                    h_s[n, _rows(r), :] = hh.astype(bf16)
                    mark(hh[8:])

            half = D // ST // 2
            return [(150, mean), (250, scale), (200, functools.partial(apply, range(half))),
                    (200, functools.partial(apply, range(half, 2 * half)))]

        def qkv_piece(i, j, budget):
            rhs = []
            for t in range(TPB):
                run(budget)
                rhs += anchor([words(h_s, i * TPB + t)], LANES // 2 - 8)
            y = _dot(_operand(k_tiles(wqkvT_s, _rows(j, QP))), _operand(rhs))
            for r in range(QP // ST):
                for t in range(TPB):
                    qkv_s[1 + i * TPB + t, _rows(j * (QP // ST) + r), :] = y[_rows(r), _tile(t)].astype(bf16)
            return y

        def halo():
            for r in range(D // ST, 3 * D // ST):
                qkv_s[0, _rows(r), :] = jnp.broadcast_to(qkv_s[1, _rows(r), 0:1].astype(f32), (ST, LANES)).astype(bf16)

        lane = lax.broadcasted_iota(jnp.int32, (8, LANES), 1)

        def shifted(cur, prev, w):
            s = DIL * w
            return cur if w == 0 else pltpu.roll(jnp.where(lane >= LANES - s, prev, cur), s, 1)

        def attn_steps(n, hg):
            qkv = qkv_s.bitcast(u32)
            acc = [None] * W

            def rows(part, p):
                return pl.ds(part * RH + hg * 8 * (DH // 2) + p, 8, stride=DH // 2)

            def scores(ps, last):
                for p in ps:
                    qlo, qhi = _unpack(qkv[n + 1, rows(0, p), :])
                    cur, prev = qkv[n + 1, rows(1, p), :], qkv[n, rows(1, p), :]
                    for w in range(W):
                        klo, khi = _unpack(shifted(cur, prev, w))
                        acc[w] = _add(acc[w], qlo * klo + qhi * khi)
                if last:
                    lg = [a * (DH ** -0.5) for a in acc]
                    if n == 0:
                        lg = [lg[0]] + [jnp.where(lane >= DIL * w, lg[w], -1e9) for w in range(1, W)]
                    m = functools.reduce(jnp.maximum, lg)
                    e = [jnp.exp(l - m) for l in lg]
                    inv = 1.0 / functools.reduce(_add, e)
                    acc[:] = [x * inv for x in e]
                for a in acc:
                    mark(a)

            def values(ps):
                for p in ps:
                    cur, prev = qkv[n + 1, rows(2, p), :], qkv[n, rows(2, p), :]
                    olo = ohi = None
                    for w in range(W):
                        vlo, vhi = _unpack(shifted(cur, prev, w))
                        olo, ohi = _add(olo, acc[w] * vlo), _add(ohi, acc[w] * vhi)
                    o = pltpu.pack_elementwise([olo, ohi], packed_dtype=bf16).astype(u32)
                    o_s[n, rows(0, p), :] = o
                    mark(o)

            return [(400, functools.partial(scores, range(0, 5), False)),
                    (400, functools.partial(scores, range(5, 9), True)),
                    (400, functools.partial(values, range(0, 5))),
                    (400, functools.partial(values, range(5, 9)))]

        def attn_block(i):
            return [s for t in range(TPB) for hg in range(H // 8) for s in attn_steps(i * TPB + t, hg)]

        def project(i):
            a = _dot(_operand(anchor(k_tiles(woT_s))), _operand([o_s[i * TPB + t] for t in range(TPB)]))
            st = {}

            for t in range(TPB):
                strips = []
                for r in range(D // ST):
                    x1 = x_s[_rows(r), _tile(i * TPB + t)].astype(f32) + mod(2, _rows(r)) * a[_rows(r), _tile(t)]
                    x1_s[i * TPB + t, _rows(r), :] = x1
                    strips.append(x1)
                st["m", t] = col_mean(strips)

            def parity_rows(r, e, base=0):
                return pl.ds(base + r * ST + e, 8, stride=2)

            def x1_strip(t, r):
                return jnp.concatenate([x1_s[i * TPB + t, parity_rows(r, e), :] for e in range(2)], axis=0)

            def scale(ts, go):
                for t in ts:
                    st["rstd", t] = inv_std(functools.partial(x1_strip, t), after(st["m", t], go))

            def h2(t, r, m):
                cb, sb = [jnp.concatenate([mod_s[parity_rows(r, e, k * D), :] for e in range(2)], axis=0) for k in (4, 3)]
                return (x1_strip(t, r) - twice(m)) * twice(st["rstd", t]) * cb + sb

            def transposed(strips):
                w = [pltpu.pack_elementwise([v[0:8], v[8:ST]], packed_dtype=bf16).astype(u32) for v in strips]
                return pltpu.bitcast(jnp.concatenate(w, axis=0), bf16).T

            def blocks(t, kt, go):
                t2 = t + TPB // 2
                m1, m2 = after(st["m", t], go), after(st["m", t2], go)
                strips = [[] for _ in range(7)]
                for r in range(kt * LANES // ST, (kt + 1) * LANES // ST):
                    a11, a12 = h2(t, r, m1), h2(t, r + KH // ST, m1)
                    a21, a22 = h2(t2, r, m2), h2(t2, r + KH // ST, m2)
                    for j, cmb in enumerate((a11 + a22, a21 + a22, a11, a22, a11 + a12, a21 - a11, a12 - a22)):
                        strips[j].append(cmb)
                for j in range(7):
                    ha_s[i, j, kt, _tile(t), :] = transposed(strips[j])

            def tail(go):
                for t in range(TPB):
                    m = after(st["m", t], go)
                    hl_s[i, _tile(t), 0:D - 2 * KH] = transposed([h2(t, r, m) for r in range(2 * KH // ST, D // ST)])

            half = TPB // 2
            return ([functools.partial(scale, (t, t + half)) for t in range(half)]
                    + [functools.partial(blocks, t, kt) for t in range(half) for kt in range(KH // LANES)] + [tail])

        def prep_gu(w_s, t_s, c, t):
            n1, n2 = _tile(2 * c * (NC // LANES) + t), _tile((2 * c + 1) * (NC // LANES) + t)
            for r in range(KH // ST):
                lo, hi = _rows(r), _rows(r + KH // ST)
                b11, b12 = w_s[lo, n1].astype(f32), w_s[lo, n2].astype(f32)
                b21, b22 = w_s[hi, n1].astype(f32), w_s[hi, n2].astype(f32)
                for j, cmb in enumerate((b11 + b22, b12 - b22, b21 - b11, b11 + b12, b21 + b22)):
                    t_s[j, c * (NC // LANES) + t, lo, :] = cmb.astype(bf16)
                    mark(cmb[8:])

        def prep_gu_steps(c, half):
            return [(450, functools.partial(prep_gu, *((wg_s, tg_s), (wu_s, tu_s))[half], c, t)) for t in range(NC // LANES)]

        def prep_d(c, t):
            n1, n2 = _tile(2 * c * (NC // LANES) + t), _tile((2 * c + 1) * (NC // LANES) + t)
            for r in range(RH // ST):
                lo, hi = _rows(r), _rows(r + RH // ST)
                a11, a12 = wdT_s[lo, n1].astype(f32), wdT_s[lo, n2].astype(f32)
                a21, a22 = wdT_s[hi, n1].astype(f32), wdT_s[hi, n2].astype(f32)
                for j, cmb in enumerate((a11 + a22, a21 + a22, a11, a22, a11 + a12, a21 - a11, a12 - a22)):
                    sd_s[j, c * (NC // LANES) + t, lo, :] = cmb.astype(bf16)
                    if j not in (2, 3):
                        mark(cmb[8:])

        def gate_up_dots(w_s, t_s, i, c, before):
            n1, n2 = _rows(2 * c, NC), _rows(2 * c + 1, NC)
            t = [_operand([words(t_s, j, c * (NC // LANES) + k) for k in range(NC // LANES)]) for j in range(5)]
            rhs = (t[0], w_s[0:KH, n1], t[1], t[2], w_s[KH:2 * KH, n2], t[3], t[4])
            m = []
            for j in range(7):
                before(j)
                m.append(_dot(_operand(anchor([words(ha_s, i, j, k) for k in range(KH // LANES)])), rhs[j]))
            before(7)
            l = _dot(_operand(anchor([words(hl_s, i, lanes=slice(0, D - 2 * KH))])), w_s[2 * KH:D, n1.start:n2.stop])
            return m, l

        def combine(i, c, g, u):
            def strip(r, t):
                lo, hi = _rows(r), _rows(r + TH // ST)
                n1, n2 = _tile(t), _tile(t + NC // LANES)

                def blocks(m, l):
                    m1, m2, m3, m4, m5, m6, m7 = [x[lo, n1] for x in m]
                    return (m1 + m4 - m5 + m7 + l[lo, n1], m3 + m5 + l[lo, n2],
                            m2 + m4 + l[hi, n1], m1 - m2 + m3 + m6 + l[hi, n2])

                h11, h12, h21, h22 = [a * b for a, b in zip(blocks(*g), blocks(*u))]
                b11, b12, b21, b22 = h11, h21, h12, h22
                for j, cmb in enumerate((b11 + b22, b11, b12 - b22, b21 - b11, b22, b11 + b12, b21 + b22)):
                    hb_s[i % 2, j, c * (NC // LANES) + t, lo, :] = cmb.astype(bf16)

            for r in range(TH // ST):
                for t in range(NC // LANES):
                    strip(r, t)

        def ffn_block(i, chunks, pre=None, slots=slots):
            def before(half, j):
                if 8 * half + j in slots:
                    run(fbud)

            for c in chunks:
                if pre is not None:
                    pre(c, 0)
                g = gate_up_dots(wg_s, tg_s, i, c, functools.partial(before, 0))
                if pre is not None:
                    pre(c, 1)
                u = gate_up_dots(wu_s, tu_s, i, c, functools.partial(before, 1))
                combine(i, c, g, u)

        out_copies = []

        def flush(rows, c0, n):
            idx = (rows, pl.ds(c0, n))
            cp = copy(out_s.at[idx], out_hbm.at[idx])
            cp.start()
            out_copies.append(cp)

        def down(i, proj_at):
            m = {}
            steps = []

            def prod(j):
                tiles = []
                for k in range(0, FT, 4):
                    grp = [words(sd_s, j - 1, kk) for kk in range(k, min(k + 4, FT))]
                    if len(grp) == 4 and (m or k >= 4 * dskip):
                        run(dbud)
                        grp = anchor(grp)
                    tiles += grp
                if len(m) == proj_at:
                    run(10 ** 9)
                    steps.extend(project(i + 1))
                m[j] = _dot_nt(_operand(tiles), _operand([words(hb_s, i % 2, j - 1, k) for k in range(FT)]))
                left = 7 - len(m)
                for t in range(pl.cdiv(len(steps), max(left, 1))):
                    steps.pop(0)(m[j][:, _tile(t % (TH // LANES))])

            def out(a, b, comb):
                n0 = i * TPB + b * (TPB // 2)
                for r in range(RH // ST):
                    rs = _rows(a * RH // ST + r)
                    x1 = jnp.concatenate([x1_s[n0 + k, rs, :] for k in range(TPB // 2)], axis=1)
                    gb = jnp.concatenate([mod(5, rs)] * (TPB // 2), axis=1)
                    res = x1 + gb * comb(_rows(r))
                    out_s[rs, n0 * LANES:n0 * LANES + TH] = res.astype(bf16)

            prod(2); prod(4)
            out(1, 0, lambda s: m[2][s] + m[4][s])
            prod(1); prod(5); prod(7)
            out(0, 0, lambda s: m[1][s] + m[4][s] - m[5][s] + m[7][s])
            if i == NB - 1:
                flush(slice(None), 0, i * T + TH)
            prod(3)
            out(0, 1, lambda s: m[3][s] + m[5][s])
            prod(6)
            out(1, 1, lambda s: m[1][s] - m[2][s] + m[3][s] + m[6][s])
            if i == NB - 1:
                flush(slice(None), i * T + TH, TH)

        z_s[...] = jnp.zeros_like(z_s)
        if mode is not None:
            cp_c.start(); cp_c.wait()
            if mode == "ffn":
                queue.extend(attn_block(2)[:4 * nside])
                ffn_block(1, range(3))
            elif mode == "blk":
                queue.extend(attn_block(2))
                ffn_block(1, range(NCH))
                down(1, 0)
            elif mode in ("q1", "q2", "q3"):
                i = int(mode[1])
                ln = lambda i: [step for t in range(TPB) for step in ln1_steps(i * TPB + t)]
                md = [(250, functools.partial(mod_tiles, range(j, j + 1))) for j in range(2 * D // LANES, M1 // LANES)]
                wo_t = [(300, functools.partial(lambda k: mark(transpose_into(woT_s, wo_s, k)[D - ST:]), k)) for k in range(KT)]
                a0 = attn_block(0)
                queue.extend({1: a0[:24] + ln(2), 2: a0[24:44] + ln(3) + md[:7], 3: md[7:] + wo_t[::-1] + a0[44:]}[i])
                steps = []
                for j in range(NQP):
                    if (i, j) == (3, P0):
                        run(10 ** 9)
                        steps = project(0)
                    y = qkv_piece(i, j, qbud)
                    for t in range(min(len(steps), pl.cdiv(len(steps), max(NQP - 1 - j, 1)))):
                        steps.pop(0)(y[:, _tile(t % TPB)])
                for src in (qkv_s.at[16, pl.ds(0, 256)], h_s.at[15, pl.ds(0, 256)]):
                    cp = copy(src, ha_s.at[0, 0, 0])
                    cp.start(); cp.wait()
                cp = copy(mod_s.at[pl.ds(0, D)], x1_s.at[1])
                cp.start(); cp.wait()
            elif mode == "down":
                down(1, nside)
            run(10 ** 9)
            for src in (hb_s.at[1, 0, 0], ha_s.at[2, 0, 0], hl_s.at[2, pl.ds(0, 256)]):
                cp = copy(src, ha_s.at[0, 0, 0])
                cp.start(); cp.wait()
            cp = copy(o_s.at[0, pl.ds(0, 16), :], z_s)
            cp.start(); cp.wait()
            flush(slice(None), 0, S)
            out_copies[0].wait()
            return

        cp_c.start(); cp_m0.start(); cp_x0.start(); cp_wqkv.start()
        cp_c.wait()
        cv = c_s[...].astype(f32)
        sc = (cv * jax.nn.sigmoid(cv)).astype(bf16).astype(f32)
        sc_s[...] = jnp.broadcast_to(sc, (LANES, D)).T
        cp_m0.wait()
        for j in range(0, 2 * D // LANES, 3):
            mod_tiles(range(j, j + 3), False)
        cp_x0.wait()
        cp_wqkv.wait()
        cp_x1.start(); cp_m1.start(); cp_wo.start()
        for k in range(KT):
            transpose_into(wqkvT_s, wqkv_s, k)

        def ln(i):
            return [step for t in range(TPB) for step in ln1_steps(i * TPB + t)]

        def wo_tile(k):
            mark(transpose_into(woT_s, wo_s, k)[D - ST:])

        queue.extend(ln(0))
        run(10 ** 9)
        pending.clear()
        md = [(250, functools.partial(mod_tiles, range(j, j + 1))) for j in range(2 * D // LANES, M1 // LANES)]
        wo_t = [(300, functools.partial(wo_tile, k)) for k in range(KT)]
        a0 = attn_block(0)
        todo = {(0, B0): ln(1), (1, 0): a0[:24] + ln(2), (2, 0): a0[24:44] + ln(3) + md[:7],
                (3, 0): md[7:] + wo_t[::-1] + a0[44:], (3, B2): prep_gu_steps(0, 0) + prep_gu_steps(0, 1)}
        steps = []
        for i in range(NB):
            for j in range(NQP):
                if (i, j) == (0, B0):
                    cp_x1.wait()
                if (i, j) == (1, 0):
                    run(10 ** 9)
                    cp_m1.wait(); cp_wo.wait()
                    cp_wg.start(); cp_wu.start()
                if (i, j) == (3, P0):
                    run(10 ** 9)
                    steps = project(0)
                if (i, j) == (3, B2):
                    cp_wg.wait(); cp_wu.wait()
                    cp_wd.start(); cp_m2.start()
                if j == 0:
                    run(10 ** 9)
                first = (i, j) in todo
                queue.extend(todo.get((i, j), ()))
                y = qkv_piece(i, j, 0 if first and j == 0 and i > 1 else qbud)
                if (i, j) == (0, NQP - 1):
                    halo()
                for t in range(min(len(steps), pl.cdiv(len(steps), max(NQP - 1 - j, 1)))):
                    steps.pop(0)(y[:, _tile(t % TPB)])
        run(10 ** 9)

        def finish():
            for src in (hb_s.at[1, 0, 0], hb_s.at[0, 0, 0], ha_s.at[2, 0, 0], hl_s.at[2, pl.ds(0, 256)], tg_s.at[0, 0], tu_s.at[0, 0], qkv_s.at[16, pl.ds(0, 256)]):
                cp = copy(src, ha_s.at[0, 0, 0])
                cp.start(); cp.wait()
            cp = copy(x1_s.at[0], x1_s.at[1])
            cp.start(); cp.wait()
            cp = copy(out_s.at[:, pl.ds(0, 128)], out_hbm.at[:, pl.ds(0, 128)])
            cp.start(); cp.wait()

        for i in range(NB):
            if i == stop:
                if i == 0:
                    cp_wd.wait(); cp_m2.wait()
                finish()
                return
            if i + 1 < NB:
                queue.extend(attn_block(i + 1))
            pre = None
            if i == 0:
                def pre(c, half):
                    if (c, half) == (wd_wait_chunk, 0):
                        cp_wd.wait(); cp_m2.wait()
                        extra = [(250, functools.partial(mod_tiles, range(j, j + 1))) for j in range(M1 // LANES, 6 * D // LANES)]
                        extra += [(500, functools.partial(prep_d, cc, t)) for cc in range(NCH) for t in range(NC // LANES)]
                        merged = []
                        while queue or extra:
                            merged += [q.pop(0) for q in (extra, queue) if q]
                        queue.extend(merged)
                    if c + 1 < NCH:
                        queue[:0] = prep_gu_steps(c + 1, half)

            ffn_block(i, range(NCH), pre, slots0 if i == 0 else slots)
            down(i, -1 if i + 1 == NB else proj0 if i == 0 else 0)
        for cp in out_copies:
            cp.wait()

    def fn(A_x, A_wqkv, A_wo, B_x, B_w_gate, B_w_up, B_w_down, c, w_mod):
        del B_x
        xT = jnp.swapaxes(A_x[0], 0, 1)
        wdT = jnp.swapaxes(B_w_down, 0, 1)
        any_spec = pl.BlockSpec(memory_space=pl.ANY)
        outT = pl.pallas_call(
            kern,
            out_shape=jax.ShapeDtypeStruct((D, S), bf16),
            in_specs=[any_spec] * 8,
            out_specs=any_spec,
            scratch_shapes=[
                pltpu.VMEM((D, S), bf16), pltpu.VMEM((D, 3 * D), bf16), pltpu.VMEM((D, D), bf16),
                pltpu.VMEM((D, F), bf16), pltpu.VMEM((D, F), bf16), pltpu.VMEM((D, F), bf16),
                pltpu.VMEM((1, D), bf16), pltpu.VMEM((D, 6 * D), bf16),
                pltpu.VMEM((KT, 3 * D, LANES), bf16), pltpu.VMEM((KT, D, LANES), bf16),
                pltpu.VMEM((6 * D, LANES), f32), pltpu.VMEM((D, LANES), f32),
                pltpu.VMEM((NTILE, D, LANES), bf16),
                pltpu.VMEM((NTILE + 1, 3 * D, LANES), bf16), pltpu.VMEM((NTILE, RH, LANES), u32),
                pltpu.VMEM((NTILE, D, LANES), f32),
                pltpu.VMEM((NB, 7, KH // LANES, TH, LANES), bf16), pltpu.VMEM((NB, T, LANES), bf16),
                pltpu.VMEM((5, FT, KH, LANES), bf16), pltpu.VMEM((5, FT, KH, LANES), bf16),
                pltpu.VMEM((7, FT, RH, LANES), bf16), pltpu.VMEM((2, 7, FT, TH, LANES), bf16),
                pltpu.VMEM((D, S), bf16),
                pltpu.VMEM((16, LANES), u32),
                pltpu.SemaphoreType.DMA((32,)),
            ],
            compiler_params=pltpu.CompilerParams(vmem_limit_bytes=120 * 2**20),
        )(xT, A_wqkv, A_wo, B_w_gate, B_w_up, wdT, c, w_mod)
        return jnp.swapaxes(outT, 0, 1)[None]

    return fn


@jax.jit
def pallas_adaLN_cond__sliding_local_dilated__glu_gated_bilinear__prompt_kernel(
    A_x: jax.Array,
    A_wqkv: jax.Array,
    A_wo: jax.Array,
    B_x: jax.Array,
    B_w_gate: jax.Array,
    B_w_up: jax.Array,
    B_w_down: jax.Array,
    c: jax.Array,
    w_mod: jax.Array,
):
    return make_kernel()(A_x, A_wqkv, A_wo, B_x, B_w_gate, B_w_up, B_w_down, c, w_mod)
```

```python
import functools
import jax
import jax.numpy as jnp
from jax import lax
from jax.experimental import pallas as pl
from jax.experimental.pallas import tpu as pltpu

S, D, F = 2048, 576, 4608
H, DH, W, DIL = 32, 18, 8, 2
EPS = 1e-5
NT_DIMS = (((1,), (1,)), ((), ()))
LANES = 128
NTILE = S // LANES
f32, bf16, u32 = jnp.float32, jnp.bfloat16, jnp.uint32

T = 512
TH = T // 2
TPB = T // LANES
NB = S // T
KH = 256
NC = 256
NCH = F // (2 * NC)
FT = F // 2 // LANES
RH = D // 2
KT = pl.cdiv(D, LANES)
ST = 16
QP = 192
NQP = 3 * D // QP
GC = 3
NT = NC // LANES


def _unpack(w):
    lo = pltpu.unpack_elementwise(w, index=0, packed_dtype=bf16, unpacked_dtype=f32)
    hi = pltpu.unpack_elementwise(w, index=1, packed_dtype=bf16, unpacked_dtype=f32)
    return lo, hi


def _dot(a, b):
    return jnp.dot(a, b, preferred_element_type=f32)


def _dot_nt(a, b):
    return lax.dot_general(a, b, NT_DIMS, preferred_element_type=f32)


def _add(a, b):
    return b if a is None else a + b


def _rows(r, n=ST):
    return slice(r * n, (r + 1) * n)


def _tile(n, width=1):
    if isinstance(n, int):
        return slice(n * LANES, (n + width) * LANES)
    return pl.ds(pl.multiple_of(n * LANES, LANES), width * LANES)


def _weave(a, b):
    keyed = [((k + 0.5) / len(x), x[k]) for x in (a, b) for k in range(len(x))]
    return [item for _, item in sorted(keyed, key=lambda p: p[0])]


def _operand(tiles):
    return jnp.concatenate([pltpu.bitcast(w, bf16) for w in tiles], axis=1)


def make_kernel(stop=None, WCUT=(0, 384, 768, 1728), WAT=(1, 3), prio=(0, 1), B0=5, P0=6, SK=2, lnp=3, pp=2,
                slots=(4, 6, 10, 12, 20, 22, 26, 28), slots0=((4, 5, 6, 7, 8, 9, 10, 11, 12, 13), (2, 3, 4, 6, 7, 8, 9, 10, 12, 13))):
    def kern(xT_hbm, wqkv_hbm, wo_hbm, wg_hbm, wu_hbm, wdT_hbm, c_hbm, wmod_hbm, out_hbm,
             x_s, wqkv_s, wo_s, wg_s, wu_s, wdT_s, c_s, wmod_s,
             wqkvT_s, woT_s, mod_s, sc_s, h_s, hn_s, qkv0_s, qkv_s, o_s, x1_s, ha_s, hl_s, tg_s, tu_s, sd_s, hb_s, out_s, ms_s,
             z_s, sems, out_sems):
        sem_id = iter(range(64))

        def copy(src, dst):
            return pltpu.make_async_copy(src, dst, sems.at[next(sem_id)])

        def cols(src, dst, c0, n):
            return copy(src.at[:, pl.ds(c0, n)], dst.at[:, pl.ds(c0, n)])

        cp_c = copy(c_hbm, c_s)
        cp_m0 = cols(wmod_hbm, wmod_s, 0, 2 * D)
        cp_m1 = cols(wmod_hbm, wmod_s, 2 * D, 4 * D)
        cp_w = [cols(wqkv_hbm, wqkv_s, c0, c1 - c0) for c0, c1 in zip(WCUT[:-1], WCUT[1:])]
        cp_wo = copy(wo_hbm, wo_s)
        cp_x0 = cols(xT_hbm, x_s, 0, T)
        cp_x1 = cols(xT_hbm, x_s, T, T)
        cp_x2 = cols(xT_hbm, x_s, 2 * T, S - 2 * T)
        ffn = ((wg_hbm, wg_s, (GC + 1) * 2 * NC), (wu_hbm, wu_s, (GC + 1) * 2 * NC), (wdT_hbm, wdT_s, GC * 2 * NC))
        cp_a = [cols(src, dst, 0, n) for src, dst, n in ffn]
        cp_b = [cols(src, dst, n, F - n) for src, dst, n in ffn]

        def out_copy(k, tile0, ntiles):
            idx = (slice(None), _tile(tile0, ntiles))
            return pltpu.make_async_copy(out_s.at[idx], out_hbm.at[idx], out_sems.at[k])

        waited = set()

        def wait(*cps):
            for cp in cps:
                cp.wait()
                waited.add(id(cp))

        queue = []
        pending = []

        def mark(v):
            if v.dtype != f32:
                v = pltpu.bitcast(v, f32)
            for r in range(v.shape[0] // 8):
                q = v[_rows(r, 8)]
                pending[:] = [q + pending[0]] if pending else [q]

        def pace():
            pending[:] = [pltpu.roll(pending[0], 1, 1)]

        def run(n=None):
            for _ in range(len(queue) if n is None else min(n, len(queue))):
                queue.pop(0)()

        def zero_after(v):
            return z_s[pl.ds(1, 8), :] & pltpu.bitcast(v, u32)

        def anchor(tiles, r0=0):
            if not pending:
                return tiles
            z = zero_after(pending.pop())
            out = []
            for w in tiles:
                a = r0 % w.shape[0]
                parts = ([w[:a]] if a else []) + [w[a:a + 8] | z[:, :w.shape[1]]] + ([w[a + 8:]] if a + 8 < w.shape[0] else [])
                out.append(jnp.concatenate(parts, axis=0))
            return out

        def after(x, v):
            return pltpu.bitcast(pltpu.bitcast(x, u32) | zero_after(v[0:8, 0:LANES]), f32)

        def words(ref, *idx, rows=slice(None), lanes=slice(None)):
            if rows.start is not None:
                rows = slice(rows.start // 2, rows.stop // 2)
            return ref.bitcast(u32)[(*idx, rows, lanes)]

        def k_tiles(ref, rows=slice(None)):
            return [words(ref, k, rows=rows, lanes=slice(0, min(LANES, D - k * LANES))) for k in range(KT)]

        def transpose_into(dst, src, k, c0, c1):
            assert src is not wo_s or id(cp_wo) in waited
            n = min(LANES, D - k * LANES)
            t = src[k * LANES:k * LANES + n, c0:c1].T
            dst[k, c0:c1, 0:n] = t
            if n == LANES:
                mark(t[c1 - c0 - ST:])

        def mod_tiles(js):
            assert id(cp_m0 if js[0] < 2 * D // LANES else cp_m1) in waited
            acc = [None] * len(js)
            for r in range(D // ST):
                sc = sc_s[_rows(r), :]
                for k, j in enumerate(js):
                    v = sc * wmod_s[_rows(r), _tile(j)].astype(f32)
                    acc[k] = _add(_add(acc[k], v[0:8]), v[8:ST])
            for k, j in enumerate(js):
                col = j * LANES + lax.broadcasted_iota(jnp.int32, (1, LANES), 1)
                is_scale = ((col >= D) & (col < 2 * D)) | ((col >= 4 * D) & (col < 5 * D))
                r = jnp.sum(acc[k], axis=0, keepdims=True) + jnp.where(is_scale, 1.0, 0.0)
                t = jnp.broadcast_to(r, (LANES, LANES)).T
                mod_s[_tile(j), :] = t
                mark(t[LANES - 8:])

        def mod(i, rs):
            return mod_s[i * D + rs.start:i * D + rs.stop, :]

        def col_mean(strips):
            total = functools.reduce(_add, (v[_rows(e, 8)] for v in strips for e in range(2)))
            total = jnp.sum(total, axis=0, keepdims=True) * (1.0 / D)
            return jnp.broadcast_to(total, (8, LANES))

        def twice(v):
            return jnp.concatenate([v, v], axis=0)

        def inv_std(get, m):
            return lax.rsqrt(col_mean(jnp.square(get(r) - twice(m)) for r in range(D // ST)) + EPS)

        def ln1_steps(n, dst, slot):
            st = {}

            def get(r):
                return x_s[_rows(r), _tile(n)].astype(f32)

            def mean():
                st["m"] = col_mean(get(r) for r in range(D // ST))
                mark(st["m"])

            def scale():
                st["rstd"] = inv_std(get, st["m"])
                mark(st["rstd"])

            def apply(rs, paced=True):
                for r in rs:
                    hh = (get(r) - twice(st["m"])) * twice(st["rstd"]) * mod(1, _rows(r)) + mod(0, _rows(r))
                    dst[slot, _rows(r), :] = hh.astype(bf16)
                    mark(hh)
                    if paced and r % lnp == 0:
                        pace()

            half = D // ST // 2
            return [mean, scale, functools.partial(apply, range(half)), functools.partial(apply, range(half, 2 * half))]

        def qkv_piece(i, j, skip=0):
            tiles = [words(h_s, t, rows=slice(k * LANES, min((k + 1) * LANES, D))) for t in range(TPB) for k in range(KT)]
            for g in range(4 * skip, len(tiles), 4):
                run(1)
                tiles[g:g + 4] = anchor(tiles[g:g + 4], -8)
            rhs = [jnp.concatenate(tiles[t * KT:(t + 1) * KT], axis=0) for t in range(TPB)]
            y = _dot(_operand(k_tiles(wqkvT_s, _rows(j, QP))), _operand(rhs))
            for r in range(QP // ST):
                for t in range(TPB):
                    v, rs = y[_rows(r), _tile(t)].astype(bf16), _rows(j * (QP // ST) + r)
                    if isinstance(i, int) and i == 0:
                        qkv0_s[1 + t, rs, :] = v
                    if not (isinstance(i, int) and i == 0) or t == TPB - 1:
                        qkv_s[i * TPB + t - (TPB - 1), rs, :] = v
            return y

        def halo():
            for r in range(D // ST, 3 * D // ST):
                qkv0_s[0, _rows(r), :] = jnp.broadcast_to(qkv0_s[1, _rows(r), 0:1].astype(f32), (ST, LANES)).astype(bf16)

        lane = lax.broadcasted_iota(jnp.int32, (8, LANES), 1)

        def shifted(cur, prev, w):
            s = DIL * w
            return cur if w == 0 else pltpu.roll(jnp.where(lane >= LANES - s, prev, cur), s, 1)

        def attn_steps(n, hg, first):
            qkv, tile = (qkv0_s.bitcast(u32), n + 1) if first else (qkv_s.bitcast(u32), n - (TPB - 1))
            acc = [None] * W

            def heads(ref, tile, part):
                start = part * RH + hg * 8 * (DH // 2)
                return ref.at[tile, pl.ds(start if isinstance(start, int) else pl.multiple_of(start, 8), 8 * (DH // 2))]

            def pair(p):
                return pl.ds(p, 8, stride=DH // 2), slice(None)

            def scores(ps, last):
                for p in ps:
                    qlo, qhi = _unpack(heads(qkv, tile, 0)[pair(p)])
                    cur, prev = heads(qkv, tile, 1)[pair(p)], heads(qkv, tile - 1, 1)[pair(p)]
                    for w in range(W):
                        klo, khi = _unpack(shifted(cur, prev, w))
                        acc[w] = _add(acc[w], qlo * klo + qhi * khi)
                if last:
                    lg = [a * (DH ** -0.5) for a in acc]
                    if first:
                        lg = [lg[0]] + [jnp.where(n * LANES + lane >= DIL * w, lg[w], -1e9) for w in range(1, W)]
                    m = functools.reduce(jnp.maximum, lg)
                    e = [jnp.exp(l - m) for l in lg]
                    inv = 1.0 / functools.reduce(_add, e)
                    acc[:] = [x * inv for x in e]
                for a in acc:
                    mark(a)

            def values(ps):
                for p in ps:
                    cur, prev = heads(qkv, tile, 2)[pair(p)], heads(qkv, tile - 1, 2)[pair(p)]
                    olo = ohi = None
                    for w in range(W):
                        vlo, vhi = _unpack(shifted(cur, prev, w))
                        olo, ohi = _add(olo, acc[w] * vlo), _add(ohi, acc[w] * vhi)
                    o = pltpu.pack_elementwise([olo, ohi], packed_dtype=bf16).astype(u32)
                    heads(o_s, n, 0)[pair(p)] = o
                    mark(o)

            return [functools.partial(scores, range(0, 5), False), functools.partial(scores, range(5, 9), True),
                    functools.partial(values, range(0, 5)), functools.partial(values, range(5, 9))]

        def attn_units(units, first=False):
            return [s for n, hg in units for s in attn_steps(n, hg, first)]

        def project(i):
            a = _dot(_operand(anchor(k_tiles(woT_s))), _operand([o_s[i * TPB + t] for t in range(TPB)]))
            for t in range(TPB):
                strips = []
                for r in range(D // ST):
                    x1 = x_s[_rows(r), _tile(i * TPB + t)].astype(f32) + mod(2, _rows(r)) * a[_rows(r), _tile(t)]
                    x1_s[i * TPB + t, _rows(r), :] = x1
                    strips.append(x1)
                ms_s[t] = col_mean(strips)

        def ln2_steps(i):
            st = {}

            def parity_rows(r, e, base=0):
                return pl.ds(base + r * ST + e, 8, stride=2)

            def x1_strip(t, r):
                return jnp.concatenate([x1_s[i * TPB + t, parity_rows(r, e), :] for e in range(2)], axis=0)

            def scale(ts, go):
                for t in ts:
                    st["rstd", t] = inv_std(functools.partial(x1_strip, t), after(ms_s[t], go))

            def h2(t, r, m):
                cb, sb = [jnp.concatenate([mod_s[parity_rows(r, e, k * D), :] for e in range(2)], axis=0) for k in (4, 3)]
                return (x1_strip(t, r) - twice(m)) * twice(st["rstd", t]) * cb + sb

            def transposed(strips):
                w = [pltpu.pack_elementwise([v[0:8], v[8:ST]], packed_dtype=bf16).astype(u32) for v in strips]
                return pltpu.bitcast(jnp.concatenate(w, axis=0), bf16).T

            def blocks(t, kt, go):
                t2 = t + TPB // 2
                m1, m2 = after(ms_s[t], go), after(ms_s[t2], go)
                strips = [[] for _ in range(7)]
                for r in range(kt * LANES // ST, (kt + 1) * LANES // ST):
                    a11, a12 = h2(t, r, m1), h2(t, r + KH // ST, m1)
                    a21, a22 = h2(t2, r, m2), h2(t2, r + KH // ST, m2)
                    for j, cmb in enumerate((a11 + a22, a21 + a22, a11, a22, a11 + a12, a21 - a11, a12 - a22)):
                        strips[j].append(cmb)
                for j in range(7):
                    ha_s[j, kt, _tile(t), :] = transposed(strips[j])

            def tail(go):
                for t in range(TPB):
                    m = after(ms_s[t], go)
                    hl_s[_tile(t), 0:D - 2 * KH] = transposed([h2(t, r, m) for r in range(2 * KH // ST, D // ST)])

            half = TPB // 2
            return ([functools.partial(scale, (t, t + half)) for t in range(half)]
                    + [functools.partial(blocks, t, kt) for t in range(half) for kt in range(KH // LANES)] + [tail])

        def col_tiles(c, t):
            return _tile(2 * c * NT + t), _tile((2 * c + 1) * NT + t)

        def prep_gu(w_s, t_s, c, t, rs):
            n1, n2 = col_tiles(c, t)
            for r in rs:
                lo, hi = _rows(r), _rows(r + KH // ST)
                b11, b12 = w_s[lo, n1].astype(f32), w_s[lo, n2].astype(f32)
                b21, b22 = w_s[hi, n1].astype(f32), w_s[hi, n2].astype(f32)
                for j, cmb in enumerate((b11 + b22, b12 - b22, b21 - b11, b11 + b12, b21 + b22)):
                    t_s[c, j, t, lo, :] = cmb.astype(bf16)
                    if j >= 3:
                        mark(cmb)
                if r % pp == 0:
                    pace()

        def prep_gu_steps(c, half):
            return [functools.partial(prep_gu, *((wg_s, tg_s), (wu_s, tu_s))[half], c, t, range(r, r + 8))
                    for t in range(NC // LANES) for r in range(0, KH // ST, 8)]

        def prep_d(c, t, rs):
            n1, n2 = col_tiles(c, t)
            for r in rs:
                lo, hi = _rows(r), _rows(r + RH // ST)
                a11, a12 = wdT_s[lo, n1].astype(f32), wdT_s[lo, n2].astype(f32)
                a21, a22 = wdT_s[hi, n1].astype(f32), wdT_s[hi, n2].astype(f32)
                for j, cmb in enumerate((a11 + a22, a21 + a22, a11, a22, a11 + a12, a21 - a11, a12 - a22)):
                    sd_s[j, c * (NC // LANES) + t, lo, :] = cmb.astype(bf16)
                    if j in (1, 4):
                        mark(cmb)
                if r % pp == 0:
                    pace()

        def prep_d_steps(chunks):
            return [functools.partial(prep_d, c, t, range(r, r + 9))
                    for c in chunks for t in range(NT) for r in range(0, RH // ST, 9)]

        def gate_up_dots(w_s, t_s, c, busy):
            def rhs(j):
                if j == 1:
                    return w_s[0:KH, _tile(2 * c * NT, NT)]
                if j == 4:
                    return w_s[KH:2 * KH, _tile((2 * c + 1) * NT, NT)]
                if j == 7:
                    return w_s[2 * KH:D, _tile(2 * c * NT, 2 * NT)]
                return _operand([words(t_s, c, (0, None, 1, 2, None, 3, 4)[j], k) for k in range(NT)])

            m = []
            for j in range(8):
                lhs = [words(ha_s, j, k) for k in range(KH // LANES)] if j < 7 else [words(hl_s, lanes=slice(0, D - 2 * KH))]
                for e in range(2):
                    if busy(2 * j + e):
                        run(1)
                        lhs = anchor(lhs, e * lhs[0].shape[0] // 2)
                m.append(_dot(_operand(lhs), rhs(j)))
            return m

        def combine(c, g, u):
            for r in range(TH // ST):
                for t in range(NC // LANES):
                    lo, hi = _rows(r), _rows(r + TH // ST)
                    n1, n2 = _tile(t), _tile(t + NC // LANES)

                    def blocks(m):
                        m1, m2, m3, m4, m5, m6, m7 = [x[lo, n1] for x in m[:7]]
                        return (m1 + m4 - m5 + m7 + m[7][lo, n1], m3 + m5 + m[7][lo, n2],
                                m2 + m4 + m[7][hi, n1], m1 - m2 + m3 + m6 + m[7][hi, n2])

                    h11, h12, h21, h22 = [a * b for a, b in zip(blocks(g), blocks(u))]
                    b11, b12, b21, b22 = h11, h21, h12, h22
                    for j, cmb in enumerate((b11 + b22, b11, b12 - b22, b21 - b11, b22, b11 + b12, b21 + b22)):
                        hb_s[j, c * (NC // LANES) + t, lo, :] = cmb.astype(bf16)

        def gate_up_first(c, carry):
            units = [jnp.minimum(2 * c + e, TPB * H // 8 - 1) for e in range(2)]
            for half, (w_s, t_s) in enumerate(((wg_s, tg_s), (wu_s, tu_s))):
                u = units[half]
                weights = prep_gu_steps(c, 1) if half == 0 else prep_gu_steps(jnp.minimum(c + 1, NCH - 1), 0)
                weights = _weave(weights, prep_d_steps([c])[2 * half:2 * half + 2])
                queue.extend(_weave(weights, attn_units([(TPB + u // (H // 8), u % (H // 8))])))
                dots = gate_up_dots(w_s, t_s, c, lambda a: a in slots0[half])
                assert not queue
                if half == 0:
                    gate = dots
            combine(c, gate, dots)
            pending.clear()
            return carry

        def gate_up(i, k, carry):
            n0 = jnp.minimum(i + 1, NB - 1) * TPB
            last = H // 8 - 1
            queue.extend(attn_units([(n0 + k, hg) for hg in range(H // 8)] + [(n0 + TPB - 1, k), (n0 + TPB - 1, last)]))
            for e in range(GC):
                c = GC * k + e
                combine(c, *[gate_up_dots(w_s, t_s, c, lambda a: 16 * half + a in slots)
                             for half, (w_s, t_s) in enumerate(((wg_s, tg_s), (wu_s, tu_s)))])
            assert not queue
            pending.clear()
            return carry

        def down(i):
            m = {}
            steps = ln2_steps(jnp.minimum(i + 1, NB - 1))

            def prod(j):
                m[j] = _dot_nt(_operand([words(sd_s, j - 1, k) for k in range(FT)]),
                               _operand([words(hb_s, j - 1, k) for k in range(FT)]))
                for t in range(pl.cdiv(len(steps), max(7 - len(m), 1))):
                    steps.pop(0)(m[j][:, _tile(t % (TH // LANES))])

            def out(a, b, comb):
                n0 = i * TPB + b * (TPB // 2)
                for r in range(RH // ST):
                    rs = _rows(a * RH // ST + r)
                    x1 = jnp.concatenate([x1_s[n0 + k, rs, :] for k in range(TPB // 2)], axis=1)
                    gb = jnp.concatenate([mod(5, rs)] * (TPB // 2), axis=1)
                    out_s[rs, _tile(n0, TPB // 2)] = (x1 + gb * comb(_rows(r))).astype(bf16)

            prod(2); prod(4)
            out(1, 0, lambda s: m[2][s] + m[4][s])
            prod(1); prod(5); prod(7)
            out(0, 0, lambda s: m[1][s] + m[4][s] - m[5][s] + m[7][s])
            prod(3)
            out(0, 1, lambda s: m[3][s] + m[5][s])
            prod(6)
            out(1, 1, lambda s: m[1][s] - m[2][s] + m[3][s] + m[6][s])
            assert not steps

        def block(i, carry):
            def first(c, carry):
                @pl.when(c == GC)
                def _():
                    for cp in cp_b:
                        cp.wait()

                return gate_up_first(c, carry)

            lax.fori_loop(0, jnp.where(i == 0, NCH, 0), first, None)
            lax.fori_loop(0, jnp.where(i == 0, 0, NCH // GC), functools.partial(gate_up, i), None)

            @pl.when(i + 1 < NB)
            def _():
                project(i + 1)

            down(i)
            out_copy(i, i * TPB, TPB).start()
            return carry

        z_s[...] = jnp.zeros_like(z_s)

        def finish(started):
            for cp in [c for c in started if id(c) not in waited]:
                cp.wait()
            keep = []
            srcs = (hb_s.at[0, 0], ha_s.at[0, 0], hl_s.at[pl.ds(0, 256)], tg_s.at[0, 0, 0], tu_s.at[0, 0, 0], sd_s.at[0, 0, pl.ds(0, 256)],
                    qkv_s.at[12, pl.ds(0, 256)], h_s.at[0, pl.ds(0, 256)], wqkvT_s.at[0, pl.ds(0, 256)], woT_s.at[0, pl.ds(0, 256)])
            for k, src in enumerate(srcs):
                keep.append(copy(src, out_s.at[pl.ds(0, 256), pl.ds(k * 128, 128)]))
            keep.append(copy(x1_s.at[0], x1_s.at[1]))
            keep.append(copy(mod_s.at[pl.ds(0, D)], x1_s.at[2]))
            keep.append(copy(o_s.at[0, pl.ds(0, 16)], z_s))
            keep.append(copy(out_s.at[:, pl.ds(1920, 128)], out_hbm.at[:, pl.ds(1920, 128)]))
            for cp in keep:
                cp.start()
            for cp in keep:
                cp.wait()

        early = [cp_c, cp_x0, cp_m0, *cp_w, cp_x1, cp_x2]
        late = [cp_wo, cp_m1, *cp_a, *cp_b]
        if stop is not None:
            late = late[:2] if stop == 'a' else late[:5]
        for cp in early:
            cp.start(priority=prio[0])
        for cp in late:
            cp.start(priority=prio[1])
        wait(cp_c, cp_x0)
        cv = c_s[...].astype(f32)
        sc = (cv * jax.nn.sigmoid(cv)).astype(bf16).astype(f32)
        sc_s[...] = jnp.broadcast_to(sc, (LANES, D)).T
        first = [ln1_steps(t, h_s, t) for t in range(TPB)]
        for steps in first:
            for step in steps[:2]:
                step()
        wait(cp_m0)
        for j in range(0, 2 * D // LANES, 3):
            mod_tiles(range(j, j + 3))
        for steps in first:
            for step in steps[2:]:
                step(False)

        def ln(i):
            return [step for t in range(TPB) for step in ln1_steps(i * TPB + t, hn_s, t)]

        def next_h():
            run()
            pending.clear()
            h_s[...] = hn_s[...]

        def w_t(p):
            return [functools.partial(transpose_into, wqkvT_s, wqkv_s, k, WCUT[p], WCUT[p + 1]) for k in range(KT)][::-1]

        wait(cp_w[0])
        queue.extend(w_t(0))
        run()
        pending.clear()
        todo = {WAT[0]: ([cp_w[1]], w_t(1)), WAT[1]: ([cp_w[2]], w_t(2)), B0: ([cp_x1], ln(1))}
        for j in range(NQP):
            if j in todo:
                wait(*todo[j][0])
                queue.extend(todo[j][1])
            qkv_piece(0, j, SK if j in todo else 0)
        halo()
        next_h()
        wait(cp_x2)
        if stop == "a":
            finish(early + late)
            return

        def middle(i, carry):
            units = [(i - 1, hg) for hg in range(H // 8)]
            queue.extend(_weave(attn_units(units, True) + attn_units([(i + 1, hg) for hg in range(H // 8 - 1)], True), ln(i + 1)))
            for j in range(NQP):
                qkv_piece(i, j, 0 if j else SK)
            next_h()
            return carry

        lax.fori_loop(1, NB - 1, middle, None)
        wait(cp_wo, cp_m1, *cp_a)
        if stop == "b":
            finish(early + late)
            return
        md = [functools.partial(mod_tiles, range(j, j + 1)) for j in range(2 * D // LANES, 6 * D // LANES)]
        wo_t = [functools.partial(transpose_into, woT_s, wo_s, k, 0, D) for k in range(KT)]
        queue.extend(_weave(attn_units([(n, H // 8 - 1) for n in range(TPB // 2, TPB)], True), md[:-4] + wo_t))
        steps = []
        for j in range(NQP):
            if j == P0:
                run()
                project(0)
                steps = ln2_steps(0)
                queue.extend(_weave(md[-4:], prep_gu_steps(0, 0)))
            y = qkv_piece(NB - 1, j, 0 if j else SK)
            for t in range(min(len(steps), pl.cdiv(len(steps), max(NQP - 1 - j, 1)))):
                steps.pop(0)(y[:, _tile(t % TPB)])
        run()
        pending.clear()
        if stop == 0:
            finish(early + late)
            return

        lax.fori_loop(0, NB, block, None)
        for i in range(NB):
            out_copy(i, i * TPB, TPB).wait()

    def fn(A_x, A_wqkv, A_wo, B_x, B_w_gate, B_w_up, B_w_down, c, w_mod):
        del B_x
        xT = jnp.swapaxes(A_x[0], 0, 1)
        wdT = jnp.swapaxes(B_w_down, 0, 1)
        any_spec = pl.BlockSpec(memory_space=pl.ANY)
        outT = pl.pallas_call(
            kern,
            out_shape=jax.ShapeDtypeStruct((D, S), bf16),
            in_specs=[any_spec] * 8,
            out_specs=any_spec,
            scratch_shapes=[
                pltpu.VMEM((D, S), bf16), pltpu.VMEM((D, 3 * D), bf16), pltpu.VMEM((D, D), bf16),
                pltpu.VMEM((D, F), bf16), pltpu.VMEM((D, F), bf16), pltpu.VMEM((D, F), bf16),
                pltpu.VMEM((1, D), bf16), pltpu.VMEM((D, 6 * D), bf16),
                pltpu.VMEM((KT, 3 * D, LANES), bf16), pltpu.VMEM((KT, D, LANES), bf16),
                pltpu.VMEM((6 * D, LANES), f32), pltpu.VMEM((D, LANES), f32),
                pltpu.VMEM((TPB, D, LANES), bf16), pltpu.VMEM((TPB, D, LANES), bf16),
                pltpu.VMEM((TPB + 1, 3 * D, LANES), bf16), pltpu.VMEM((NTILE - TPB + 1, 3 * D, LANES), bf16), pltpu.VMEM((NTILE, RH, LANES), u32),
                pltpu.VMEM((NTILE, D, LANES), f32),
                pltpu.VMEM((7, KH // LANES, TH, LANES), bf16), pltpu.VMEM((T, LANES), bf16),
                pltpu.VMEM((NCH, 5, NT, KH, LANES), bf16), pltpu.VMEM((NCH, 5, NT, KH, LANES), bf16),
                pltpu.VMEM((7, FT, RH, LANES), bf16), pltpu.VMEM((7, FT, TH, LANES), bf16),
                pltpu.VMEM((D, S), bf16),
                pltpu.VMEM((TPB, 8, LANES), f32), pltpu.VMEM((16, LANES), u32),
                pltpu.SemaphoreType.DMA((32,)), pltpu.SemaphoreType.DMA((NB,)),
            ],
            compiler_params=pltpu.CompilerParams(vmem_limit_bytes=120 * 2**20),
        )(xT, A_wqkv, A_wo, B_w_gate, B_w_up, wdT, c, w_mod)
        return jnp.swapaxes(outT, 0, 1)[None]

    return fn


@jax.jit
def pallas_adaLN_cond__sliding_local_dilated__glu_gated_bilinear__prompt_kernel(
    A_x: jax.Array,
    A_wqkv: jax.Array,
    A_wo: jax.Array,
    B_x: jax.Array,
    B_w_gate: jax.Array,
    B_w_up: jax.Array,
    B_w_down: jax.Array,
    c: jax.Array,
    w_mod: jax.Array,
):
    return make_kernel()(A_x, A_wqkv, A_wo, B_x, B_w_gate, B_w_up, B_w_down, c, w_mod)
```

```python
import functools
import jax
import jax.numpy as jnp
from jax import lax
from jax.experimental import pallas as pl
from jax.experimental.pallas import tpu as pltpu

S, D, F = 2048, 576, 4608
H, DH, W, DIL = 32, 18, 8, 2
EPS = 1e-5
NT_DIMS = (((1,), (1,)), ((), ()))
LANES = 128
NTILE = S // LANES
f32, bf16, u32 = jnp.float32, jnp.bfloat16, jnp.uint32

T = 512
TH = T // 2
TPB = T // LANES
NB = S // T
KH = 256
NC = 256
NCH = F // (2 * NC)
FT = F // 2 // LANES
RH = D // 2
KT = pl.cdiv(D, LANES)
ST = 16
QP = 192
NQP = 3 * D // QP
QH = RH // 2
NSP = 3 * D // RH
GC = 3
NT = NC // LANES


def _unpack(w):
    lo = pltpu.unpack_elementwise(w, index=0, packed_dtype=bf16, unpacked_dtype=f32)
    hi = pltpu.unpack_elementwise(w, index=1, packed_dtype=bf16, unpacked_dtype=f32)
    return lo, hi


def _dot(a, b):
    return jnp.dot(a, b, preferred_element_type=f32)


def _dot_nt(a, b):
    return lax.dot_general(a, b, NT_DIMS, preferred_element_type=f32)


def _add(a, b):
    return b if a is None else a + b


def _rows(r, n=ST):
    return slice(r * n, (r + 1) * n)


def _tile(n, width=1):
    if isinstance(n, int):
        return slice(n * LANES, (n + width) * LANES)
    return pl.ds(pl.multiple_of(n * LANES, LANES), width * LANES)


def _weave(a, b):
    keyed = [((k + 0.5) / len(x), x[k]) for x in (a, b) for k in range(len(x))]
    return [item for _, item in sorted(keyed, key=lambda p: p[0])]


def _lhs_blocks(a11, a12, a21, a22):
    return a11 + a22, a21 + a22, a11, a22, a11 + a12, a21 - a11, a12 - a22


def _rhs_blocks(b11, b12, b21, b22):
    return b11 + b22, b11, b12 - b22, b21 - b11, b22, b11 + b12, b21 + b22


def _out_blocks(m1, m2, m3, m4, m5, m6, m7):
    return m1 + m4 - m5 + m7, m3 + m5, m2 + m4, m1 - m2 + m3 + m6


def _operand(tiles):
    return jnp.concatenate([pltpu.bitcast(w, bf16) for w in tiles], axis=1)


def make_kernel(stop=None, WCUT=(0, 384, 1024, 1728), WAT=(1, 4), prio=(0, 1), P0=3, SK=2, SK0=2, gap=1, wm=2, wp=9, bp=2, order=('awawawawdd', 'dwadwawawa'), qskip=4, qmod=6, qmod3=4, da=(0, 2, 4), LS=((0, 3, 6), (1, 4, 7), (1,)),
                slots=(4, 6, 10, 12, 20, 22, 26, 28), slots0=((4, 5, 6, 7, 8, 9, 10, 11, 13, 15), (2, 3, 4, 6, 7, 8, 9, 10, 12, 13))):
    def kern(xT_hbm, wqkv_hbm, wo_hbm, wg_hbm, wu_hbm, wdT_hbm, c_hbm, wmod_hbm, out_hbm,
             x_s, wqkv_s, wo_s, wg_s, wu_s, wdT_s, c_s, wmod_s,
             wqkvT_s, woT_s, mod_s, sc_s, wa_s, h_s, hb1_s, ht1_s, hbn_s, htn_s, qkv0_s, qkv_s, o_s, x1_s, ha_s, hl_s, tg_s, tu_s, sd_s, hb_s, out_s, ms_s,
             z_s, sems, out_sems):
        sem_id = iter(range(64))

        def copy(src, dst):
            return pltpu.make_async_copy(src, dst, sems.at[next(sem_id)])

        def cols(src, dst, c0, n):
            return copy(src.at[:, pl.ds(c0, n)], dst.at[:, pl.ds(c0, n)])

        cp_c = copy(c_hbm, c_s)
        cp_m0 = [cols(wmod_hbm, wmod_s, c0, 2 * D // 3) for c0 in range(0, 2 * D, 2 * D // 3)]
        cp_m1 = cols(wmod_hbm, wmod_s, 2 * D, 4 * D)
        cp_w = [cols(wqkv_hbm, wqkv_s, c0, c1 - c0) for c0, c1 in zip(WCUT[:-1], WCUT[1:])]
        cp_wo = copy(wo_hbm, wo_s)
        cp_x0 = cols(xT_hbm, x_s, 0, T)
        cp_x1 = cols(xT_hbm, x_s, T, T)
        cp_x2 = cols(xT_hbm, x_s, 2 * T, S - 2 * T)
        ffn = ((wg_hbm, wg_s, (GC + 1) * 2 * NC), (wu_hbm, wu_s, (GC + 1) * 2 * NC), (wdT_hbm, wdT_s, GC * 2 * NC))
        cp_a = [cols(src, dst, 0, n) for src, dst, n in ffn]
        cp_b = [cols(src, dst, n, F - n) for src, dst, n in ffn]

        def out_copy(k, tile0, ntiles):
            idx = (slice(None), _tile(tile0, ntiles))
            return pltpu.make_async_copy(out_s.at[idx], out_hbm.at[idx], out_sems.at[k])

        waited = set()

        def wait(*cps):
            for cp in cps:
                cp.wait()
                waited.add(id(cp))

        queue = []
        pending = []

        def mark(v):
            if v.dtype != f32:
                v = pltpu.bitcast(v, f32)
            for r in range(v.shape[0] // 8):
                q = v[_rows(r, 8)]
                pending[:] = [q + pending[0]] if pending else [q]

        def pace():
            pending[:] = [pltpu.roll(pending[0], 1, 1)]

        def run(n=None):
            for _ in range(len(queue) if n is None else min(n, len(queue))):
                queue.pop(0)()

        def zero_after(v):
            return z_s[pl.ds(1, 8), :] & pltpu.bitcast(v, u32)

        def anchor(tiles, r0=0):
            if not pending:
                return tiles
            z = zero_after(pending.pop())
            out = []
            for w in tiles:
                a = r0 % w.shape[0]
                parts = ([w[:a]] if a else []) + [w[a:a + 8] | z[:, :w.shape[1]]] + ([w[a + 8:]] if a + 8 < w.shape[0] else [])
                out.append(jnp.concatenate(parts, axis=0))
            return out

        def after(x, v):
            return pltpu.bitcast(pltpu.bitcast(x, u32) | zero_after(v[0:8, 0:LANES]), f32)

        def words(ref, *idx, rows=slice(None), lanes=slice(None)):
            if rows.start is not None:
                rows = slice(rows.start // 2, rows.stop // 2)
            return ref.bitcast(u32)[(*idx, rows, lanes)]

        def k_tiles(ref, rows=slice(None)):
            return [words(ref, k, rows=rows, lanes=slice(0, min(LANES, D - k * LANES))) for k in range(KT)]

        def transpose_into(dst, src, k, c0, c1):
            assert src is not wo_s or id(cp_wo) in waited
            n = min(LANES, D - k * LANES)
            t = src[k * LANES:k * LANES + n, c0:c1].T
            dst[k, c0:c1, 0:n] = t
            if n == LANES:
                mark(t[c1 - c0 - ST:])

        def mod_tiles(js):
            assert id(cp_m0[js[0] // 3] if js[0] < 2 * D // LANES else cp_m1) in waited
            acc = [None] * len(js)
            for r in range(D // ST):
                sc = sc_s[_rows(r), :]
                for k, j in enumerate(js):
                    v = sc * wmod_s[_rows(r), _tile(j)].astype(f32)
                    acc[k] = _add(_add(acc[k], v[0:8]), v[8:ST])
            for k, j in enumerate(js):
                col = j * LANES + lax.broadcasted_iota(jnp.int32, (1, LANES), 1)
                is_scale = ((col >= D) & (col < 2 * D)) | ((col >= 4 * D) & (col < 5 * D))
                r = jnp.sum(acc[k], axis=0, keepdims=True) + jnp.where(is_scale, 1.0, 0.0)
                t = jnp.broadcast_to(r, (LANES, LANES)).T
                mod_s[_tile(j), :] = t
                mark(t[LANES - 8:])

        def mod_steps(c0, c1):
            return [functools.partial(mod_tiles, range(j, j + 1)) for j in range(pl.cdiv(c0, LANES), pl.cdiv(c1, LANES))]

        def mod(i, rs):
            return mod_s[i * D + rs.start:i * D + rs.stop, :]

        def col_mean(strips):
            total = functools.reduce(_add, (v[_rows(e, 8)] for v in strips for e in range(2)))
            total = jnp.sum(total, axis=0, keepdims=True) * (1.0 / D)
            return jnp.broadcast_to(total, (8, LANES))

        def twice(v):
            return jnp.concatenate([v, v], axis=0)

        def inv_std(get, m):
            return lax.rsqrt(col_mean(jnp.square(get(r) - twice(m)) for r in range(D // ST)) + EPS)

        def ln1_steps(i, hb=None, ht=None):
            st = {}

            def get(r, p):
                return x_s[_rows(r, 8), _tile(i * TPB + 2 * p, 2)].astype(f32)

            def mean_of(f):
                total = jnp.sum(functools.reduce(_add, map(f, range(D // 8))), axis=0, keepdims=True) * (1.0 / D)
                return jnp.broadcast_to(total, (8, 2 * LANES))

            def mean(p):
                st["m", p] = mean_of(lambda r: get(r, p))
                mark(st["m", p][:, _tile(0)]); mark(st["m", p][:, _tile(1)])

            def scale(p):
                st["rstd", p] = lax.rsqrt(mean_of(lambda r: jnp.square(get(r, p) - st["m", p])) + EPS)
                mark(st["rstd", p][:, _tile(0)]); mark(st["rstd", p][:, _tile(1)])

            def strip(r, p):
                xn = [(get(2 * r + e, p) - st["m", p]) * st["rstd", p] for e in range(2)]
                return [jnp.concatenate([v[:, _tile(t)] for v in xn], axis=0) * mod(1, _rows(r)) + mod(0, _rows(r))
                        for t in range(2)]

            def whole():
                for r in range(D // ST):
                    for p in range(2):
                        for t, v in enumerate(strip(r, p)):
                            h_s[2 * p + t, _rows(r), :] = v.astype(bf16)

            def blocks(rs):
                for r in rs:
                    quads = [strip(r + a * KH // ST, p) for a in range(2) for p in range(2)]
                    for t in range(2):
                        for j, v in enumerate(_rhs_blocks(*[q[t] for q in quads])):
                            hb[j, t, _rows(r), :] = v.astype(bf16)
                            if j in (2, 3):
                                mark(v)
                        if t < bp:
                            pace()

            def tail():
                for r in range(2 * KH // ST, D // ST):
                    for p in range(2):
                        for t, v in enumerate(strip(r, p)):
                            ht[2 * p + t, _rows(r - 2 * KH // ST), :] = v.astype(bf16)
                            mark(v)
                    pace()

            stats = [functools.partial(f, p) for f in (mean, scale) for p in range(2)]
            if hb is None:
                return stats, whole
            return stats + [functools.partial(blocks, range(r, r + 2)) for r in range(0, KH // ST, 2)] + [tail]

        def split_wqkv(p, k):
            for r in range(QH // ST):
                quads = [_unpack(words(wqkvT_s, k + b * KH // LANES, rows=_rows((2 * p + a) * QH // ST + r)))
                         for a in range(2) for b in range(2)]
                even, odd = [_lhs_blocks(*[q[e] for q in quads]) for e in range(2)]
                for n, j in enumerate((0, 1, 4, 5, 6)):
                    w = pltpu.pack_elementwise([even[j], odd[j]], packed_dtype=bf16).astype(u32)
                    wa_s[p, n, k, _rows(r, 8), :] = w
                    if n < wm:
                        mark(w)
                if r % wp == 1:
                    pace()

        def qkv_split_piece(i, p, busy):
            m = []
            for j in range(8):
                if j == 7:
                    lhs = [words(wqkvT_s, KT - 1, rows=_rows(p, RH), lanes=slice(0, D - 2 * KH))]
                    rhs = [words(ht1_s, t) for t in range(TPB)]
                else:
                    lhs = [words(wqkvT_s, k + (j - 2) * KH // LANES, rows=_rows(2 * p + j - 2, QH)) if j in (2, 3)
                           else wa_s[p, j if j < 2 else j - 2, k] for k in range(KH // LANES)]
                    rhs = [words(hb1_s, j, t) for t in range(TPB // 2)]
                for e in range(1 + (j == 7)):
                    if busy(9 * p + j + e):
                        run(1)
                        lhs = anchor(lhs, e * QH // 2)
                m.append(_dot(_operand(lhs), _operand(rhs)))
            for r in range(QH // ST):
                for t in range(TPB // 2):
                    for q, v in enumerate(_out_blocks(*[x[_rows(r), _tile(t)] for x in m[:7]])):
                        a, tt = q // 2, q % 2 * (TPB // 2) + t
                        v = v + m[7][_rows(r + a * QH // ST), _tile(tt)]
                        qkv_s[i * TPB + tt - (TPB - 1), _rows((2 * p + a) * QH // ST + r), :] = v.astype(bf16)
            return m

        def qkv_piece(j, skip):
            tiles = [words(h_s, t, rows=slice(k * LANES, min((k + 1) * LANES, D))) for t in range(TPB) for k in range(KT)]
            for g in range(4 * skip, len(tiles), 4):
                run(1)
                tiles[g:g + 4] = anchor(tiles[g:g + 4], -8)
            rhs = [jnp.concatenate(tiles[t * KT:(t + 1) * KT], axis=0) for t in range(TPB)]
            y = _dot(_operand(k_tiles(wqkvT_s, _rows(j, QP))), _operand(rhs))
            for r in range(QP // ST):
                for t in range(TPB):
                    v, rs = y[_rows(r), _tile(t)].astype(bf16), _rows(j * (QP // ST) + r)
                    qkv0_s[1 + t, rs, :] = v
                    if t == TPB - 1:
                        qkv_s[0, rs, :] = v

        def halo():
            for r in range(D // ST, 3 * D // ST):
                w = words(qkv0_s, 1, rows=_rows(r))
                qkv0_s.bitcast(u32)[0, _rows(r, 8), :] = jnp.broadcast_to(w[:, 0:1], (8, LANES))

        lane = lax.broadcasted_iota(jnp.int32, (8, LANES), 1)

        def shifted(cur, prev, w):
            s = DIL * w
            return cur if w == 0 else pltpu.roll(jnp.where(lane >= LANES - s, prev, cur), s, 1)

        def attn_steps(n, hg, first):
            qkv = (qkv0_s if first else qkv_s).bitcast(u32).at[pl.ds(n if first else n - TPB, 2)]
            acc = [None] * W

            def heads(ref, tile, part):
                start = part * RH + hg * 8 * (DH // 2)
                return ref.at[tile, pl.ds(start if isinstance(start, int) else pl.multiple_of(start, 8), 8 * (DH // 2))]

            def pair(p):
                return pl.ds(p, 8, stride=DH // 2), slice(None)

            def scores(ps, last):
                for p in ps:
                    qlo, qhi = _unpack(heads(qkv, 1, 0)[pair(p)])
                    cur, prev = heads(qkv, 1, 1)[pair(p)], heads(qkv, 0, 1)[pair(p)]
                    for w in range(W):
                        klo, khi = _unpack(shifted(cur, prev, w))
                        acc[w] = _add(acc[w], qlo * klo + qhi * khi)
                if last:
                    lg = [a * (DH ** -0.5) for a in acc]
                    if first:
                        lg = [lg[0]] + [jnp.where(n * LANES + lane >= DIL * w, lg[w], -1e9) for w in range(1, W)]
                    m = functools.reduce(jnp.maximum, lg)
                    e = [jnp.exp(l - m) for l in lg]
                    inv = 1.0 / functools.reduce(_add, e)
                    acc[:] = [x * inv for x in e]
                for a in acc:
                    mark(a)

            def values(ps):
                for p in ps:
                    cur, prev = heads(qkv, 1, 2)[pair(p)], heads(qkv, 0, 2)[pair(p)]
                    olo = ohi = None
                    for w in range(W):
                        vlo, vhi = _unpack(shifted(cur, prev, w))
                        olo, ohi = _add(olo, acc[w] * vlo), _add(ohi, acc[w] * vhi)
                    o = pltpu.pack_elementwise([olo, ohi], packed_dtype=bf16).astype(u32)
                    heads(o_s, n, 0)[pair(p)] = o
                    mark(o)

            return [functools.partial(scores, range(0, 5), False), functools.partial(scores, range(5, 9), True),
                    functools.partial(values, range(0, 5)), functools.partial(values, range(5, 9))]

        def attn_units(units, first=False):
            return [s for n, hg in units for s in attn_steps(n, hg, first)]

        def project(i):
            a = _dot(_operand(anchor(k_tiles(woT_s))), _operand([o_s[i * TPB + t] for t in range(TPB)]))
            for t in range(TPB):
                strips = []
                for r in range(D // ST):
                    x1 = x_s[_rows(r), _tile(i * TPB + t)].astype(f32) + mod(2, _rows(r)) * a[_rows(r), _tile(t)]
                    x1_s[i * TPB + t, _rows(r), :] = x1
                    strips.append(x1)
                ms_s[t] = col_mean(strips)

        def ln2_steps(i):
            st = {}

            def parity_rows(r, e, base=0):
                return pl.ds(base + r * ST + e, 8, stride=2)

            def x1_strip(t, r):
                return jnp.concatenate([x1_s[i * TPB + t, parity_rows(r, e), :] for e in range(2)], axis=0)

            def scale(ts, go):
                for t in ts:
                    st["rstd", t] = inv_std(functools.partial(x1_strip, t), after(ms_s[t], go))

            def h2(t, r, m):
                cb, sb = [jnp.concatenate([mod_s[parity_rows(r, e, k * D), :] for e in range(2)], axis=0) for k in (4, 3)]
                return (x1_strip(t, r) - twice(m)) * twice(st["rstd", t]) * cb + sb

            def transposed(strips):
                w = [pltpu.pack_elementwise([v[0:8], v[8:ST]], packed_dtype=bf16).astype(u32) for v in strips]
                return pltpu.bitcast(jnp.concatenate(w, axis=0), bf16).T

            def blocks(t, kt, go):
                t2 = t + TPB // 2
                m1, m2 = after(ms_s[t], go), after(ms_s[t2], go)
                strips = [[] for _ in range(7)]
                for r in range(kt * LANES // ST, (kt + 1) * LANES // ST):
                    a11, a12 = h2(t, r, m1), h2(t, r + KH // ST, m1)
                    a21, a22 = h2(t2, r, m2), h2(t2, r + KH // ST, m2)
                    for j, cmb in enumerate((a11 + a22, a21 + a22, a11, a22, a11 + a12, a21 - a11, a12 - a22)):
                        strips[j].append(cmb)
                for j in range(7):
                    ha_s[j, kt, _tile(t), :] = transposed(strips[j])

            def tail(go):
                for t in range(TPB):
                    m = after(ms_s[t], go)
                    hl_s[_tile(t), 0:D - 2 * KH] = transposed([h2(t, r, m) for r in range(2 * KH // ST, D // ST)])

            half = TPB // 2
            return ([functools.partial(scale, (t, t + half)) for t in range(half)]
                    + [functools.partial(blocks, t, kt) for t in range(half) for kt in range(KH // LANES)] + [tail])

        def quadrants(w_s, c, r, off):
            return [[w_s[pl.ds(r * ST + 8 * e + a * off, 8), _tile((2 * c + b) * NT, NT)].astype(f32) for e in range(2)]
                    for a in range(2) for b in range(2)]

        def store_blocks(dst, halves, marked):
            for j, (lo, hi) in enumerate(halves):
                for t in range(NT):
                    v = jnp.concatenate([lo[:, _tile(t)], hi[:, _tile(t)]], axis=0)
                    dst(j, t, v.astype(bf16))
                    if j in marked:
                        mark(v)
            pace()

        def prep_gu(w_s, t_s, c, rs):
            for r in rs:
                def dst(j, t, v):
                    t_s[c, j, t, _rows(r), :] = v

                blocks = [(b11 + b22, b12 - b22, b21 - b11, b11 + b12, b21 + b22)
                          for b11, b12, b21, b22 in zip(*quadrants(w_s, c, r, KH))]
                store_blocks(dst, zip(*blocks), (3, 4))

        def prep_gu_steps(c, half):
            return [functools.partial(prep_gu, *((wg_s, tg_s), (wu_s, tu_s))[half], c, range(r, r + 4))
                    for r in range(0, KH // ST, 4)]

        def prep_d(c, rs):
            for r in rs:
                def dst(j, t, v):
                    sd_s[j, c * NT + t, _rows(r), :] = v

                blocks = [(a11 + a22, a21 + a22, a11, a22, a11 + a12, a21 - a11, a12 - a22)
                          for a11, a12, a21, a22 in zip(*quadrants(wdT_s, c, r, RH))]
                store_blocks(dst, zip(*blocks), (1, 4))

        def prep_d_steps(c):
            return [functools.partial(prep_d, c, rs) for rs in (range(0, 5), range(5, 9), range(9, 14), range(14, 18))]

        def gate_up_dots(w_s, t_s, c, busy):
            def rhs(j):
                if j == 1:
                    return w_s[0:KH, _tile(2 * c * NT, NT)]
                if j == 4:
                    return w_s[KH:2 * KH, _tile((2 * c + 1) * NT, NT)]
                if j == 7:
                    return w_s[2 * KH:D, _tile(2 * c * NT, 2 * NT)]
                return _operand([words(t_s, c, (0, None, 1, 2, None, 3, 4)[j], k) for k in range(NT)])

            m = []
            for j in range(8):
                lhs = [words(ha_s, j, k) for k in range(KH // LANES)] if j < 7 else [words(hl_s, lanes=slice(0, D - 2 * KH))]
                for e in range(2):
                    if busy(2 * j + e):
                        run(1)
                        lhs = anchor(lhs, e * lhs[0].shape[0] // 2)
                m.append(_dot(_operand(lhs), rhs(j)))
            return m

        def combine(c, g, u):
            for r in range(TH // ST):
                for t in range(NC // LANES):
                    lo, hi = _rows(r), _rows(r + TH // ST)
                    n1, n2 = _tile(t), _tile(t + NC // LANES)

                    def blocks(m):
                        m1, m2, m3, m4, m5, m6, m7 = [x[lo, n1] for x in m[:7]]
                        return (m1 + m4 - m5 + m7 + m[7][lo, n1], m3 + m5 + m[7][lo, n2],
                                m2 + m4 + m[7][hi, n1], m1 - m2 + m3 + m6 + m[7][hi, n2])

                    h11, h12, h21, h22 = [a * b for a, b in zip(blocks(g), blocks(u))]
                    b11, b12, b21, b22 = h11, h21, h12, h22
                    for j, cmb in enumerate((b11 + b22, b11, b12 - b22, b21 - b11, b22, b11 + b12, b21 + b22)):
                        hb_s[j, c * (NC // LANES) + t, lo, :] = cmb.astype(bf16)

        def gate_up_first(c, carry):
            units = [jnp.minimum(2 * c + e, TPB * H // 8 - 1) for e in range(2)]
            for half, (w_s, t_s) in enumerate(((wg_s, tg_s), (wu_s, tu_s))):
                u = units[half]
                weights = prep_gu_steps(c, 1) if half == 0 else prep_gu_steps(jnp.minimum(c + 1, NCH - 1), 0)
                unit = attn_units([(TPB + u // (H // 8), u % (H // 8))])
                items = {"w": weights, "d": prep_d_steps(c)[da[half]:da[half + 1]], "a": list(unit)}
                queue.extend(items[ch].pop(0) for ch in order[half])
                dots = gate_up_dots(w_s, t_s, c, lambda a: a in slots0[half])
                assert not queue
                if half == 0:
                    gate = dots
            combine(c, gate, dots)
            pending.clear()
            return carry

        def gate_up(i, k, carry):
            n0 = jnp.minimum(i + 1, NB - 1) * TPB
            last = H // 8 - 1
            queue.extend(attn_units([(n0 + k, hg) for hg in range(H // 8)] + [(n0 + TPB - 1, k), (n0 + TPB - 1, last)]))
            for e in range(GC):
                c = GC * k + e
                combine(c, *[gate_up_dots(w_s, t_s, c, lambda a: 16 * half + a in slots)
                             for half, (w_s, t_s) in enumerate(((wg_s, tg_s), (wu_s, tu_s)))])
            assert not queue
            pending.clear()
            return carry

        def down(i):
            m = {}
            steps = ln2_steps(jnp.minimum(i + 1, NB - 1))

            queue.extend(mod_steps(5 * D, 6 * D))

            def prod(j):
                tiles = [words(sd_s, j - 1, k) for k in range(FT)]
                for k in range(0 if m else 8, 16, 4):
                    run(1 if m else 2)
                    tiles[k:k + 4] = anchor(tiles[k:k + 4])
                m[j] = _dot_nt(_operand(tiles), _operand([words(hb_s, j - 1, k) for k in range(FT)]))
                for t in range(pl.cdiv(len(steps), max(7 - len(m), 1))):
                    steps.pop(0)(m[j][:, _tile(t % (TH // LANES))])

            def out(a, b, comb):
                n0 = i * TPB + b * (TPB // 2)
                for r in range(RH // ST):
                    rs = _rows(a * RH // ST + r)
                    x1 = jnp.concatenate([x1_s[n0 + k, rs, :] for k in range(TPB // 2)], axis=1)
                    gb = jnp.concatenate([mod(5, rs)] * (TPB // 2), axis=1)
                    out_s[rs, _tile(n0, TPB // 2)] = (x1 + gb * comb(_rows(r))).astype(bf16)

            prod(2); prod(4)
            out(1, 0, lambda s: m[2][s] + m[4][s])
            prod(1); prod(5); prod(7)
            out(0, 0, lambda s: m[1][s] + m[4][s] - m[5][s] + m[7][s])
            prod(3)
            out(0, 1, lambda s: m[3][s] + m[5][s])
            prod(6)
            out(1, 1, lambda s: m[1][s] - m[2][s] + m[3][s] + m[6][s])
            assert not steps

        def block(i, carry):
            def first(c, carry):
                @pl.when(c == GC)
                def _():
                    for cp in cp_b:
                        cp.wait()

                return gate_up_first(c, carry)

            lax.fori_loop(0, jnp.where(i == 0, NCH, 0), first, None)
            lax.fori_loop(0, jnp.where(i == 0, 0, NCH // GC), functools.partial(gate_up, i), None)

            @pl.when(i + 1 < NB)
            def _():
                project(i + 1)

            down(i)
            out_copy(i, i * TPB, TPB).start()
            return carry

        z_s[...] = jnp.zeros_like(z_s)

        def finish(started):
            for cp in [c for c in started if id(c) not in waited]:
                cp.wait()
            keep = []
            srcs = (hb_s.at[0, 0], ha_s.at[0, 0], hl_s.at[pl.ds(0, 256)], tg_s.at[0, 0, 0], tu_s.at[0, 0, 0], sd_s.at[0, 0, pl.ds(0, 256)],
                    qkv_s.at[12, pl.ds(0, 256)], hb1_s.at[0, 0], wqkvT_s.at[0, pl.ds(0, 256)], woT_s.at[0, pl.ds(0, 256)])
            for k, src in enumerate(srcs):
                keep.append(copy(src, out_s.at[pl.ds(0, 256), pl.ds(k * 128, 128)]))
            keep.append(copy(x1_s.at[0], x1_s.at[1]))
            keep.append(copy(mod_s.at[pl.ds(0, D)], x1_s.at[2]))
            keep.append(copy(o_s.at[0, pl.ds(0, 16)], z_s))
            keep.append(copy(out_s.at[:, pl.ds(1920, 128)], out_hbm.at[:, pl.ds(1920, 128)]))
            for cp in keep:
                cp.start()
            for cp in keep:
                cp.wait()

        early = [cp_c, cp_x0, *cp_m0, *cp_w, cp_x1, cp_x2]
        late = [cp_wo, cp_m1, *cp_a, *cp_b]
        if stop is not None:
            late = late[:2] if stop == 'a' else late[:5]
        for cp in early:
            cp.start(priority=prio[0])
        for cp in late:
            cp.start(priority=prio[1])
        wait(cp_c, cp_x0)
        cv = c_s[...].astype(f32)
        sc = (cv * jax.nn.sigmoid(cv)).astype(bf16).astype(f32)
        sc_s[...] = jnp.broadcast_to(sc, (LANES, D)).T
        stats, apply = ln1_steps(0)
        for step in stats:
            step()
        for j, cp in enumerate(cp_m0):
            wait(cp)
            mod_tiles(range(3 * j, 3 * j + 3))
        apply()

        def next_h():
            run()
            pending.clear()
            hb1_s[...] = hbn_s[...]
            ht1_s[...] = htn_s[...]

        def w_t(p):
            return [functools.partial(transpose_into, wqkvT_s, wqkv_s, k, WCUT[p], WCUT[p + 1]) for k in range(KT)][::-1]

        wait(cp_w[0])
        queue.extend(w_t(0))
        run()
        pending.clear()
        wa = [functools.partial(split_wqkv, p, k) for p in range(NSP) for k in range(KH // LANES)]
        ready = WCUT[2] // RH * (KH // LANES)
        ln = ln1_steps(1, hb1_s, ht1_s)
        idle = [lambda: None]
        todo = {WAT[0]: ([cp_w[1]], w_t(1) + wa[:2] + idle * gap + wa[2:ready]),
                WAT[1]: ([cp_w[2], cp_x1], w_t(2) + ln[:2] + wa[ready:ready + 1] + ln[2:4] + wa[ready + 1:ready + 3]
                         + _weave(ln[4:], wa[ready + 3:]))}
        for j in range(NQP):
            if j in todo:
                wait(*todo[j][0])
                queue.extend(todo[j][1])
            qkv_piece(j, SK0 if j in todo else 0)
        halo()
        run()
        pending.clear()
        wait(cp_x2)
        if stop == "a":
            finish(early + late)
            return

        def middle(i, carry):
            units = [(i - 1, hg) for hg in range(H // 8)]
            queue.extend(_weave(attn_units(units, True) + attn_units([(i + 1, hg) for hg in range(H // 8 - 1)], True), ln1_steps(i + 1, hbn_s, htn_s)))
            for p in range(NSP):
                qkv_split_piece(i, p, lambda a: a >= qskip and a % qmod)
            next_h()
            return carry

        lax.fori_loop(1, NB - 1, middle, None)
        wait(cp_wo, cp_m1, *cp_a)
        if stop == "b":
            finish(early + late)
            return
        md = mod_steps(2 * D, 5 * D)
        gate = pl.cdiv(D, LANES)
        wo_t = [functools.partial(transpose_into, woT_s, wo_s, k, 0, D) for k in range(KT)]
        queue.extend(_weave(attn_units([(n, H // 8 - 1) for n in range(TPB // 2, TPB)], True), md[:gate] + wo_t))
        for p in range(NSP):
            if p == P0:
                run()
                project(0)
                queue.extend(md[gate:] + prep_gu_steps(0, 0))
                steps = ln2_steps(0)
            m = qkv_split_piece(NB - 1, p, lambda a: a >= qskip and a % qmod3)
            for j in LS[p - P0] if p >= P0 else ():
                steps.pop(0)(m[j])
        assert not steps
        run()
        pending.clear()
        if stop == 0:
            finish(early + late)
            return

        lax.fori_loop(0, NB, block, None)
        for i in range(NB):
            out_copy(i, i * TPB, TPB).wait()

    def fn(A_x, A_wqkv, A_wo, B_x, B_w_gate, B_w_up, B_w_down, c, w_mod):
        del B_x
        xT = jnp.swapaxes(A_x[0], 0, 1)
        wdT = jnp.swapaxes(B_w_down, 0, 1)
        any_spec = pl.BlockSpec(memory_space=pl.ANY)
        outT = pl.pallas_call(
            kern,
            out_shape=jax.ShapeDtypeStruct((D, S), bf16),
            in_specs=[any_spec] * 8,
            out_specs=any_spec,
            scratch_shapes=[
                pltpu.VMEM((D, S), bf16), pltpu.VMEM((D, 3 * D), bf16), pltpu.VMEM((D, D), bf16),
                pltpu.VMEM((D, F), bf16), pltpu.VMEM((D, F), bf16), pltpu.VMEM((D, F), bf16),
                pltpu.VMEM((1, D), bf16), pltpu.VMEM((D, 6 * D), bf16),
                pltpu.VMEM((KT, 3 * D, LANES), bf16), pltpu.VMEM((KT, D, LANES), bf16),
                pltpu.VMEM((6 * D, LANES), f32), pltpu.VMEM((D, LANES), f32),
                pltpu.VMEM((NSP, 5, KH // LANES, QH // 2, LANES), u32), pltpu.VMEM((TPB, D, LANES), bf16),
                *[pltpu.VMEM((7, TPB // 2, KH, LANES), bf16), pltpu.VMEM((TPB, D - 2 * KH, LANES), bf16)] * 2,
                pltpu.VMEM((TPB + 1, 3 * D, LANES), bf16), pltpu.VMEM((NTILE - TPB + 1, 3 * D, LANES), bf16), pltpu.VMEM((NTILE, RH, LANES), u32),
                pltpu.VMEM((NTILE, D, LANES), f32),
                pltpu.VMEM((7, KH // LANES, TH, LANES), bf16), pltpu.VMEM((T, LANES), bf16),
                pltpu.VMEM((NCH, 5, NT, KH, LANES), bf16), pltpu.VMEM((NCH, 5, NT, KH, LANES), bf16),
                pltpu.VMEM((7, FT, RH, LANES), bf16), pltpu.VMEM((7, FT, TH, LANES), bf16),
                pltpu.VMEM((D, S), bf16),
                pltpu.VMEM((TPB, 8, LANES), f32), pltpu.VMEM((16, LANES), u32),
                pltpu.SemaphoreType.DMA((32,)), pltpu.SemaphoreType.DMA((NB,)),
            ],
            compiler_params=pltpu.CompilerParams(vmem_limit_bytes=120 * 2**20),
        )(xT, A_wqkv, A_wo, B_w_gate, B_w_up, wdT, c, w_mod)
        return jnp.swapaxes(outT, 0, 1)[None]

    return fn


@jax.jit
def pallas_adaLN_cond__sliding_local_dilated__glu_gated_bilinear__prompt_kernel(
    A_x: jax.Array,
    A_wqkv: jax.Array,
    A_wo: jax.Array,
    B_x: jax.Array,
    B_w_gate: jax.Array,
    B_w_up: jax.Array,
    B_w_down: jax.Array,
    c: jax.Array,
    w_mod: jax.Array,
):
    return make_kernel()(A_x, A_wqkv, A_wo, B_x, B_w_gate, B_w_up, B_w_down, c, w_mod)
```

```python
import functools
import jax
import jax.numpy as jnp
from jax import lax
from jax.experimental import pallas as pl
from jax.experimental.pallas import tpu as pltpu

S, D, F = 2048, 576, 4608
H, DH, W, DIL = 32, 18, 8, 2
EPS = 1e-5
NT_DIMS = (((1,), (1,)), ((), ()))
LANES = 128
NTILE = S // LANES
f32, bf16, u32 = jnp.float32, jnp.bfloat16, jnp.uint32

T = 512
TH = T // 2
TPB = T // LANES
NB = S // T
KH = 256
NC = 256
NCH = F // (2 * NC)
FT = F // 2 // LANES
RH = D // 2
KT = pl.cdiv(D, LANES)
ST = 16
QP = 192
NQP = 3 * D // QP
QH = RH // 2
NSP = 3 * D // RH
GC = 3
NT = NC // LANES


def _unpack(w):
    lo = pltpu.unpack_elementwise(w, index=0, packed_dtype=bf16, unpacked_dtype=f32)
    hi = pltpu.unpack_elementwise(w, index=1, packed_dtype=bf16, unpacked_dtype=f32)
    return lo, hi


def _dot(a, b):
    return jnp.dot(a, b, preferred_element_type=f32)


def _dot_nt(a, b):
    return lax.dot_general(a, b, NT_DIMS, preferred_element_type=f32)


def _add(a, b):
    return b if a is None else a + b


def _rows(r, n=ST):
    return slice(r * n, (r + 1) * n)


def _tile(n, width=1):
    if isinstance(n, int):
        return slice(n * LANES, (n + width) * LANES)
    return pl.ds(pl.multiple_of(n * LANES, LANES), width * LANES)


def _weave(a, b):
    keyed = [((k + 0.5) / len(x), x[k]) for x in (a, b) for k in range(len(x))]
    return [item for _, item in sorted(keyed, key=lambda p: p[0])]


def _lhs_blocks(a11, a12, a21, a22):
    return a11 + a22, a21 + a22, a11, a22, a11 + a12, a21 - a11, a12 - a22


def _rhs_blocks(b11, b12, b21, b22):
    return b11 + b22, b11, b12 - b22, b21 - b11, b22, b11 + b12, b21 + b22


def _out_blocks(m, tail):
    m1, m2, m3, m4, m5, m6, m7 = m
    l11, l12, l21, l22 = tail
    return l11 + m7 - m5 + m4 + m1, l12 + m5 + m3, l21 + m4 + m2, l22 + m6 + m3 - m2 + m1


def _operand(tiles):
    return jnp.concatenate([pltpu.bitcast(w, bf16) for w in tiles], axis=1)


def make_kernel(stop=None, WCUT=(0, 384, 1024, 1728), WAT=(1, 4), prio=(0, 1), P0=3, SK=2, SK0=2, gap=1, wm=2, wp=9, bp=2, order=('awawawawdd', 'dwadwawawa'), qskip=4, qmod=5, qmod3=3, da=(0, 2, 4), LS=((0, 4), (0, 3, 6), (1, 4)),
                slots=(4, 6, 10, 12, 20, 22, 26, 28), slots0=((4, 5, 6, 7, 8, 9, 10, 11, 13, 15), (2, 3, 4, 6, 7, 8, 9, 10, 12, 13))):
    def kern(xT_hbm, wqkv_hbm, wo_hbm, wg_hbm, wu_hbm, wdT_hbm, c_hbm, wmod_hbm, out_hbm,
             x_s, wqkv_s, wo_s, wg_s, wu_s, wdT_s, c_s, wmod_s,
             wqkvT_s, woT_s, mod_s, sc_s, wa_s, h_s, hb1_s, ht1_s, hbn_s, htn_s, qkv0_s, qkv_s, o_s, x1_s, ha_s, hl_s, tg_s, tu_s, sd_s, hb_s, out_s, ms_s,
             z_s, sems, out_sems):
        sem_id = iter(range(64))

        def copy(src, dst):
            return pltpu.make_async_copy(src, dst, sems.at[next(sem_id)])

        def cols(src, dst, c0, n):
            return copy(src.at[:, pl.ds(c0, n)], dst.at[:, pl.ds(c0, n)])

        cp_c = copy(c_hbm, c_s)
        cp_m0 = [cols(wmod_hbm, wmod_s, c0, 2 * D // 3) for c0 in range(0, 2 * D, 2 * D // 3)]
        cp_m1 = cols(wmod_hbm, wmod_s, 2 * D, 4 * D)
        cp_w = [cols(wqkv_hbm, wqkv_s, c0, c1 - c0) for c0, c1 in zip(WCUT[:-1], WCUT[1:])]
        cp_wo = copy(wo_hbm, wo_s)
        cp_x0 = cols(xT_hbm, x_s, 0, T)
        cp_x1 = cols(xT_hbm, x_s, T, T)
        cp_x2 = cols(xT_hbm, x_s, 2 * T, S - 2 * T)
        ffn = ((wg_hbm, wg_s, (GC + 1) * 2 * NC), (wu_hbm, wu_s, (GC + 1) * 2 * NC), (wdT_hbm, wdT_s, GC * 2 * NC))
        cp_a = [cols(src, dst, 0, n) for src, dst, n in ffn]
        cp_b = [cols(src, dst, n, F - n) for src, dst, n in ffn]

        def out_copy(k, tile0, ntiles):
            idx = (slice(None), _tile(tile0, ntiles))
            return pltpu.make_async_copy(out_s.at[idx], out_hbm.at[idx], out_sems.at[k])

        waited = set()
        mod_done = set()

        def wait(*cps):
            for cp in cps:
                cp.wait()
                waited.add(id(cp))

        queue = []
        pending = []

        def mark(v):
            if v.dtype != f32:
                v = pltpu.bitcast(v, f32)
            for r in range(v.shape[0] // 8):
                q = v[_rows(r, 8)]
                pending[:] = [q + pending[0]] if pending else [q]

        def pace():
            pending[:] = [pltpu.roll(pending[0], 1, 1)]

        def run(n=None):
            for _ in range(len(queue) if n is None else min(n, len(queue))):
                queue.pop(0)()

        def zero_after(v):
            return z_s[pl.ds(1, 8), :] & pltpu.bitcast(v, u32)

        def anchor(tiles, r0=0):
            if not pending:
                return tiles
            z = zero_after(pending.pop())
            out = []
            for w in tiles:
                a = r0 % w.shape[0]
                parts = ([w[:a]] if a else []) + [w[a:a + 8] | z[:, :w.shape[1]]] + ([w[a + 8:]] if a + 8 < w.shape[0] else [])
                out.append(jnp.concatenate(parts, axis=0))
            return out

        def after(x, v):
            return pltpu.bitcast(pltpu.bitcast(x, u32) | zero_after(v[0:8, 0:LANES]), f32)

        def words(ref, *idx, rows=slice(None), lanes=slice(None)):
            if rows.start is not None:
                rows = slice(rows.start // 2, rows.stop // 2)
            return ref.bitcast(u32)[(*idx, rows, lanes)]

        def k_tiles(ref, rows=slice(None)):
            return [words(ref, k, rows=rows, lanes=slice(0, min(LANES, D - k * LANES))) for k in range(KT)]

        def transpose_into(dst, src, k, c0, c1):
            assert src is not wo_s or id(cp_wo) in waited
            n = min(LANES, D - k * LANES)
            t = src[k * LANES:k * LANES + n, c0:c1].T
            dst[k, c0:c1, 0:n] = t
            if n == LANES:
                mark(t[c1 - c0 - ST:])

        def mod_tiles(js):
            assert id(cp_m0[js[0] // 3] if js[0] < 2 * D // LANES else cp_m1) in waited
            acc = [None] * len(js)
            for r in range(D // ST):
                sc = sc_s[_rows(r), :]
                for k, j in enumerate(js):
                    v = sc * wmod_s[_rows(r), _tile(j)].astype(f32)
                    acc[k] = _add(_add(acc[k], v[0:8]), v[8:ST])
            for k, j in enumerate(js):
                col = j * LANES + lax.broadcasted_iota(jnp.int32, (1, LANES), 1)
                is_scale = ((col >= D) & (col < 2 * D)) | ((col >= 4 * D) & (col < 5 * D))
                r = jnp.sum(acc[k], axis=0, keepdims=True) + jnp.where(is_scale, 1.0, 0.0)
                t = jnp.broadcast_to(r, (LANES, LANES)).T
                mod_s[_tile(j), :] = t
                mod_done.add(j)
                mark(t[LANES - 8:])

        def mod_steps(c0, c1):
            return [functools.partial(mod_tiles, range(j, j + 1)) for j in range(pl.cdiv(c0, LANES), pl.cdiv(c1, LANES))]

        def mod(i, rs):
            assert (i * D + rs.start) // LANES in mod_done
            return mod_s[i * D + rs.start:i * D + rs.stop, :]

        def col_mean(strips):
            total = functools.reduce(_add, (v[_rows(e, 8)] for v in strips for e in range(2)))
            total = jnp.sum(total, axis=0, keepdims=True) * (1.0 / D)
            return jnp.broadcast_to(total, (8, LANES))

        def twice(v):
            return jnp.concatenate([v, v], axis=0)

        def inv_std(get, m):
            return lax.rsqrt(col_mean(jnp.square(get(r) - twice(m)) for r in range(D // ST)) + EPS)

        def ln1_steps(i, hb=None, ht=None):
            st = {}

            def get(r, p):
                return x_s[_rows(r, 8), _tile(i * TPB + 2 * p, 2)].astype(f32)

            def mean_of(f):
                total = jnp.sum(functools.reduce(_add, map(f, range(D // 8))), axis=0, keepdims=True) * (1.0 / D)
                return jnp.broadcast_to(total, (8, 2 * LANES))

            def mean(p):
                st["m", p] = mean_of(lambda r: get(r, p))
                mark(st["m", p][:, _tile(0)]); mark(st["m", p][:, _tile(1)])

            def scale(p):
                st["rstd", p] = lax.rsqrt(mean_of(lambda r: jnp.square(get(r, p) - st["m", p])) + EPS)
                mark(st["rstd", p][:, _tile(0)]); mark(st["rstd", p][:, _tile(1)])

            def strip(r, p):
                xn = [(get(2 * r + e, p) - st["m", p]) * st["rstd", p] for e in range(2)]
                return [jnp.concatenate([v[:, _tile(t)] for v in xn], axis=0) * mod(1, _rows(r)) + mod(0, _rows(r))
                        for t in range(2)]

            def whole():
                for r in range(D // ST):
                    for p in range(2):
                        for t, v in enumerate(strip(r, p)):
                            h_s[2 * p + t, _rows(r), :] = v.astype(bf16)

            def blocks(rs):
                for r in rs:
                    quads = [strip(r + a * KH // ST, p) for a in range(2) for p in range(2)]
                    for t in range(2):
                        for j, v in enumerate(_rhs_blocks(*[q[t] for q in quads])):
                            hb[j, t, _rows(r), :] = v.astype(bf16)
                            if j in (2, 3):
                                mark(v)
                        if t < bp:
                            pace()

            def tail():
                for r in range(2 * KH // ST, D // ST):
                    for p in range(2):
                        for t, v in enumerate(strip(r, p)):
                            ht[2 * p + t, _rows(r - 2 * KH // ST), :] = v.astype(bf16)
                            mark(v)
                    pace()

            stats = [functools.partial(f, p) for f in (mean, scale) for p in range(2)]
            if hb is None:
                return stats, whole
            return stats + [functools.partial(blocks, range(r, r + 2)) for r in range(0, KH // ST, 2)] + [tail]

        def split_wqkv(p, k):
            for r in range(QH // ST):
                quads = [_unpack(words(wqkvT_s, k + b * KH // LANES, rows=_rows((2 * p + a) * QH // ST + r)))
                         for a in range(2) for b in range(2)]
                even, odd = [_lhs_blocks(*[q[e] for q in quads]) for e in range(2)]
                for n, j in enumerate((0, 1, 4, 5, 6)):
                    w = pltpu.pack_elementwise([even[j], odd[j]], packed_dtype=bf16).astype(u32)
                    wa_s[p, n, k, _rows(r, 8), :] = w
                    if n < wm:
                        mark(w)
                if r % wp == 1:
                    pace()

        def qkv_split_piece(i, p, busy):
            m = []
            for j in range(8):
                if j == 7:
                    lhs = [words(wqkvT_s, KT - 1, rows=_rows(p, RH), lanes=slice(0, D - 2 * KH))]
                    rhs = [words(ht1_s, t) for t in range(TPB)]
                else:
                    lhs = [words(wqkvT_s, k + (j - 2) * KH // LANES, rows=_rows(2 * p + j - 2, QH)) if j in (2, 3)
                           else wa_s[p, j if j < 2 else j - 2, k] for k in range(KH // LANES)]
                    rhs = [words(hb1_s, j, t) for t in range(TPB // 2)]
                for e in range(1 + (j == 7)):
                    if busy(9 * p + j + e):
                        run(1)
                        lhs = anchor(lhs, e * QH // 2)
                m.append(_dot(_operand(lhs), _operand(rhs)))
            for r in range(QH // ST):
                for t in range(TPB // 2):
                    tail = [m[7][_rows(r + a * QH // ST), _tile(b * TPB // 2 + t)] for a in range(2) for b in range(2)]
                    for q, v in enumerate(_out_blocks([x[_rows(r), _tile(t)] for x in m[:7]], tail)):
                        a, tt = q // 2, q % 2 * (TPB // 2) + t
                        qkv_s[i * TPB + tt - (TPB - 1), _rows((2 * p + a) * QH // ST + r), :] = v.astype(bf16)
            return m

        def qkv_piece(j, skip):
            tiles = [words(h_s, t, rows=slice(k * LANES, min((k + 1) * LANES, D))) for t in range(TPB) for k in range(KT)]
            for g in range(4 * skip, len(tiles), 4):
                run(1)
                tiles[g:g + 4] = anchor(tiles[g:g + 4], -8)
            rhs = [jnp.concatenate(tiles[t * KT:(t + 1) * KT], axis=0) for t in range(TPB)]
            y = _dot(_operand(k_tiles(wqkvT_s, _rows(j, QP))), _operand(rhs))
            for r in range(QP // ST):
                for t in range(TPB):
                    v, rs = y[_rows(r), _tile(t)].astype(bf16), _rows(j * (QP // ST) + r)
                    qkv0_s[1 + t, rs, :] = v
                    if t == TPB - 1:
                        qkv_s[0, rs, :] = v

        def halo():
            for r in range(D // ST, 3 * D // ST):
                w = words(qkv0_s, 1, rows=_rows(r))
                qkv0_s.bitcast(u32)[0, _rows(r, 8), :] = jnp.broadcast_to(w[:, 0:1], (8, LANES))

        lane = lax.broadcasted_iota(jnp.int32, (8, LANES), 1)

        def shifted(cur, prev, w):
            s = DIL * w
            return cur if w == 0 else pltpu.roll(jnp.where(lane >= LANES - s, prev, cur), s, 1)

        def attn_steps(n, hg, first):
            qkv = (qkv0_s if first else qkv_s).bitcast(u32).at[pl.ds(n if first else n - TPB, 2)]
            acc = [None] * W

            def heads(ref, tile, part):
                start = part * RH + hg * 8 * (DH // 2)
                return ref.at[tile, pl.ds(start if isinstance(start, int) else pl.multiple_of(start, 8), 8 * (DH // 2))]

            def pair(p):
                return pl.ds(p, 8, stride=DH // 2), slice(None)

            def scores(ps, last):
                for p in ps:
                    qlo, qhi = _unpack(heads(qkv, 1, 0)[pair(p)])
                    cur, prev = heads(qkv, 1, 1)[pair(p)], heads(qkv, 0, 1)[pair(p)]
                    for w in range(W):
                        klo, khi = _unpack(shifted(cur, prev, w))
                        acc[w] = _add(acc[w], qlo * klo + qhi * khi)
                if last:
                    lg = [a * (DH ** -0.5) for a in acc]
                    if first:
                        lg = [lg[0]] + [jnp.where(n * LANES + lane >= DIL * w, lg[w], -1e9) for w in range(1, W)]
                    m = functools.reduce(jnp.maximum, lg)
                    e = [jnp.exp(l - m) for l in lg]
                    inv = 1.0 / functools.reduce(_add, e)
                    acc[:] = [x * inv for x in e]
                for a in acc:
                    mark(a)

            def values(ps):
                for p in ps:
                    cur, prev = heads(qkv, 1, 2)[pair(p)], heads(qkv, 0, 2)[pair(p)]
                    olo = ohi = None
                    for w in range(W):
                        vlo, vhi = _unpack(shifted(cur, prev, w))
                        olo, ohi = _add(olo, acc[w] * vlo), _add(ohi, acc[w] * vhi)
                    o = pltpu.pack_elementwise([olo, ohi], packed_dtype=bf16).astype(u32)
                    heads(o_s, n, 0)[pair(p)] = o
                    mark(o)

            return [functools.partial(scores, range(0, 5), False), functools.partial(scores, range(5, 9), True),
                    functools.partial(values, range(0, 5)), functools.partial(values, range(5, 9))]

        def attn_units(units, first=False):
            return [s for n, hg in units for s in attn_steps(n, hg, first)]

        def project(i):
            a = _dot(_operand(anchor(k_tiles(woT_s))), _operand([o_s[i * TPB + t] for t in range(TPB)]))
            for t in range(TPB):
                strips = []
                for r in range(D // ST):
                    x1 = x_s[_rows(r), _tile(i * TPB + t)].astype(f32) + mod(2, _rows(r)) * a[_rows(r), _tile(t)]
                    x1_s[i * TPB + t, _rows(r), :] = x1
                    strips.append(x1)
                ms_s[t] = col_mean(strips)

        def ln2_steps(i):
            st = {}

            def parity_rows(r, e, base=0):
                return pl.ds(base + r * ST + e, 8, stride=2)

            def x1_strip(t, r):
                return jnp.concatenate([x1_s[i * TPB + t, parity_rows(r, e), :] for e in range(2)], axis=0)

            def scale(ts, go):
                for t in ts:
                    st["rstd", t] = inv_std(functools.partial(x1_strip, t), after(ms_s[t], go))

            def h2(t, r, m):
                assert {(k * D + r * ST) // LANES for k in (3, 4)} <= mod_done
                cb, sb = [jnp.concatenate([mod_s[parity_rows(r, e, k * D), :] for e in range(2)], axis=0) for k in (4, 3)]
                return (x1_strip(t, r) - twice(m)) * twice(st["rstd", t]) * cb + sb

            def transposed(strips):
                w = [pltpu.pack_elementwise([v[0:8], v[8:ST]], packed_dtype=bf16).astype(u32) for v in strips]
                return pltpu.bitcast(jnp.concatenate(w, axis=0), bf16).T

            def blocks(t, kt, go):
                t2 = t + TPB // 2
                m1, m2 = after(ms_s[t], go), after(ms_s[t2], go)
                strips = [[] for _ in range(7)]
                for r in range(kt * LANES // ST, (kt + 1) * LANES // ST):
                    a11, a12 = h2(t, r, m1), h2(t, r + KH // ST, m1)
                    a21, a22 = h2(t2, r, m2), h2(t2, r + KH // ST, m2)
                    for j, cmb in enumerate((a11 + a22, a21 + a22, a11, a22, a11 + a12, a21 - a11, a12 - a22)):
                        strips[j].append(cmb)
                for j in range(7):
                    ha_s[j, kt, _tile(t), :] = transposed(strips[j])

            def tail(go):
                for t in range(TPB):
                    m = after(ms_s[t], go)
                    blk = transposed([h2(t, r, m) for r in range(2 * KH // ST, D // ST)])
                    for r in range(LANES // ST):
                        half, strip = divmod(t * LANES // ST + r, TH // ST)
                        hl_s[_rows(2 * strip + half), 0:D - 2 * KH] = blk[_rows(r)]

            half = TPB // 2
            return ([functools.partial(scale, (t, t + half)) for t in range(half)]
                    + [functools.partial(blocks, t, kt) for t in range(half) for kt in range(KH // LANES)] + [tail])

        def quadrants(w_s, c, r, off):
            return [[w_s[pl.ds(r * ST + 8 * e + a * off, 8), _tile((2 * c + b) * NT, NT)].astype(f32) for e in range(2)]
                    for a in range(2) for b in range(2)]

        def store_blocks(dst, halves, marked):
            for j, (lo, hi) in enumerate(halves):
                for t in range(NT):
                    v = jnp.concatenate([lo[:, _tile(t)], hi[:, _tile(t)]], axis=0)
                    dst(j, t, v.astype(bf16))
                    if j in marked:
                        mark(v)
            pace()

        def prep_gu(w_s, t_s, c, rs):
            for r in rs:
                def dst(j, t, v):
                    t_s[c, j, t, _rows(r), :] = v

                blocks = [(b11 + b22, b12 - b22, b21 - b11, b11 + b12, b21 + b22)
                          for b11, b12, b21, b22 in zip(*quadrants(w_s, c, r, KH))]
                store_blocks(dst, zip(*blocks), (3, 4))

        def prep_gu_steps(c, half):
            return [functools.partial(prep_gu, *((wg_s, tg_s), (wu_s, tu_s))[half], c, range(r, r + 4))
                    for r in range(0, KH // ST, 4)]

        def prep_d(c, rs):
            for r in rs:
                def dst(j, t, v):
                    sd_s[j, c * NT + t, _rows(r), :] = v

                blocks = [(a11 + a22, a21 + a22, a11, a22, a11 + a12, a21 - a11, a12 - a22)
                          for a11, a12, a21, a22 in zip(*quadrants(wdT_s, c, r, RH))]
                store_blocks(dst, zip(*blocks), (1, 4))

        def prep_d_steps(c):
            return [functools.partial(prep_d, c, rs) for rs in (range(0, 5), range(5, 9), range(9, 14), range(14, 18))]

        def gate_up_dots(w_s, t_s, c, busy):
            def rhs(j):
                if j == 1:
                    return w_s[0:KH, _tile(2 * c * NT, NT)]
                if j == 4:
                    return w_s[KH:2 * KH, _tile((2 * c + 1) * NT, NT)]
                if j == 7:
                    return w_s[2 * KH:D, _tile(2 * c * NT, 2 * NT)]
                return _operand([words(t_s, c, (0, None, 1, 2, None, 3, 4)[j], k) for k in range(NT)])

            m = []
            for j in range(8):
                lhs = [words(ha_s, j, k) for k in range(KH // LANES)] if j < 7 else [words(hl_s, lanes=slice(0, D - 2 * KH))]
                for e in range(2):
                    if busy(2 * j + e):
                        run(1)
                        lhs = anchor(lhs, e * lhs[0].shape[0] // 2)
                m.append(_dot(_operand(lhs), rhs(j)))
            return m

        def combine(c, g, u):
            for r in range(TH // ST):
                for t in range(NC // LANES):
                    lo = _rows(r)

                    def blocks(m):
                        tail = [m[7][_rows(2 * r + a), _tile(b * NT + t)] for a in range(2) for b in range(2)]
                        return _out_blocks([x[lo, _tile(t)] for x in m[:7]], tail)

                    h11, h12, h21, h22 = [a * b for a, b in zip(blocks(g), blocks(u))]
                    b11, b12, b21, b22 = h11, h21, h12, h22
                    for j, cmb in enumerate((b11 + b22, b11, b12 - b22, b21 - b11, b22, b11 + b12, b21 + b22)):
                        hb_s[j, c * (NC // LANES) + t, lo, :] = cmb.astype(bf16)

        def gate_up_first(c, carry):
            units = [jnp.minimum(2 * c + e, TPB * H // 8 - 1) for e in range(2)]
            for half, (w_s, t_s) in enumerate(((wg_s, tg_s), (wu_s, tu_s))):
                u = units[half]
                weights = prep_gu_steps(c, 1) if half == 0 else prep_gu_steps(jnp.minimum(c + 1, NCH - 1), 0)
                unit = attn_units([(TPB + u // (H // 8), u % (H // 8))])
                items = {"w": weights, "d": prep_d_steps(c)[da[half]:da[half + 1]], "a": list(unit)}
                queue.extend(items[ch].pop(0) for ch in order[half])
                dots = gate_up_dots(w_s, t_s, c, lambda a: a in slots0[half])
                assert not queue
                if half == 0:
                    gate = dots
            combine(c, gate, dots)
            pending.clear()
            return carry

        def gate_up(i, k, carry):
            n0 = jnp.minimum(i + 1, NB - 1) * TPB
            last = H // 8 - 1
            queue.extend(attn_units([(n0 + k, hg) for hg in range(H // 8)] + [(n0 + TPB - 1, k), (n0 + TPB - 1, last)]))
            for e in range(GC):
                c = GC * k + e
                combine(c, *[gate_up_dots(w_s, t_s, c, lambda a: 16 * half + a in slots)
                             for half, (w_s, t_s) in enumerate(((wg_s, tg_s), (wu_s, tu_s)))])
            assert not queue
            pending.clear()
            return carry

        def down(i):
            m = {}
            steps = ln2_steps(jnp.minimum(i + 1, NB - 1))

            queue.extend(mod_steps(5 * D, 6 * D))

            def prod(j):
                tiles = [words(sd_s, j - 1, k) for k in range(FT)]
                for k in range(0 if m else 8, 16, 4):
                    run(1 if m else 2)
                    tiles[k:k + 4] = anchor(tiles[k:k + 4])
                m[j] = _dot_nt(_operand(tiles), _operand([words(hb_s, j - 1, k) for k in range(FT)]))
                for t in range(pl.cdiv(len(steps), max(7 - len(m), 1))):
                    steps.pop(0)(m[j][:, _tile(t % (TH // LANES))])

            def out(a, b, comb):
                n0 = i * TPB + b * (TPB // 2)
                for r in range(RH // ST):
                    rs = _rows(a * RH // ST + r)
                    x1 = jnp.concatenate([x1_s[n0 + k, rs, :] for k in range(TPB // 2)], axis=1)
                    gb = jnp.concatenate([mod(5, rs)] * (TPB // 2), axis=1)
                    out_s[rs, _tile(n0, TPB // 2)] = (x1 + gb * comb(_rows(r))).astype(bf16)

            prod(2); prod(4)
            out(1, 0, lambda s: m[2][s] + m[4][s])
            prod(1); prod(5); prod(7)
            out(0, 0, lambda s: m[7][s] - m[5][s] + m[4][s] + m[1][s])
            prod(3)
            out(0, 1, lambda s: m[3][s] + m[5][s])
            prod(6)
            out(1, 1, lambda s: m[6][s] + m[3][s] - m[2][s] + m[1][s])
            assert not steps

        def block(i, carry):
            def first(c, carry):
                @pl.when(c == GC)
                def _():
                    for cp in cp_b:
                        cp.wait()

                return gate_up_first(c, carry)

            lax.fori_loop(0, jnp.where(i == 0, NCH, 0), first, None)
            lax.fori_loop(0, jnp.where(i == 0, 0, NCH // GC), functools.partial(gate_up, i), None)

            @pl.when(i + 1 < NB)
            def _():
                project(i + 1)

            down(i)
            out_copy(i, i * TPB, TPB).start()
            return carry

        z_s[...] = jnp.zeros_like(z_s)

        def finish(started):
            for cp in [c for c in started if id(c) not in waited]:
                cp.wait()
            keep = []
            srcs = (hb_s.at[0, 0], ha_s.at[0, 0], hl_s.at[pl.ds(0, 256)], tg_s.at[0, 0, 0], tu_s.at[0, 0, 0], sd_s.at[0, 0, pl.ds(0, 256)],
                    qkv_s.at[12, pl.ds(0, 256)], hb1_s.at[0, 0], wqkvT_s.at[0, pl.ds(0, 256)], woT_s.at[0, pl.ds(0, 256)])
            for k, src in enumerate(srcs):
                keep.append(copy(src, out_s.at[pl.ds(0, 256), pl.ds(k * 128, 128)]))
            keep.append(copy(x1_s.at[0], x1_s.at[1]))
            keep.append(copy(mod_s.at[pl.ds(0, D)], x1_s.at[2]))
            keep.append(copy(o_s.at[0, pl.ds(0, 16)], z_s))
            keep.append(copy(out_s.at[:, pl.ds(1920, 128)], out_hbm.at[:, pl.ds(1920, 128)]))
            for cp in keep:
                cp.start()
            for cp in keep:
                cp.wait()

        early = [cp_c, cp_x0, *cp_m0, *cp_w, cp_x1, cp_x2]
        late = [cp_wo, cp_m1, *cp_a, *cp_b]
        if stop is not None:
            late = late[:2] if stop == 'a' else late[:5]
        for cp in early:
            cp.start(priority=prio[0])
        for cp in late:
            cp.start(priority=prio[1])
        wait(cp_c, cp_x0)
        cv = c_s[...].astype(f32)
        sc = (cv * jax.nn.sigmoid(cv)).astype(bf16).astype(f32)
        sc_s[...] = jnp.broadcast_to(sc, (LANES, D)).T
        stats, apply = ln1_steps(0)
        for step in stats:
            step()
        for j, cp in enumerate(cp_m0):
            wait(cp)
            mod_tiles(range(3 * j, 3 * j + 3))
        apply()

        def next_h():
            run()
            pending.clear()
            hb1_s[...] = hbn_s[...]
            ht1_s[...] = htn_s[...]

        def w_t(p):
            return [functools.partial(transpose_into, wqkvT_s, wqkv_s, k, WCUT[p], WCUT[p + 1]) for k in range(KT)][::-1]

        wait(cp_w[0])
        queue.extend(w_t(0))
        run()
        pending.clear()
        wa = [functools.partial(split_wqkv, p, k) for p in range(NSP) for k in range(KH // LANES)]
        ready = WCUT[2] // RH * (KH // LANES)
        ln = ln1_steps(1, hb1_s, ht1_s)
        idle = [lambda: None]
        todo = {WAT[0]: ([cp_w[1]], w_t(1) + wa[:2] + idle * gap + wa[2:ready]),
                WAT[1]: ([cp_w[2], cp_x1], w_t(2) + ln[:2] + wa[ready:ready + 1] + ln[2:4] + wa[ready + 1:ready + 3]
                         + _weave(ln[4:], wa[ready + 3:]))}
        for j in range(NQP):
            if j in todo:
                wait(*todo[j][0])
                queue.extend(todo[j][1])
            qkv_piece(j, SK0 if j in todo else 0)
        halo()
        run()
        pending.clear()
        wait(cp_x2)
        if stop == "a":
            finish(early + late)
            return

        def middle(i, carry):
            units = [(i - 1, hg) for hg in range(H // 8)]
            queue.extend(_weave(attn_units(units, True) + attn_units([(i + 1, hg) for hg in range(H // 8 - 1)], True), ln1_steps(i + 1, hbn_s, htn_s)))
            for p in range(NSP):
                qkv_split_piece(i, p, lambda a: a >= qskip and a % qmod)
            next_h()
            return carry

        lax.fori_loop(1, NB - 1, middle, None)
        wait(cp_wo, cp_m1, *cp_a)
        if stop == "b":
            finish(early + late)
            return
        md = mod_steps(2 * D, 5 * D)
        gate = pl.cdiv(D, LANES)
        wo_t = [functools.partial(transpose_into, woT_s, wo_s, k, 0, D) for k in range(KT)]
        queue.extend(_weave(attn_units([(n, H // 8 - 1) for n in range(TPB // 2, TPB)], True), md[:gate] + wo_t))
        for p in range(NSP):
            if p == P0:
                run()
                project(0)
                queue.extend(md[gate:] + prep_gu_steps(0, 0))
                steps = ln2_steps(0)
            m = qkv_split_piece(NB - 1, p, lambda a: a >= qskip and a % qmod3)
            for j in LS[p - P0] if p >= P0 else ():
                steps.pop(0)(m[j])
        assert not steps
        run()
        pending.clear()
        if stop == 0:
            finish(early + late)
            return

        lax.fori_loop(0, NB, block, None)
        for i in range(NB):
            out_copy(i, i * TPB, TPB).wait()

    def fn(A_x, A_wqkv, A_wo, B_x, B_w_gate, B_w_up, B_w_down, c, w_mod):
        del B_x
        xT = jnp.swapaxes(A_x[0], 0, 1)
        wdT = jnp.swapaxes(B_w_down, 0, 1)
        any_spec = pl.BlockSpec(memory_space=pl.ANY)
        outT = pl.pallas_call(
            kern,
            out_shape=jax.ShapeDtypeStruct((D, S), bf16),
            in_specs=[any_spec] * 8,
            out_specs=any_spec,
            scratch_shapes=[
                pltpu.VMEM((D, S), bf16), pltpu.VMEM((D, 3 * D), bf16), pltpu.VMEM((D, D), bf16),
                pltpu.VMEM((D, F), bf16), pltpu.VMEM((D, F), bf16), pltpu.VMEM((D, F), bf16),
                pltpu.VMEM((1, D), bf16), pltpu.VMEM((D, 6 * D), bf16),
                pltpu.VMEM((KT, 3 * D, LANES), bf16), pltpu.VMEM((KT, D, LANES), bf16),
                pltpu.VMEM((6 * D, LANES), f32), pltpu.VMEM((D, LANES), f32),
                pltpu.VMEM((NSP, 5, KH // LANES, QH // 2, LANES), u32), pltpu.VMEM((TPB, D, LANES), bf16),
                *[pltpu.VMEM((7, TPB // 2, KH, LANES), bf16), pltpu.VMEM((TPB, D - 2 * KH, LANES), bf16)] * 2,
                pltpu.VMEM((TPB + 1, 3 * D, LANES), bf16), pltpu.VMEM((NTILE - TPB + 1, 3 * D, LANES), bf16), pltpu.VMEM((NTILE, RH, LANES), u32),
                pltpu.VMEM((NTILE, D, LANES), f32),
                pltpu.VMEM((7, KH // LANES, TH, LANES), bf16), pltpu.VMEM((T, LANES), bf16),
                pltpu.VMEM((NCH, 5, NT, KH, LANES), bf16), pltpu.VMEM((NCH, 5, NT, KH, LANES), bf16),
                pltpu.VMEM((7, FT, RH, LANES), bf16), pltpu.VMEM((7, FT, TH, LANES), bf16),
                pltpu.VMEM((D, S), bf16),
                pltpu.VMEM((TPB, 8, LANES), f32), pltpu.VMEM((16, LANES), u32),
                pltpu.SemaphoreType.DMA((32,)), pltpu.SemaphoreType.DMA((NB,)),
            ],
            compiler_params=pltpu.CompilerParams(vmem_limit_bytes=120 * 2**20),
        )(xT, A_wqkv, A_wo, B_w_gate, B_w_up, wdT, c, w_mod)
        return jnp.swapaxes(outT, 0, 1)[None]

    return fn


@jax.jit
def pallas_adaLN_cond__sliding_local_dilated__glu_gated_bilinear__prompt_kernel(
    A_x: jax.Array,
    A_wqkv: jax.Array,
    A_wo: jax.Array,
    B_x: jax.Array,
    B_w_gate: jax.Array,
    B_w_up: jax.Array,
    B_w_down: jax.Array,
    c: jax.Array,
    w_mod: jax.Array,
):
    return make_kernel()(A_x, A_wqkv, A_wo, B_x, B_w_gate, B_w_up, B_w_down, c, w_mod)
```

```python
import functools

import jax
import jax.numpy as jnp
from jax import lax
from jax.experimental import pallas as pl
from jax.experimental.pallas import tpu as pltpu

S, D, F = 2048, 576, 4608
H, DH, W, DIL = 32, 18, 8, 2
EPS = 1e-5
f32, bf16, u32 = jnp.float32, jnp.bfloat16, jnp.uint32

LANES = 128
ST = 16
NTILE = S // LANES
KT = pl.cdiv(D, LANES)
RH = D // 2
HG = H // 8

T = 512
TH = T // 2
TPB = T // LANES
NB = S // T
KH = 256
NC = 256
NT = NC // LANES
NCH = F // (2 * NC)
FT = F // 2 // LANES
GC = 3
QP = 192
NQP = 3 * D // QP
QH = RH // 2
NSP = 3 * D // RH

MOD_CUTS = (0, 3, 6, 9)
WQKV_CUTS = (0, 384, 1024, 3 * D)


def _unpack(w):
    return [pltpu.unpack_elementwise(w, index=e, packed_dtype=bf16, unpacked_dtype=f32) for e in range(2)]


def _pack(even, odd):
    return pltpu.pack_elementwise([even, odd], packed_dtype=bf16).astype(u32)


def _operand(tiles):
    return jnp.concatenate([pltpu.bitcast(w, bf16) for w in tiles], axis=1)


def _dot(a, b):
    return jnp.dot(a, b, preferred_element_type=f32)


def _dot_nt(a, b):
    return lax.dot_general(a, b, (((1,), (1,)), ((), ())), preferred_element_type=f32)


def _lhs_blocks(a11, a12, a21, a22):
    return a11 + a22, a21 + a22, a11, a22, a11 + a12, a21 - a11, a12 - a22


def _rhs_blocks(b11, b12, b21, b22):
    return b11 + b22, b11, b12 - b22, b21 - b11, b22, b11 + b12, b21 + b22


def _out_blocks(m, tail):
    m1, m2, m3, m4, m5, m6, m7 = m
    l11, l12, l21, l22 = tail
    return l11 + m7 - m5 + m4 + m1, l12 + m5 + m3, l21 + m4 + m2, l22 + m6 + m3 - m2 + m1


def _add(a, b):
    return b if a is None else a + b


def _rows(r, n=ST):
    return slice(r * n, (r + 1) * n)


def _tile(n, width=1):
    if isinstance(n, int):
        return slice(n * LANES, (n + width) * LANES)
    return pl.ds(pl.multiple_of(n * LANES, LANES), width * LANES)


def _weave(a, b):
    keyed = [((k + 0.5) / len(x), x[k]) for x in (a, b) for k in range(len(x))]
    return [item for _, item in sorted(keyed, key=lambda p: p[0])]


def _ordered(order, **lists):
    lists = {name[0]: list(v) for name, v in lists.items()}
    merged = [lists[ch].pop(0) for ch in order]
    assert not any(lists.values())
    return merged


def _kernel(xT_hbm, wqkv_hbm, wo_hbm, wg_hbm, wu_hbm, wdT_hbm, c_hbm, wmod_hbm, out_hbm,
            x_s, wqkv_s, wo_s, wg_s, wu_s, wdT_s, c_s, wmod_s,
            wqkvT_s, woT_s, mod_s, sc_s, wa_s, h_s, hb1_s, ht1_s, hbn_s, htn_s, qkv0_s, qkv_s, o_s,
            x1_s, ha_s, hl_s, tg_s, tu_s, sd_s, hb_s, out_s, ms_s, z_s, sems, out_sems):
    sem_ids = iter(range(sems.shape[0]))

    def copy(src, dst):
        return pltpu.make_async_copy(src, dst, sems.at[next(sem_ids)])

    def cols(src, dst, c0, c1):
        return copy(src.at[:, pl.ds(c0, c1 - c0)], dst.at[:, pl.ds(c0, c1 - c0)])

    cp_c = copy(c_hbm, c_s)
    cp_m0 = [cols(wmod_hbm, wmod_s, t0 * LANES, t1 * LANES) for t0, t1 in zip(MOD_CUTS[:-1], MOD_CUTS[1:])]
    cp_m1 = cols(wmod_hbm, wmod_s, 2 * D, 6 * D)
    cp_w = [cols(wqkv_hbm, wqkv_s, c0, c1) for c0, c1 in zip(WQKV_CUTS[:-1], WQKV_CUTS[1:])]
    cp_wo = copy(wo_hbm, wo_s)
    cp_x0 = [cols(xT_hbm, x_s, p * TH, (p + 1) * TH) for p in range(2)]
    cp_x1 = cols(xT_hbm, x_s, T, 2 * T)
    cp_x2 = cols(xT_hbm, x_s, 2 * T, S)
    ffn = ((wg_hbm, wg_s, (GC + 1) * 2 * NC), (wu_hbm, wu_s, (GC + 1) * 2 * NC), (wdT_hbm, wdT_s, GC * 2 * NC))
    cp_a = [cols(src, dst, 0, n) for src, dst, n in ffn]
    cp_b = [cols(src, dst, n, F) for src, dst, n in ffn]

    def out_copy(i, q):
        rows = (slice(0, D), slice(0, RH), slice(RH, D))[q]
        idx = (rows, _tile(i * TPB + (q > 0) * TPB // 2, TPB // 2))
        return pltpu.make_async_copy(out_s.at[idx], out_hbm.at[idx], out_sems.at[3 * i + q])

    def wait(*cps):
        for cp in cps:
            cp.wait()

    queue = []
    pending = []

    def mark(v):
        if v.dtype != f32:
            v = pltpu.bitcast(v, f32)
        for r in range(v.shape[0] // 8):
            q = v[_rows(r, 8)]
            pending[:] = [q + pending[0]] if pending else [q]

    def pace():
        pending[:] = [pltpu.roll(pending[0], 1, 1)]

    def run(n=None):
        for _ in range(len(queue) if n is None else min(n, len(queue))):
            queue.pop(0)()

    def drain():
        run()
        pending.clear()

    def zero_after(v):
        return z_s[pl.ds(1, 8), :] & pltpu.bitcast(v, u32)

    def anchor(tiles, r0=0):
        if not pending:
            return tiles
        z = zero_after(pending.pop())
        out = []
        for w in tiles:
            a = r0 % w.shape[0]
            parts = [w[:a]] if a else []
            parts.append(w[a:a + 8] | z[:, :w.shape[1]])
            if a + 8 < w.shape[0]:
                parts.append(w[a + 8:])
            out.append(jnp.concatenate(parts, axis=0))
        return out

    def after(x, v):
        return pltpu.bitcast(pltpu.bitcast(x, u32) | zero_after(v[0:8, 0:LANES]), f32)

    def words(ref, *idx, rows=slice(None), lanes=slice(None)):
        if rows.start is not None:
            rows = slice(rows.start // 2, rows.stop // 2)
        return ref.bitcast(u32)[(*idx, rows, lanes)]

    def k_tiles(ref, rows=slice(None)):
        return [words(ref, k, rows=rows, lanes=slice(0, min(LANES, D - k * LANES))) for k in range(KT)]

    def transpose_into(dst, src, k, c0, c1):
        n = min(LANES, D - k * LANES)
        t = src[k * LANES:k * LANES + n, c0:c1].T
        dst[k, c0:c1, 0:n] = t
        if n == LANES:
            mark(t[c1 - c0 - ST:])

    mod_done = []

    def mod_tiles(js):
        acc = [None] * len(js)
        for r in range(D // ST):
            sc = sc_s[_rows(r), :]
            for k, j in enumerate(js):
                v = sc * wmod_s[_rows(r), _tile(j)].astype(f32)
                acc[k] = _add(_add(acc[k], v[0:8]), v[8:ST])
        for k, j in enumerate(js):
            col = j * LANES + lax.broadcasted_iota(jnp.int32, (1, LANES), 1)
            is_scale = ((col >= D) & (col < 2 * D)) | ((col >= 4 * D) & (col < 5 * D))
            r = jnp.sum(acc[k], axis=0, keepdims=True) + jnp.where(is_scale, 1.0, 0.0)
            t = jnp.broadcast_to(r, (LANES, LANES)).T
            mod_s[_tile(j), :] = t
            mod_done.append(j)
            mark(t[LANES - 8:])

    def mod_steps(c0, c1):
        return [functools.partial(mod_tiles, range(j, j + 1)) for j in range(pl.cdiv(c0, LANES), pl.cdiv(c1, LANES))]

    def mod(i, rs):
        assert (i * D + rs.start) // LANES in mod_done
        return mod_s[i * D + rs.start:i * D + rs.stop, :]

    def ln1_steps(i, hb=None, ht=None):
        st = {}

        def get(r, p):
            return x_s[_rows(r, 8), _tile(i * TPB + 2 * p, 2)].astype(f32)

        def mean_of(f):
            total = jnp.sum(functools.reduce(_add, map(f, range(D // 8))), axis=0, keepdims=True) * (1.0 / D)
            return jnp.broadcast_to(total, (8, 2 * LANES))

        def mean(p):
            st["m", p] = mean_of(lambda r: get(r, p))
            mark(st["m", p][:, _tile(0)])
            mark(st["m", p][:, _tile(1)])

        def scale(p):
            st["rstd", p] = lax.rsqrt(mean_of(lambda r: jnp.square(get(r, p) - st["m", p])) + EPS)
            mark(st["rstd", p][:, _tile(0)])
            mark(st["rstd", p][:, _tile(1)])

        def strip(r, p):
            xn = [(get(2 * r + e, p) - st["m", p]) * st["rstd", p] for e in range(2)]
            return [jnp.concatenate([v[:, _tile(t)] for v in xn], axis=0) * mod(1, _rows(r)) + mod(0, _rows(r))
                    for t in range(2)]

        def whole(p):
            for r in range(D // ST):
                for t, v in enumerate(strip(r, p)):
                    h_s[2 * p + t, _rows(r), :] = v.astype(bf16)

        def blocks(rs):
            for r in rs:
                quads = [strip(r + a * KH // ST, p) for a in range(2) for p in range(2)]
                for t in range(2):
                    for j, v in enumerate(_rhs_blocks(*[q[t] for q in quads])):
                        hb[j, t, _rows(r), :] = v.astype(bf16)
                        if j in (2, 3):
                            mark(v)
                    pace()

        def tail():
            for r in range(2 * KH // ST, D // ST):
                for p in range(2):
                    for t, v in enumerate(strip(r, p)):
                        ht[2 * p + t, _rows(r - 2 * KH // ST), :] = v.astype(bf16)
                        mark(v)
                pace()

        stats = [functools.partial(f, p) for f in (mean, scale) for p in range(2)]
        if hb is None:
            return stats, whole
        return stats + [functools.partial(blocks, range(r, r + 2)) for r in range(0, KH // ST, 2)] + [tail]

    def split_wqkv(p, k):
        for r in range(QH // ST):
            quads = [_unpack(words(wqkvT_s, k + b * KH // LANES, rows=_rows((2 * p + a) * QH // ST + r)))
                     for a in range(2) for b in range(2)]
            even, odd = [_lhs_blocks(*[q[e] for q in quads]) for e in range(2)]
            for n, j in enumerate((0, 1, 4, 5, 6)):
                w = _pack(even[j], odd[j])
                wa_s[p, n, k, _rows(r, 8), :] = w
                if n < 2:
                    mark(w)
            if r % 5 == 1:
                pace()

    def qkv_first(j, skip):
        tiles = [words(h_s, t, rows=slice(k * LANES, min((k + 1) * LANES, D))) for t in range(TPB) for k in range(KT)]
        for g in range(4 * skip, len(tiles), 4):
            run(1)
            tiles[g:g + 4] = anchor(tiles[g:g + 4], -8)
        rhs = [jnp.concatenate(tiles[t * KT:(t + 1) * KT], axis=0) for t in range(TPB)]
        y = _dot(_operand(k_tiles(wqkvT_s, _rows(j, QP))), _operand(rhs))
        for r in range(QP // ST):
            for t in range(TPB):
                v, rs = y[_rows(r), _tile(t)].astype(bf16), _rows(j * (QP // ST) + r)
                qkv0_s[1 + t, rs, :] = v
                if t == TPB - 1:
                    qkv_s[0, rs, :] = v

    def qkv_piece(i, p, busy):
        m = []
        for j in range(8):
            if j == 7:
                lhs = [words(wqkvT_s, KT - 1, rows=_rows(p, RH), lanes=slice(0, D - 2 * KH))]
                rhs = [words(ht1_s, t) for t in range(TPB)]
            else:
                lhs = [words(wqkvT_s, k + (j - 2) * KH // LANES, rows=_rows(2 * p + j - 2, QH)) if j in (2, 3)
                       else wa_s[p, j if j < 2 else j - 2, k] for k in range(KH // LANES)]
                rhs = [words(hb1_s, j, t) for t in range(TPB // 2)]
            for e in range(1 + (j == 7)):
                if busy(9 * p + j + e):
                    run(1)
                    lhs = anchor(lhs, e * QH // 2)
            m.append(_dot(_operand(lhs), _operand(rhs)))
        for r in range(QH // ST):
            for t in range(TPB // 2):
                tail = [m[7][_rows(r + a * QH // ST), _tile(b * TPB // 2 + t)] for a in range(2) for b in range(2)]
                for q, v in enumerate(_out_blocks([x[_rows(r), _tile(t)] for x in m[:7]], tail)):
                    a, tt = q // 2, q % 2 * (TPB // 2) + t
                    qkv_s[i * TPB + tt - (TPB - 1), _rows((2 * p + a) * QH // ST + r), :] = v.astype(bf16)
        return m

    def halo():
        for r in range(D // ST, 3 * D // ST):
            w = words(qkv0_s, 1, rows=_rows(r))
            qkv0_s.bitcast(u32)[0, _rows(r, 8), :] = jnp.broadcast_to(w[:, 0:1], (8, LANES))

    lane = lax.broadcasted_iota(jnp.int32, (8, LANES), 1)

    def shifted(cur, prev, w):
        s = DIL * w
        return cur if w == 0 else pltpu.roll(jnp.where(lane >= LANES - s, prev, cur), s, 1)

    def attn_steps(n, hg, first):
        qkv = (qkv0_s if first else qkv_s).bitcast(u32).at[pl.ds(n if first else n - TPB, 2)]
        acc = [None] * W

        def heads(ref, tile, part):
            start = part * RH + hg * 8 * (DH // 2)
            return ref.at[tile, pl.ds(start if isinstance(start, int) else pl.multiple_of(start, 8), 8 * (DH // 2))]

        def pair(p):
            return pl.ds(p, 8, stride=DH // 2), slice(None)

        def scores(ps, last):
            for p in ps:
                q0, q1 = _unpack(heads(qkv, 1, 0)[pair(p)])
                cur, prev = heads(qkv, 1, 1)[pair(p)], heads(qkv, 0, 1)[pair(p)]
                for w in range(W):
                    k0, k1 = _unpack(shifted(cur, prev, w))
                    acc[w] = _add(acc[w], q0 * k0 + q1 * k1)
            if last:
                lg = [a * (DH ** -0.5) for a in acc]
                if first:
                    lg = [lg[0]] + [jnp.where(n * LANES + lane >= DIL * w, lg[w], -1e9) for w in range(1, W)]
                m = functools.reduce(jnp.maximum, lg)
                e = [jnp.exp(v - m) for v in lg]
                inv = 1.0 / functools.reduce(_add, e)
                acc[:] = [v * inv for v in e]
            for a in acc:
                mark(a)

        def values(ps):
            for p in ps:
                cur, prev = heads(qkv, 1, 2)[pair(p)], heads(qkv, 0, 2)[pair(p)]
                o0 = o1 = None
                for w in range(W):
                    v0, v1 = _unpack(shifted(cur, prev, w))
                    o0, o1 = _add(o0, acc[w] * v0), _add(o1, acc[w] * v1)
                o = _pack(o0, o1)
                heads(o_s, n, 0)[pair(p)] = o
                mark(o)

        return [functools.partial(scores, range(0, 5), False), functools.partial(scores, range(5, 9), True),
                functools.partial(values, range(0, 5)), functools.partial(values, range(5, 9))]

    def attn_units(units, first=False):
        return [s for n, hg in units for s in attn_steps(n, hg, first)]

    def col_mean(strips):
        total = functools.reduce(_add, (v[_rows(e, 8)] for v in strips for e in range(2)))
        total = jnp.sum(total, axis=0, keepdims=True) * (1.0 / D)
        return jnp.broadcast_to(total, (8, LANES))

    def project(i):
        a = _dot(_operand(anchor(k_tiles(woT_s))), _operand([o_s[i * TPB + t] for t in range(TPB)]))
        for t in range(TPB):
            strips = []
            for r in range(D // ST):
                x1 = x_s[_rows(r), _tile(i * TPB + t)].astype(f32) + mod(2, _rows(r)) * a[_rows(r), _tile(t)]
                x1_s[i * TPB + t, _rows(r), :] = x1
                strips.append(x1)
            ms_s[t] = col_mean(strips)

    def ln2_steps(i):
        st = {}

        def twice(v):
            return jnp.concatenate([v, v], axis=0)

        def parity_rows(r, e, base=0):
            return pl.ds(base + r * ST + e, 8, stride=2)

        def x1_strip(t, r):
            return jnp.concatenate([x1_s[i * TPB + t, parity_rows(r, e), :] for e in range(2)], axis=0)

        def scale(ts, go):
            for t in ts:
                m = after(ms_s[t], go)
                st[t] = lax.rsqrt(col_mean(jnp.square(x1_strip(t, r) - twice(m)) for r in range(D // ST)) + EPS)

        def h2(t, r, m):
            assert all((k * D + r * ST) // LANES in mod_done for k in (3, 4))
            cb, sb = [jnp.concatenate([mod_s[parity_rows(r, e, k * D), :] for e in range(2)], axis=0) for k in (4, 3)]
            return (x1_strip(t, r) - twice(m)) * twice(st[t]) * cb + sb

        def transposed(strips):
            return pltpu.bitcast(jnp.concatenate([_pack(v[0:8], v[8:ST]) for v in strips], axis=0), bf16).T

        def blocks(t, kt, go):
            t2 = t + TPB // 2
            m1, m2 = after(ms_s[t], go), after(ms_s[t2], go)
            strips = [_lhs_blocks(h2(t, r, m1), h2(t, r + KH // ST, m1), h2(t2, r, m2), h2(t2, r + KH // ST, m2))
                      for r in range(kt * LANES // ST, (kt + 1) * LANES // ST)]
            for j in range(7):
                ha_s[j, kt, _tile(t), :] = transposed([s[j] for s in strips])

        def tail(go):
            for t in range(TPB):
                m = after(ms_s[t], go)
                blk = transposed([h2(t, r, m) for r in range(2 * KH // ST, D // ST)])
                for r in range(LANES // ST):
                    half, strip = divmod(t * LANES // ST + r, TH // ST)
                    hl_s[_rows(2 * strip + half), 0:D - 2 * KH] = blk[_rows(r)]

        half = TPB // 2
        return ([functools.partial(scale, (t, t + half)) for t in range(half)]
                + [functools.partial(blocks, t, kt) for t in range(half) for kt in range(KH // LANES)] + [tail])

    gate_and_up = ((wg_s, tg_s), (wu_s, tu_s))

    def quadrants(w_s, c, r, off):
        return [[w_s[pl.ds(r * ST + 8 * e + a * off, 8), _tile((2 * c + b) * NT, NT)].astype(f32) for e in range(2)]
                for a in range(2) for b in range(2)]

    def store_blocks(dst, halves, marked):
        for j, (lo, hi) in enumerate(halves):
            for t in range(NT):
                v = jnp.concatenate([lo[:, _tile(t)], hi[:, _tile(t)]], axis=0)
                dst(j, t, v.astype(bf16))
                if j in marked:
                    mark(v)
        pace()

    def split_gate_up(half, c):
        w_s, t_s = gate_and_up[half]

        def step(rs):
            for r in rs:
                def dst(j, t, v):
                    t_s[c, j, t, _rows(r), :] = v

                blocks = [_rhs_blocks(*q) for q in zip(*quadrants(w_s, c, r, KH))]
                store_blocks(dst, [(blocks[0][j], blocks[1][j]) for j in (0, 2, 3, 5, 6)], (3, 4))

        return [functools.partial(step, range(r, r + 4)) for r in range(0, KH // ST, 4)]

    def split_down(c):
        def step(rs):
            for r in rs:
                def dst(j, t, v):
                    sd_s[j, c * NT + t, _rows(r), :] = v

                store_blocks(dst, zip(*[_lhs_blocks(*q) for q in zip(*quadrants(wdT_s, c, r, RH))]), (1, 4))

        return [functools.partial(step, rs) for rs in (range(0, 5), range(5, 9), range(9, 14), range(14, 18))]

    def gate_up_products(half, c, points):
        w_s, t_s = gate_and_up[half]

        def rhs(j):
            if j == 1:
                return w_s[0:KH, _tile(2 * c * NT, NT)]
            if j == 4:
                return w_s[KH:2 * KH, _tile((2 * c + 1) * NT, NT)]
            if j == 7:
                return w_s[2 * KH:D, _tile(2 * c * NT, 2 * NT)]
            return _operand([words(t_s, c, (0, None, 1, 2, None, 3, 4)[j], k) for k in range(NT)])

        m = []
        for j in range(8):
            lhs = [words(ha_s, j, k) for k in range(KH // LANES)] if j < 7 else [words(hl_s, lanes=slice(0, D - 2 * KH))]
            for e in range(2):
                if 2 * j + e in points:
                    run(1)
                    lhs = anchor(lhs, e * lhs[0].shape[0] // 2)
            m.append(_dot(_operand(lhs), rhs(j)))
        return m

    def gated(c, g, u):
        for r in range(TH // ST):
            for t in range(NT):
                def blocks(m):
                    tail = [m[7][_rows(2 * r + a), _tile(b * NT + t)] for a in range(2) for b in range(2)]
                    return _out_blocks([x[_rows(r), _tile(t)] for x in m[:7]], tail)

                h11, h12, h21, h22 = [a * b for a, b in zip(blocks(g), blocks(u))]
                for j, v in enumerate(_rhs_blocks(h11, h21, h12, h22)):
                    hb_s[j, c * NT + t, _rows(r), :] = v.astype(bf16)

    def gate_up_first(c, carry):
        @pl.when(c == GC)
        def _():
            wait(*cp_b)

        units = [jnp.minimum(2 * c + e, TPB * HG - 1) for e in range(2)]
        orders = ("awawawawdd", "dwadwawawa")
        points = ((4, 5, 6, 7, 8, 9, 10, 11, 13, 15), (2, 3, 4, 6, 7, 8, 9, 10, 12, 13))
        m = []
        for half, u in enumerate(units):
            weights = split_gate_up(1, c) if half == 0 else split_gate_up(0, jnp.minimum(c + 1, NCH - 1))
            queue.extend(_ordered(orders[half], weights=weights, attention=attn_units([(TPB + u // HG, u % HG)]),
                                  down=split_down(c)[2 * half:2 * half + 2]))
            m.append(gate_up_products(half, c, points[half]))
            assert not queue
        gated(c, *m)
        pending.clear()
        return carry

    def gate_up(i, k, carry):
        n0 = jnp.minimum(i + 1, NB - 1) * TPB
        queue.extend(attn_units([(n0 + k, hg) for hg in range(HG)] + [(n0 + TPB - 1, k), (n0 + TPB - 1, HG - 1)]))
        points = ((6, 9, 11, 13), (6, 9, 10, 12))
        for e in range(GC):
            c = GC * k + e
            gated(c, *[gate_up_products(half, c, points[half]) for half in range(2)])
        assert not queue
        pending.clear()
        return carry

    def down(i):
        m = {}
        steps = ln2_steps(jnp.minimum(i + 1, NB - 1))
        queue.extend(mod_steps(5 * D, 6 * D))

        def product(j):
            tiles = [words(sd_s, j - 1, k) for k in range(FT)]
            for k in range(0 if m else 8, 16, 4):
                run(1 if m else 2)
                tiles[k:k + 4] = anchor(tiles[k:k + 4])
            m[j] = _dot_nt(_operand(tiles), _operand([words(hb_s, j - 1, k) for k in range(FT)]))
            for t in range(pl.cdiv(len(steps), max(6 - len(m), 1))):
                steps.pop(0)(m[j][:, _tile(t % (TH // LANES))])

        def out(a, b, block):
            n0 = i * TPB + b * (TPB // 2)
            for r in range(RH // ST):
                rs = _rows(a * RH // ST + r)
                x1 = jnp.concatenate([x1_s[n0 + k, rs, :] for k in range(TPB // 2)], axis=1)
                gb = jnp.concatenate([mod(5, rs)] * (TPB // 2), axis=1)
                out_s[rs, _tile(n0, TPB // 2)] = (x1 + gb * block(_rows(r))).astype(bf16)

        product(2)
        product(4)
        out(1, 0, lambda s: m[2][s] + m[4][s])
        product(1)
        product(5)
        product(7)
        out(0, 0, lambda s: m[7][s] - m[5][s] + m[4][s] + m[1][s])
        product(3)
        out(0, 1, lambda s: m[3][s] + m[5][s])
        out_copy(i, 0).start()
        out_copy(i, 1).start()
        product(6)
        out(1, 1, lambda s: m[6][s] + m[3][s] - m[2][s] + m[1][s])
        out_copy(i, 2).start()
        assert not steps

    z_s[...] = jnp.zeros_like(z_s)

    for cp in (cp_c, *cp_m0, cp_w[0], *cp_x0, *cp_w[1:], cp_x1, cp_x2, cp_wo, cp_m1, *cp_a, *cp_b):
        cp.start()
    wait(cp_c)
    cv = c_s[...].astype(f32)
    sc = (cv * jax.nn.sigmoid(cv)).astype(bf16).astype(f32)
    sc_s[...] = jnp.broadcast_to(sc, (LANES, D)).T
    stats, whole = ln1_steps(0)
    for cp, t0, t1 in zip(cp_m0, MOD_CUTS[:-1], MOD_CUTS[1:]):
        wait(cp)
        mod_tiles(range(t0, t1))
    wait(cp_w[0])
    for k in range(KT):
        transpose_into(wqkvT_s, wqkv_s, k, WQKV_CUTS[0], WQKV_CUTS[1])
    for p in range(2):
        wait(cp_x0[p])
        stats[p]()
        stats[p + 2]()
        whole(p)
    pending.clear()

    def transposes(c0, c1):
        return [functools.partial(transpose_into, wqkvT_s, wqkv_s, k, c0, c1) for k in range(KT)]

    def next_piece():
        for step in transposes(WQKV_CUTS[2], 6 * QP):
            step()

    splits = [functools.partial(split_wqkv, p, k) for p in range(NSP) for k in range(KH // LANES)]
    ready = WQKV_CUTS[2] // RH * (KH // LANES)
    arrivals = {
        1: ([cp_w[1]], transposes(*WQKV_CUTS[1:3])[::-1] + splits[:2] + [lambda: None] + splits[2:ready]),
        4: ([cp_w[2], cp_x1], _ordered("lnltltlstltstllslslslslll", next_columns=[next_piece], splits=splits[ready:],
                                       transposes=transposes(6 * QP, 3 * D), layernorm=ln1_steps(1, hb1_s, ht1_s))),
    }
    for j in range(NQP):
        if j in arrivals:
            wait(*arrivals[j][0])
            queue.extend(arrivals[j][1])
        qkv_first(j, 2 if j in arrivals else 0)
    halo()
    drain()
    wait(cp_x2)

    def middle(i, carry):
        units = [(i - 1, hg) for hg in range(HG)] + [(i + 1, hg) for hg in range(HG - 1)]
        queue.extend(_weave(attn_units(units, True), ln1_steps(i + 1, hbn_s, htn_s)))
        for p in range(NSP):
            qkv_piece(i, p, lambda a: a >= 4 and a % 5)
        drain()
        hb1_s[...] = hbn_s[...]
        ht1_s[...] = htn_s[...]
        return carry

    lax.fori_loop(1, NB - 1, middle, None)

    wait(cp_wo, cp_m1, *cp_a)
    vectors = mod_steps(2 * D, 5 * D)
    wo_steps = [functools.partial(transpose_into, woT_s, wo_s, k, 0, D) for k in range(KT)]
    queue.extend(_weave(attn_units([(n, HG - 1) for n in range(TPB // 2, TPB)], True), vectors[:KT] + wo_steps))
    steps = []
    for p, releases in enumerate(((), (), (), (3, 6), (1, 4, 6), (1, 2))):
        if p == NSP // 2:
            run()
            project(0)
            queue.extend(vectors[KT:] + split_gate_up(0, 0))
            steps = ln2_steps(0)
        m = qkv_piece(NB - 1, p, lambda a: a >= 4 and a % 3)
        for j in releases:
            steps.pop(0)(m[j])
    assert not steps
    drain()

    def block(i, carry):
        lax.fori_loop(0, jnp.where(i == 0, NCH, 0), gate_up_first, None)
        lax.fori_loop(0, jnp.where(i == 0, 0, NCH // GC), functools.partial(gate_up, i), None)

        @pl.when(i + 1 < NB)
        def _():
            project(i + 1)

        down(i)
        return carry

    lax.fori_loop(0, NB, block, None)
    for i in range(NB):
        wait(*[out_copy(i, q) for q in range(3)])


@jax.jit
def pallas_adaLN_cond__sliding_local_dilated__glu_gated_bilinear__prompt_kernel(
    A_x: jax.Array,
    A_wqkv: jax.Array,
    A_wo: jax.Array,
    B_x: jax.Array,
    B_w_gate: jax.Array,
    B_w_up: jax.Array,
    B_w_down: jax.Array,
    c: jax.Array,
    w_mod: jax.Array,
):
    del B_x
    vmem = pltpu.VMEM
    ln1_blocks = [vmem((7, TPB // 2, KH, LANES), bf16), vmem((TPB, D - 2 * KH, LANES), bf16)]
    in_hbm = pl.BlockSpec(memory_space=pl.ANY)
    outT = pl.pallas_call(
        _kernel,
        out_shape=jax.ShapeDtypeStruct((D, S), bf16),
        in_specs=[in_hbm] * 8,
        out_specs=in_hbm,
        scratch_shapes=[
            vmem((D, S), bf16), vmem((D, 3 * D), bf16), vmem((D, D), bf16),
            vmem((D, F), bf16), vmem((D, F), bf16), vmem((D, F), bf16),
            vmem((1, D), bf16), vmem((D, 6 * D), bf16),
            vmem((KT, 3 * D, LANES), bf16), vmem((KT, D, LANES), bf16),
            vmem((6 * D, LANES), f32), vmem((D, LANES), f32),
            vmem((NSP, 5, KH // LANES, QH // 2, LANES), u32),
            vmem((TPB, D, LANES), bf16), *ln1_blocks, *ln1_blocks,
            vmem((TPB + 1, 3 * D, LANES), bf16),
            vmem((NTILE - TPB + 1, 3 * D, LANES), bf16),
            vmem((NTILE, RH, LANES), u32), vmem((NTILE, D, LANES), f32),
            vmem((7, KH // LANES, TH, LANES), bf16), vmem((T, LANES), bf16),
            vmem((NCH, 5, NT, KH, LANES), bf16), vmem((NCH, 5, NT, KH, LANES), bf16),
            vmem((7, FT, RH, LANES), bf16), vmem((7, FT, TH, LANES), bf16),
            vmem((D, S), bf16),
            vmem((TPB, 8, LANES), f32), vmem((16, LANES), u32),
            pltpu.SemaphoreType.DMA((19,)), pltpu.SemaphoreType.DMA((3 * NB,)),
        ],
        compiler_params=pltpu.CompilerParams(vmem_limit_bytes=120 * 2**20),
    )(A_x.reshape(S, D).T, A_wqkv, A_wo, B_w_gate, B_w_up, B_w_down.T, c, w_mod)
    return outT.T.reshape(1, S, D)
```

```python
import functools

import jax
import jax.numpy as jnp
from jax import lax
from jax.experimental import pallas as pl
from jax.experimental.pallas import tpu as pltpu

S, D, F = 2048, 576, 4608
H, DH, W, DIL = 32, 18, 8, 2
EPS = 1e-5
f32, bf16, u32 = jnp.float32, jnp.bfloat16, jnp.uint32

LANES = 128
ST = 16
NTILE = S // LANES
KT = pl.cdiv(D, LANES)
RH = D // 2
HG = H // 8

T = 512
TH = T // 2
TPB = T // LANES
NB = S // T
KH = 256
NC = 256
NT = NC // LANES
NCH = F // (2 * NC)
FT = F // 2 // LANES
GC = 3
QP = 192
NQP = 3 * D // QP
QH = RH // 2
NSP = 3 * D // RH

MOD_CUTS = (0, 3, 6, 9)
WQKV_CUTS = (0, 384, 1024, 3 * D)


def _unpack(w):
    return [pltpu.unpack_elementwise(w, index=e, packed_dtype=bf16, unpacked_dtype=f32) for e in range(2)]


def _pack(even, odd):
    return pltpu.pack_elementwise([even, odd], packed_dtype=bf16).astype(u32)


def _operand(tiles):
    return jnp.concatenate([pltpu.bitcast(w, bf16) for w in tiles], axis=1)


def _dot(a, b):
    return jnp.dot(a, b, preferred_element_type=f32)


def _dot_nt(a, b):
    return lax.dot_general(a, b, (((1,), (1,)), ((), ())), preferred_element_type=f32)


def _lhs_blocks(a11, a12, a21, a22):
    return a11 + a22, a21 + a22, a11, a22, a11 + a12, a21 - a11, a12 - a22


def _rhs_blocks(b11, b12, b21, b22):
    return b11 + b22, b11, b12 - b22, b21 - b11, b22, b11 + b12, b21 + b22


def _out_blocks(m, tail):
    m1, m2, m3, m4, m5, m6, m7 = m
    l11, l12, l21, l22 = tail
    return l11 + m7 - m5 + m4 + m1, l12 + m5 + m3, l21 + m4 + m2, l22 + m6 + m3 - m2 + m1


def _add(a, b):
    return b if a is None else a + b


def _rows(r, n=ST):
    return slice(r * n, (r + 1) * n)


def _tile(n, width=1):
    if isinstance(n, int):
        return slice(n * LANES, (n + width) * LANES)
    return pl.ds(pl.multiple_of(n * LANES, LANES), width * LANES)


def _weave(a, b):
    keyed = [((k + 0.5) / len(x), x[k]) for x in (a, b) for k in range(len(x))]
    return [item for _, item in sorted(keyed, key=lambda p: p[0])]


def _ordered(order, **lists):
    lists = {name[0]: list(v) for name, v in lists.items()}
    merged = [lists[ch].pop(0) for ch in order]
    assert not any(lists.values())
    return merged


def _kernel(xT_hbm, wqkv_hbm, wo_hbm, wg_hbm, wu_hbm, wdT_hbm, c_hbm, wmod_hbm, out_hbm,
            x_s, wqkv_s, wo_s, wg_s, wu_s, wdT_s, c_s, wmod_s,
            wqkvT_s, woT_s, mod_s, sc_s, wa_s, wb_s, h_s, hb1_s, ht1_s, hbn_s, htn_s, qkv0_s, qkv_s, o_s,
            x1_s, ha_s, hl_s, tg_s, tu_s, sd_s, hb_s, out_s, ms_s, z_s, sems, out_sems):
    sem_ids = iter(range(sems.shape[0]))

    def copy(src, dst):
        return pltpu.make_async_copy(src, dst, sems.at[next(sem_ids)])

    def cols(src, dst, c0, c1):
        return copy(src.at[:, pl.ds(c0, c1 - c0)], dst.at[:, pl.ds(c0, c1 - c0)])

    cp_c = copy(c_hbm, c_s)
    cp_m0 = [cols(wmod_hbm, wmod_s, t0 * LANES, t1 * LANES) for t0, t1 in zip(MOD_CUTS[:-1], MOD_CUTS[1:])]
    cp_m1 = cols(wmod_hbm, wmod_s, 2 * D, 6 * D)
    cp_w = [cols(wqkv_hbm, wqkv_s, c0, c1) for c0, c1 in zip(WQKV_CUTS[:-1], WQKV_CUTS[1:])]
    cp_wo = copy(wo_hbm, wo_s)
    cp_x0 = [cols(xT_hbm, x_s, p * TH, (p + 1) * TH) for p in range(2)]
    cp_x1 = cols(xT_hbm, x_s, T, 2 * T)
    cp_x2 = cols(xT_hbm, x_s, 2 * T, S)
    ffn = ((wg_hbm, wg_s, (GC + 1) * 2 * NC), (wu_hbm, wu_s, (GC + 1) * 2 * NC), (wdT_hbm, wdT_s, GC * 2 * NC))
    cp_a = [cols(src, dst, 0, n) for src, dst, n in ffn]
    cp_b = [cols(src, dst, n, F) for src, dst, n in ffn]

    def out_copy(i, q):
        rows = (slice(0, D), slice(0, RH), slice(RH, D))[q]
        idx = (rows, _tile(i * TPB + (q > 0) * TPB // 2, TPB // 2))
        return pltpu.make_async_copy(out_s.at[idx], out_hbm.at[idx], out_sems.at[3 * i + q])

    def wait(*cps):
        for cp in cps:
            cp.wait()

    queue = []
    pending = []

    def mark(v):
        if v.dtype != f32:
            v = pltpu.bitcast(v, f32)
        for r in range(v.shape[0] // 8):
            q = v[_rows(r, 8)]
            pending[:] = [q + pending[0]] if pending else [q]

    def pace():
        pending[:] = [pltpu.roll(pending[0], 1, 1)]

    def run(n=None):
        for _ in range(len(queue) if n is None else min(n, len(queue))):
            queue.pop(0)()

    def drain():
        run()
        pending.clear()

    def zero_after(v):
        return z_s[pl.ds(1, 8), :] & pltpu.bitcast(v, u32)

    def anchor(tiles, r0=0):
        if not pending:
            return tiles
        z = zero_after(pending.pop())
        out = []
        for w in tiles:
            a = r0 % w.shape[0]
            parts = [w[:a]] if a else []
            parts.append(w[a:a + 8] | z[:, :w.shape[1]])
            if a + 8 < w.shape[0]:
                parts.append(w[a + 8:])
            out.append(jnp.concatenate(parts, axis=0))
        return out

    def after(x, v):
        return pltpu.bitcast(pltpu.bitcast(x, u32) | zero_after(v[0:8, 0:LANES]), f32)

    def words(ref, *idx, rows=slice(None), lanes=slice(None)):
        if rows.start is not None:
            rows = slice(rows.start // 2, rows.stop // 2)
        return ref.bitcast(u32)[(*idx, rows, lanes)]

    def k_tiles(ref, rows=slice(None)):
        return [words(ref, k, rows=rows, lanes=slice(0, min(LANES, D - k * LANES))) for k in range(KT)]

    def transpose_into(dst, src, k, c0, c1):
        n = min(LANES, D - k * LANES)
        t = src[k * LANES:k * LANES + n, c0:c1].T
        dst[k, c0:c1, 0:n] = t
        if n == LANES:
            mark(t[c1 - c0 - ST:])

    mod_done = []

    def mod_tiles(js):
        acc = [None] * len(js)
        for r in range(D // ST):
            sc = sc_s[_rows(r), :]
            for k, j in enumerate(js):
                v = sc * wmod_s[_rows(r), _tile(j)].astype(f32)
                acc[k] = _add(_add(acc[k], v[0:8]), v[8:ST])
        for k, j in enumerate(js):
            col = j * LANES + lax.broadcasted_iota(jnp.int32, (1, LANES), 1)
            is_scale = ((col >= D) & (col < 2 * D)) | ((col >= 4 * D) & (col < 5 * D))
            r = jnp.sum(acc[k], axis=0, keepdims=True) + jnp.where(is_scale, 1.0, 0.0)
            t = jnp.broadcast_to(r, (LANES, LANES)).T
            mod_s[_tile(j), :] = t
            mod_done.append(j)
            mark(t[LANES - 8:])

    def mod_steps(c0, c1):
        return [functools.partial(mod_tiles, range(j, j + 1)) for j in range(pl.cdiv(c0, LANES), pl.cdiv(c1, LANES))]

    def mod(i, rs):
        assert (i * D + rs.start) // LANES in mod_done
        return mod_s[i * D + rs.start:i * D + rs.stop, :]

    def ln1_steps(i, hb=None, ht=None):
        st = {}

        def get(r, p):
            return x_s[_rows(r, 8), _tile(i * TPB + 2 * p, 2)].astype(f32)

        def mean_of(f):
            total = jnp.sum(functools.reduce(_add, map(f, range(D // 8))), axis=0, keepdims=True) * (1.0 / D)
            return jnp.broadcast_to(total, (8, 2 * LANES))

        def mean(p):
            st["m", p] = mean_of(lambda r: get(r, p))
            mark(st["m", p][:, _tile(0)])
            mark(st["m", p][:, _tile(1)])

        def scale(p):
            st["rstd", p] = lax.rsqrt(mean_of(lambda r: jnp.square(get(r, p) - st["m", p])) + EPS)
            mark(st["rstd", p][:, _tile(0)])
            mark(st["rstd", p][:, _tile(1)])

        def strip(r, p):
            xn = [(get(2 * r + e, p) - st["m", p]) * st["rstd", p] for e in range(2)]
            return [jnp.concatenate([v[:, _tile(t)] for v in xn], axis=0) * mod(1, _rows(r)) + mod(0, _rows(r))
                    for t in range(2)]

        def whole(p):
            for r in range(D // ST):
                for t, v in enumerate(strip(r, p)):
                    h_s[2 * p + t, _rows(r), :] = v.astype(bf16)

        def blocks(rs):
            for r in rs:
                quads = [strip(r + a * KH // ST, p) for a in range(2) for p in range(2)]
                for t in range(2):
                    for j, v in enumerate(_rhs_blocks(*[q[t] for q in quads])):
                        hb[j, t, _rows(r), :] = v.astype(bf16)
                        if j in (2, 3):
                            mark(v)
                    pace()

        def tail():
            for r in range(2 * KH // ST, D // ST):
                for p in range(2):
                    for t, v in enumerate(strip(r, p)):
                        ht[2 * p + t, _rows(r - 2 * KH // ST), :] = v.astype(bf16)
                        mark(v)
                pace()

        stats = [functools.partial(f, p) for f in (mean, scale) for p in range(2)]
        if hb is None:
            return stats, whole
        return stats + [functools.partial(blocks, range(r, r + 2)) for r in range(0, KH // ST, 2)] + [tail]

    def split_rows(src, dst, k, row0, half, rs):
        for r in rs:
            quads = [_unpack(words(src, k + b * KH // LANES, rows=_rows((row0 + a * half) // ST + r)))
                     for a in range(2) for b in range(2)]
            even, odd = [_lhs_blocks(*[q[e] for q in quads]) for e in range(2)]
            for n, j in enumerate((0, 1, 4, 5, 6)):
                w = _pack(even[j], odd[j])
                dst[n, k, _rows(r, 8), :] = w
                if n < 2:
                    mark(w)
            if r % 5 == 1:
                pace()

    def lhs_block(src, blocks, j, row0, half):
        if j == 7:
            return [words(src, KT - 1, rows=slice(row0, row0 + 2 * half), lanes=slice(0, D - 2 * KH))]
        if j in (2, 3):
            rows = slice(row0 + (j - 2) * half, row0 + (j - 1) * half)
            return [words(src, k + (j - 2) * KH // LANES, rows=rows) for k in range(KH // LANES)]
        return [blocks[j if j < 2 else j - 2, k] for k in range(KH // LANES)]

    def qkv_first(j, skip):
        tiles = [words(h_s, t, rows=slice(k * LANES, min((k + 1) * LANES, D))) for t in range(TPB) for k in range(KT)]
        for g in range(4 * skip, len(tiles), 4):
            run(1)
            tiles[g:g + 4] = anchor(tiles[g:g + 4], -8)
        rhs = [jnp.concatenate(tiles[t * KT:(t + 1) * KT], axis=0) for t in range(TPB)]
        y = _dot(_operand(k_tiles(wqkvT_s, _rows(j, QP))), _operand(rhs))
        for r in range(QP // ST):
            for t in range(TPB):
                v, rs = y[_rows(r), _tile(t)].astype(bf16), _rows(j * (QP // ST) + r)
                qkv0_s[1 + t, rs, :] = v
                if t == TPB - 1:
                    qkv_s[0, rs, :] = v

    def qkv_piece(i, p, busy):
        m = []
        for j in range(8):
            lhs = lhs_block(wqkvT_s, wa_s.at[p], j, p * RH, QH)
            rhs = [words(ht1_s, t) for t in range(TPB)] if j == 7 else [words(hb1_s, j, t) for t in range(TPB // 2)]
            for e in range(1 + (j == 7)):
                if busy(9 * p + j + e):
                    run(1)
                    lhs = anchor(lhs, e * QH // 2)
            m.append(_dot(_operand(lhs), _operand(rhs)))
        for r in range(QH // ST):
            for t in range(TPB // 2):
                tail = [m[7][_rows(r + a * QH // ST), _tile(b * TPB // 2 + t)] for a in range(2) for b in range(2)]
                for q, v in enumerate(_out_blocks([x[_rows(r), _tile(t)] for x in m[:7]], tail)):
                    a, tt = q // 2, q % 2 * (TPB // 2) + t
                    qkv_s[i * TPB + tt - (TPB - 1), _rows((2 * p + a) * QH // ST + r), :] = v.astype(bf16)
        return m

    def halo():
        for r in range(D // ST, 3 * D // ST):
            w = words(qkv0_s, 1, rows=_rows(r))
            qkv0_s.bitcast(u32)[0, _rows(r, 8), :] = jnp.broadcast_to(w[:, 0:1], (8, LANES))

    lane = lax.broadcasted_iota(jnp.int32, (8, LANES), 1)

    def shifted(cur, prev, w):
        s = DIL * w
        return cur if w == 0 else pltpu.roll(jnp.where(lane >= LANES - s, prev, cur), s, 1)

    def attn_steps(n, hg, first):
        qkv = (qkv0_s if first else qkv_s).bitcast(u32).at[pl.ds(n if first else n - TPB, 2)]
        acc = [None] * W

        def heads(ref, tile, part):
            start = part * RH + hg * 8 * (DH // 2)
            return ref.at[tile, pl.ds(start if isinstance(start, int) else pl.multiple_of(start, 8), 8 * (DH // 2))]

        def pair(p):
            return pl.ds(p, 8, stride=DH // 2), slice(None)

        def scores(ps, last):
            for p in ps:
                q0, q1 = _unpack(heads(qkv, 1, 0)[pair(p)])
                cur, prev = heads(qkv, 1, 1)[pair(p)], heads(qkv, 0, 1)[pair(p)]
                for w in range(W):
                    k0, k1 = _unpack(shifted(cur, prev, w))
                    acc[w] = _add(acc[w], q0 * k0 + q1 * k1)
            if last:
                lg = [a * (DH ** -0.5) for a in acc]
                if first:
                    lg = [lg[0]] + [jnp.where(n * LANES + lane >= DIL * w, lg[w], -1e9) for w in range(1, W)]
                m = functools.reduce(jnp.maximum, lg)
                e = [jnp.exp(v - m) for v in lg]
                inv = 1.0 / functools.reduce(_add, e)
                acc[:] = [v * inv for v in e]
            for a in acc:
                mark(a)

        def values(ps):
            for p in ps:
                cur, prev = heads(qkv, 1, 2)[pair(p)], heads(qkv, 0, 2)[pair(p)]
                o0 = o1 = None
                for w in range(W):
                    v0, v1 = _unpack(shifted(cur, prev, w))
                    o0, o1 = _add(o0, acc[w] * v0), _add(o1, acc[w] * v1)
                o = _pack(o0, o1)
                heads(o_s, n, 0)[pair(p)] = o
                mark(o)

        return [functools.partial(scores, range(0, 5), False), functools.partial(scores, range(5, 9), True),
                functools.partial(values, range(0, 5)), functools.partial(values, range(5, 9))]

    def attn_units(units, first=False):
        return [s for n, hg in units for s in attn_steps(n, hg, first)]

    def col_mean(strips):
        total = functools.reduce(_add, (v[_rows(e, 8)] for v in strips for e in range(2)))
        total = jnp.sum(total, axis=0, keepdims=True) * (1.0 / D)
        return jnp.broadcast_to(total, (8, LANES))

    def project(i):
        half = TPB // 2

        def rhs(j):
            if j == 7:
                return [o_s[i * TPB + t, KH:RH, :] for t in range(TPB)]
            if j in (1, 4):
                return [o_s[i * TPB + (j // 4) * half + t, _rows(j // 4, KH // 2), :] for t in range(half)]
            return [jnp.concatenate([s[j] for s in sums[t]], axis=0) for t in range(half)]

        def summed(t, r):
            quads = [_unpack(o_s[i * TPB + b * half + t, _rows(a * KH // ST + r, 8), :]) for a in range(2) for b in range(2)]
            return [_pack(*v) for v in zip(*[_rhs_blocks(*[q[e] for q in quads]) for e in range(2)])]

        sums = [[summed(t, r) for r in range(KH // ST)] for t in range(half)]
        m = [None] * 8
        for j in (1, 4, 7, 2, 3, 0, 5, 6):
            m[j] = _dot(_operand(anchor(lhs_block(woT_s, wb_s, j, 0, RH))), _operand(rhs(j)))
        strips = [[] for _ in range(TPB)]
        for r in range(RH // ST):
            for t in range(half):
                m1, m2, m3, m4, m5, m6, m7 = [x[_rows(r), _tile(t)] for x in m[:7]]
                for q, v in enumerate((m7 - m5 + m4 + m1, m3 + m5, m4 + m2, m6 + m3 - m2 + m1)):
                    rs, tt = _rows(q // 2 * RH // ST + r), q % 2 * half + t
                    x1 = x_s[rs, _tile(i * TPB + tt)].astype(f32) + mod(2, rs) * (v + m[7][rs, _tile(tt)])
                    x1_s[i * TPB + tt, rs, :] = x1
                    strips[tt].append(x1)
        for t in range(TPB):
            ms_s[t] = col_mean(strips[t])

    def ln2_steps(i):
        st = {}

        def twice(v):
            return jnp.concatenate([v, v], axis=0)

        def parity_rows(r, e, base=0):
            return pl.ds(base + r * ST + e, 8, stride=2)

        def x1_strip(t, r):
            return jnp.concatenate([x1_s[i * TPB + t, parity_rows(r, e), :] for e in range(2)], axis=0)

        def scale(ts, go):
            for t in ts:
                m = after(ms_s[t], go)
                st[t] = lax.rsqrt(col_mean(jnp.square(x1_strip(t, r) - twice(m)) for r in range(D // ST)) + EPS)

        def h2(t, r, m):
            assert all((k * D + r * ST) // LANES in mod_done for k in (3, 4))
            cb, sb = [jnp.concatenate([mod_s[parity_rows(r, e, k * D), :] for e in range(2)], axis=0) for k in (4, 3)]
            return (x1_strip(t, r) - twice(m)) * twice(st[t]) * cb + sb

        def transposed(strips):
            return pltpu.bitcast(jnp.concatenate([_pack(v[0:8], v[8:ST]) for v in strips], axis=0), bf16).T

        def blocks(t, kt, go):
            t2 = t + TPB // 2
            m1, m2 = after(ms_s[t], go), after(ms_s[t2], go)
            strips = [_lhs_blocks(h2(t, r, m1), h2(t, r + KH // ST, m1), h2(t2, r, m2), h2(t2, r + KH // ST, m2))
                      for r in range(kt * LANES // ST, (kt + 1) * LANES // ST)]
            for j in range(7):
                ha_s[j, kt, _tile(t), :] = transposed([s[j] for s in strips])

        def tail(go):
            for t in range(TPB):
                m = after(ms_s[t], go)
                blk = transposed([h2(t, r, m) for r in range(2 * KH // ST, D // ST)])
                for r in range(LANES // ST):
                    half, strip = divmod(t * LANES // ST + r, TH // ST)
                    hl_s[_rows(2 * strip + half), 0:D - 2 * KH] = blk[_rows(r)]

        half = TPB // 2
        return ([functools.partial(scale, (t, t + half)) for t in range(half)]
                + [functools.partial(blocks, t, kt) for t in range(half) for kt in range(KH // LANES)] + [tail])

    gate_and_up = ((wg_s, tg_s), (wu_s, tu_s))

    def quadrants(w_s, c, r, off):
        return [[w_s[pl.ds(r * ST + 8 * e + a * off, 8), _tile((2 * c + b) * NT, NT)].astype(f32) for e in range(2)]
                for a in range(2) for b in range(2)]

    def store_blocks(dst, halves, marked):
        for j, (lo, hi) in enumerate(halves):
            for t in range(NT):
                v = jnp.concatenate([lo[:, _tile(t)], hi[:, _tile(t)]], axis=0)
                dst(j, t, v.astype(bf16))
                if j in marked:
                    mark(v)
        pace()

    def split_gate_up(half, c):
        w_s, t_s = gate_and_up[half]

        def step(rs):
            for r in rs:
                def dst(j, t, v):
                    t_s[c, j, t, _rows(r), :] = v

                blocks = [_rhs_blocks(*q) for q in zip(*quadrants(w_s, c, r, KH))]
                store_blocks(dst, [(blocks[0][j], blocks[1][j]) for j in (0, 2, 3, 5, 6)], (3, 4))

        return [functools.partial(step, range(r, r + 4)) for r in range(0, KH // ST, 4)]

    def split_down(c):
        def step(rs):
            for r in rs:
                def dst(j, t, v):
                    sd_s[j, c * NT + t, _rows(r), :] = v

                store_blocks(dst, zip(*[_lhs_blocks(*q) for q in zip(*quadrants(wdT_s, c, r, RH))]), (1, 4))

        return [functools.partial(step, rs) for rs in (range(0, 5), range(5, 9), range(9, 14), range(14, 18))]

    def gate_up_products(half, c, points):
        w_s, t_s = gate_and_up[half]

        def rhs(j):
            if j == 1:
                return w_s[0:KH, _tile(2 * c * NT, NT)]
            if j == 4:
                return w_s[KH:2 * KH, _tile((2 * c + 1) * NT, NT)]
            if j == 7:
                return w_s[2 * KH:D, _tile(2 * c * NT, 2 * NT)]
            return _operand([words(t_s, c, (0, None, 1, 2, None, 3, 4)[j], k) for k in range(NT)])

        m = []
        for j in range(8):
            lhs = [words(ha_s, j, k) for k in range(KH // LANES)] if j < 7 else [words(hl_s, lanes=slice(0, D - 2 * KH))]
            for e in range(2):
                if 2 * j + e in points:
                    run(1)
                    lhs = anchor(lhs, e * lhs[0].shape[0] // 2)
            m.append(_dot(_operand(lhs), rhs(j)))
        return m

    def gated(c, g, u):
        for r in range(TH // ST):
            for t in range(NT):
                def blocks(m):
                    tail = [m[7][_rows(2 * r + a), _tile(b * NT + t)] for a in range(2) for b in range(2)]
                    return _out_blocks([x[_rows(r), _tile(t)] for x in m[:7]], tail)

                h11, h12, h21, h22 = [a * b for a, b in zip(blocks(g), blocks(u))]
                for j, v in enumerate(_rhs_blocks(h11, h21, h12, h22)):
                    hb_s[j, c * NT + t, _rows(r), :] = v.astype(bf16)

    def gate_up_first(c, carry):
        @pl.when(c == GC)
        def _():
            wait(*cp_b)

        units = [jnp.minimum(2 * c + e, TPB * HG - 1) for e in range(2)]
        orders = ("awawawawdd", "dwadwawawa")
        points = ((4, 5, 6, 7, 8, 9, 10, 11, 13, 15), (2, 3, 4, 6, 7, 8, 9, 10, 12, 13))
        m = []
        for half, u in enumerate(units):
            weights = split_gate_up(1, c) if half == 0 else split_gate_up(0, jnp.minimum(c + 1, NCH - 1))
            queue.extend(_ordered(orders[half], weights=weights, attention=attn_units([(TPB + u // HG, u % HG)]),
                                  down=split_down(c)[2 * half:2 * half + 2]))
            m.append(gate_up_products(half, c, points[half]))
            assert not queue
        gated(c, *m)
        pending.clear()
        return carry

    def gate_up(i, k, carry):
        n0 = jnp.minimum(i + 1, NB - 1) * TPB
        queue.extend(attn_units([(n0 + k, hg) for hg in range(HG)] + [(n0 + TPB - 1, k), (n0 + TPB - 1, HG - 1)]))
        points = ((6, 9, 11, 13), (6, 9, 10, 12))
        for e in range(GC):
            c = GC * k + e
            gated(c, *[gate_up_products(half, c, points[half]) for half in range(2)])
        assert not queue
        pending.clear()
        return carry

    def down(i):
        m = {}
        steps = ln2_steps(jnp.minimum(i + 1, NB - 1))
        queue.extend(mod_steps(5 * D, 6 * D))

        def product(j):
            tiles = [words(sd_s, j - 1, k) for k in range(FT)]
            for k in range(0 if m else 8, 16, 4):
                run(1 if m else 2)
                tiles[k:k + 4] = anchor(tiles[k:k + 4])
            m[j] = _dot_nt(_operand(tiles), _operand([words(hb_s, j - 1, k) for k in range(FT)]))
            for t in range(pl.cdiv(len(steps), max(6 - len(m), 1))):
                steps.pop(0)(m[j][:, _tile(t % (TH // LANES))])

        def out(a, b, block):
            n0 = i * TPB + b * (TPB // 2)
            for r in range(RH // ST):
                rs = _rows(a * RH // ST + r)
                x1 = jnp.concatenate([x1_s[n0 + k, rs, :] for k in range(TPB // 2)], axis=1)
                gb = jnp.concatenate([mod(5, rs)] * (TPB // 2), axis=1)
                out_s[rs, _tile(n0, TPB // 2)] = (x1 + gb * block(_rows(r))).astype(bf16)

        product(2)
        product(4)
        out(1, 0, lambda s: m[2][s] + m[4][s])
        product(1)
        product(5)
        product(7)
        out(0, 0, lambda s: m[7][s] - m[5][s] + m[4][s] + m[1][s])
        product(3)
        out(0, 1, lambda s: m[3][s] + m[5][s])
        out_copy(i, 0).start()
        out_copy(i, 1).start()
        product(6)
        out(1, 1, lambda s: m[6][s] + m[3][s] - m[2][s] + m[1][s])
        out_copy(i, 2).start()
        assert not steps

    z_s[...] = jnp.zeros_like(z_s)

    for cp in (cp_c, *cp_m0, cp_w[0], *cp_x0, *cp_w[1:], cp_x1, cp_x2, cp_wo, cp_m1, *cp_a, *cp_b):
        cp.start()
    wait(cp_c)
    cv = c_s[...].astype(f32)
    sc = (cv * jax.nn.sigmoid(cv)).astype(bf16).astype(f32)
    sc_s[...] = jnp.broadcast_to(sc, (LANES, D)).T
    stats, whole = ln1_steps(0)
    for cp, t0, t1 in zip(cp_m0, MOD_CUTS[:-1], MOD_CUTS[1:]):
        wait(cp)
        mod_tiles(range(t0, t1))
    wait(cp_w[0])
    for k in range(KT):
        transpose_into(wqkvT_s, wqkv_s, k, WQKV_CUTS[0], WQKV_CUTS[1])
    for p in range(2):
        wait(cp_x0[p])
        stats[p]()
        stats[p + 2]()
        whole(p)
    pending.clear()

    def transposes(c0, c1):
        return [functools.partial(transpose_into, wqkvT_s, wqkv_s, k, c0, c1) for k in range(KT)]

    def next_piece():
        for step in transposes(WQKV_CUTS[2], 6 * QP):
            step()

    splits = [functools.partial(split_rows, wqkvT_s, wa_s.at[p], k, p * RH, QH, range(QH // ST))
              for p in range(NSP) for k in range(KH // LANES)]
    ready = WQKV_CUTS[2] // RH * (KH // LANES)
    arrivals = {
        1: ([cp_w[1]], transposes(*WQKV_CUTS[1:3])[::-1] + splits[:2] + [lambda: None] + splits[2:ready]),
        4: ([cp_w[2], cp_x1], _ordered("lnltltlstltstllslslslslll", next_columns=[next_piece], splits=splits[ready:],
                                       transposes=transposes(6 * QP, 3 * D), layernorm=ln1_steps(1, hb1_s, ht1_s))),
    }
    for j in range(NQP):
        if j in arrivals:
            wait(*arrivals[j][0])
            queue.extend(arrivals[j][1])
        qkv_first(j, 2 if j in arrivals else 0)
    halo()
    drain()
    wait(cp_x2)

    def middle(i, carry):
        units = [(i - 1, hg) for hg in range(HG)] + [(i + 1, hg) for hg in range(HG - 1)]
        queue.extend(_weave(attn_units(units, True), ln1_steps(i + 1, hbn_s, htn_s)))
        for p in range(NSP):
            qkv_piece(i, p, lambda a: a >= 4 and a % 5)
        drain()
        hb1_s[...] = hbn_s[...]
        ht1_s[...] = htn_s[...]
        return carry

    lax.fori_loop(1, NB - 1, middle, None)

    wait(cp_wo, cp_m1, *cp_a)
    vectors = mod_steps(2 * D, 5 * D)
    wo_steps = [functools.partial(transpose_into, woT_s, wo_s, k, 0, D) for k in range(KT)]
    wo_splits = [functools.partial(split_rows, woT_s, wb_s, k, 0, RH, range(r, r + QH // ST))
                 for k in range(KH // LANES) for r in (0, QH // ST)]
    queue.extend(_weave(attn_units([(n, HG - 1) for n in range(TPB // 2, TPB)], True),
                        _ordered("vwvwvwvwvwssss", vectors=vectors[:KT], wo=wo_steps, splits=wo_splits)))
    steps = []
    for p, releases in enumerate(((), (), (), (3, 6), (1, 4, 6), (1, 2))):
        if p == NSP // 2:
            run()
            project(0)
            queue.extend(vectors[KT:] + split_gate_up(0, 0))
            steps = ln2_steps(0)
        m = qkv_piece(NB - 1, p, lambda a: a >= 4 and a % 3)
        for j in releases:
            steps.pop(0)(m[j])
    assert not steps
    drain()

    def block(i, carry):
        lax.fori_loop(0, jnp.where(i == 0, NCH, 0), gate_up_first, None)
        lax.fori_loop(0, jnp.where(i == 0, 0, NCH // GC), functools.partial(gate_up, i), None)

        @pl.when(i + 1 < NB)
        def _():
            project(i + 1)

        down(i)
        return carry

    lax.fori_loop(0, NB, block, None)
    for i in range(NB):
        wait(*[out_copy(i, q) for q in range(3)])


@jax.jit
def pallas_adaLN_cond__sliding_local_dilated__glu_gated_bilinear__prompt_kernel(
    A_x: jax.Array,
    A_wqkv: jax.Array,
    A_wo: jax.Array,
    B_x: jax.Array,
    B_w_gate: jax.Array,
    B_w_up: jax.Array,
    B_w_down: jax.Array,
    c: jax.Array,
    w_mod: jax.Array,
):
    del B_x
    vmem = pltpu.VMEM
    ln1_blocks = [vmem((7, TPB // 2, KH, LANES), bf16), vmem((TPB, D - 2 * KH, LANES), bf16)]
    in_hbm = pl.BlockSpec(memory_space=pl.ANY)
    outT = pl.pallas_call(
        _kernel,
        out_shape=jax.ShapeDtypeStruct((D, S), bf16),
        in_specs=[in_hbm] * 8,
        out_specs=in_hbm,
        scratch_shapes=[
            vmem((D, S), bf16), vmem((D, 3 * D), bf16), vmem((D, D), bf16),
            vmem((D, F), bf16), vmem((D, F), bf16), vmem((D, F), bf16),
            vmem((1, D), bf16), vmem((D, 6 * D), bf16),
            vmem((KT, 3 * D, LANES), bf16), vmem((KT, D, LANES), bf16),
            vmem((6 * D, LANES), f32), vmem((D, LANES), f32),
            vmem((NSP, 5, KH // LANES, QH // 2, LANES), u32),
            vmem((5, KH // LANES, RH // 2, LANES), u32),
            vmem((TPB, D, LANES), bf16), *ln1_blocks, *ln1_blocks,
            vmem((TPB + 1, 3 * D, LANES), bf16),
            vmem((NTILE - TPB + 1, 3 * D, LANES), bf16),
            vmem((NTILE, RH, LANES), u32), vmem((NTILE, D, LANES), f32),
            vmem((7, KH // LANES, TH, LANES), bf16), vmem((T, LANES), bf16),
            vmem((NCH, 5, NT, KH, LANES), bf16), vmem((NCH, 5, NT, KH, LANES), bf16),
            vmem((7, FT, RH, LANES), bf16), vmem((7, FT, TH, LANES), bf16),
            vmem((D, S), bf16),
            vmem((TPB, 8, LANES), f32), vmem((16, LANES), u32),
            pltpu.SemaphoreType.DMA((19,)), pltpu.SemaphoreType.DMA((3 * NB,)),
        ],
        compiler_params=pltpu.CompilerParams(
            vmem_limit_bytes=120 * 2**20, disable_bounds_checks=True, disable_semaphore_checks=True),
    )(A_x.reshape(S, D).T, A_wqkv, A_wo, B_w_gate, B_w_up, B_w_down.T, c, w_mod)
    return outT.T.reshape(1, S, D)
```
